```python
import jax
import jax.numpy as jnp

def _softmax(x, axis=-1):
    return jax.nn.softmax(x, axis=axis)

def _gelu(x):
    return jax.nn.gelu(x, approximate=True)

def _silu(x):
    return jax.nn.silu(x)

def _sigmoid(x):
    return jax.nn.sigmoid(x)

def _layernorm(x, axis=-1, eps=1e-05):
    m = jnp.mean(x, axis=axis, keepdims=True)
    v = jnp.var(x, axis=axis, keepdims=True)
    return (x - m) / jnp.sqrt(v + eps)

def _scatter_add(tgt, idx, src, axis=0):
    return tgt.at[idx].add(src)

def _segment_sum(src, seg, n):
    return jax.ops.segment_sum(src, seg, n)

class _Rng:

    def __init__(self, key):
        self._k = key

    def _next(self):
        self._k, sub = jax.random.split(self._k)
        return sub

    def normal(self, shape):
        return jax.random.normal(self._next(), shape, dtype=jnp.bfloat16)

    def randint(self, lo, hi, shape):
        return jax.random.randint(self._next(), shape, lo, hi, dtype=jnp.int32)

    def uniform(self, shape, lo=0.0, hi=1.0):
        return jax.random.uniform(self._next(), shape, jnp.bfloat16, lo, hi)

    def permutation(self, n):
        return jax.random.permutation(self._next(), n)
kernel_name = 'adaLN_cond__spectral_gfnet__mixer_token_mlp__prompt'

def setup_inputs():
    _rng = _Rng(jax.random.key(int.from_bytes(__import__("os").urandom(4), "little")))
    _w = lambda a: (lambda t: t.astype(jnp.bfloat16) if jnp.issubdtype(t.dtype, jnp.floating) else t)(jnp.asarray(a))

    def _A_setup():
        B, S, D = (1, 2048, 576)
        Df = D // 2 + 1
        return {'x': _w((lambda *s: _rng.normal(s) * 0.05)(B, S, D)), 'w_r': _w((lambda *s: _rng.normal(s) * 0.05)(S, Df) * 0.02), 'w_i': _w((lambda *s: _rng.normal(s) * 0.05)(S, Df) * 0.02)}
    _A_in = _A_setup()

    def _B_setup():
        B, S, D, F = (1, 2048, 576, 4608)
        return {'x': _w((lambda *s: _rng.normal(s) * 0.05)(B, S, D)), 'w1': _w((lambda *s: _rng.normal(s) * 0.05)(S, F) * S ** (-0.5)), 'b1': _w((lambda *s: _rng.normal(s) * 0.05)(F) * 0.02), 'w2': _w((lambda *s: _rng.normal(s) * 0.05)(F, S) * F ** (-0.5)), 'b2': _w((lambda *s: _rng.normal(s) * 0.05)(S) * 0.02)}
    _B_in = _B_setup()
    return {'A_x': _A_in['x'], 'A_w_r': _A_in['w_r'], 'A_w_i': _A_in['w_i'], 'B_x': _B_in['x'], 'B_w1': _B_in['w1'], 'B_b1': _B_in['b1'], 'B_w2': _B_in['w2'], 'B_b2': _B_in['b2'], 'c': _w((lambda *s: _rng.normal(s) * 0.05)(1, 576)), 'w_mod': _w((lambda *s: _rng.normal(s) * 0.05)(576, 6 * 576) * 576 ** (-0.5))}

def reference(A_x, A_w_r, A_w_i, B_x, B_w1, B_b1, B_w2, B_b2, c, w_mod):

    def _A_ref(x, w_r, w_i):
        B, S, D = x.shape
        X = (lambda x, axes=(-2, -1): jnp.fft.rfft2(x.astype(jnp.float32), axes=axes))(x, axes=(-2, -1))
        W = w_r + 1j * w_i
        X = X * W
        y = (lambda x, s, axes=(-2, -1): jnp.fft.irfft2(x, s=s, axes=axes).astype(jnp.bfloat16))(X, (S, D), axes=(-2, -1))
        return y

    def _B_ref(x, w1, b1, w2, b2):
        B, S, D = x.shape
        h = _layernorm(x, axis=-1)
        u = jnp.einsum('bsd,sf->bdf', h, w1) + b1
        u = _gelu(u)
        y = jnp.einsum('bdf,fs->bds', u, w2) + b2
        return (lambda x, *d: x.transpose(*d))(y, 0, 2, 1)
    x = A_x
    mod = (_silu(c) @ w_mod).reshape(c.shape[0], 6, 1, -1)
    sa, ca, ga, sb, cb, gb = (mod[:, 0].copy(), mod[:, 1].copy(), mod[:, 2].copy(), mod[:, 3].copy(), mod[:, 4].copy(), mod[:, 5].copy())
    h = _layernorm(x, axis=-1) * (1 + ca) + sa
    x = x + ga * _A_ref(h, A_w_r, A_w_i)
    h = _layernorm(x, axis=-1) * (1 + cb) + sb
    x = x + gb * _B_ref(h, B_w1, B_b1, B_w2, B_b2)
    return x
```

```python
import math

import jax
import jax.numpy as jnp
import numpy as np
from jax import lax
import jax.experimental.pallas as pl
import jax.experimental.pallas.tpu as pltpu

S, D, F = 2048, 576, 4608
DF = D // 2 + 1
EPS = 1e-5
NT = S // 128
G0 = 40
ZR = 4 * 128 + 2 * G0
WROWS = 296

_C9 = [math.cos(2 * math.pi * j / 9) for j in range(9)]
_S9 = [math.sin(2 * math.pi * j / 9) for j in range(9)]


def _sigmas(r):
    if r == 0:
        return [0, 9]
    return [r, r + 9, 9 - r, 18 - r]


def _constants():
    dp = np.arange(64)
    ff = np.zeros((5, 128, 128))
    fi = np.zeros((5, 128, 128))
    scale = 1.0 / (D * S)
    for r in range(1, 5):
        l = np.array([18 * m + sg for sg in _sigmas(r) for m in range(16)])
        th = 2 * np.pi * np.outer(l, dp) / D
        sg = np.where(l % 9 == r, 1.0, -1.0)[:, None]
        co, si = np.cos(th), np.sin(th)
        ff[r - 1] = np.block([[co, -_S9[3] * sg * si], [-si, -_S9[3] * sg * co]])
        fi[r - 1] = 2 * scale * np.block(
            [[co.T, -si.T], [_S9[3] * (sg * si).T, _S9[3] * (sg * co).T]])
    l = np.array([18 * m + sg for sg in _sigmas(0) for m in range(16)] + [D // 2])
    th = 2 * np.pi * np.outer(l, dp) / D
    edge = (l == 0) | (l == D // 2)
    co, si = np.cos(th), np.where(edge[:, None], 0.0, np.sin(th))
    ff[4, :33, :64] = co
    ff[4, G0:G0 + 33, :64] = -si
    cl = np.where(edge, 1.0, 2.0)[None, :]
    fi[4, :64, :33] = scale * cl * co.T
    fi[4, :64, G0:G0 + 33] = -scale * cl * si.T
    b = np.arange(128)
    p = np.arange(128)
    g = np.zeros((NT, 256, 128))
    for k1 in range(NT):
        k = 128 * ((p // 8 - k1) % 16) + 16 * (p % 8) + k1
        th = 2 * np.pi * ((np.outer(b, k) % S) / S)
        g[k1, :128] = np.cos(th)
        g[k1, 128:] = -np.sin(th)
    bf = jnp.bfloat16
    return np.concatenate([ff, fi], 0).astype(np.float32).astype(bf), g.astype(np.float32).astype(bf)


_FMAT, _GMAT = _constants()


def _radix9_even(h0, e1, e2, e3, e4):
    p = h0 + e3
    q = e1 + e2 + e4
    t0 = p + q
    t3 = p - 0.5 * q
    g = h0 - 0.5 * e3
    u = e1 - e4
    v = e2 - e4
    a = _C9[1] * u + _C9[2] * v
    b = _C9[2] * u + _C9[4] * v
    return t0, g + a, g + b, t3, g - a - b


def _radix9_odd(o1, o2, o3, o4):
    t3 = o1 - o2 + o4
    u = o1 + o2
    v = o2 + o4
    a = (_S9[1] / _S9[3]) * u + (_S9[4] / _S9[3]) * v
    b = (_S9[2] / _S9[3]) * u - (_S9[1] / _S9[3]) * v
    return a + o3, b - o3, t3, b - a + o3


def _radix4(z0, z1, z2, z3, sign):
    ar, ai = z0[0] + z2[0], z0[1] + z2[1]
    br, bi = z0[0] - z2[0], z0[1] - z2[1]
    cr, ci = z1[0] + z3[0], z1[1] + z3[1]
    dr, di = z1[0] - z3[0], z1[1] - z3[1]
    plus = (br - di, bi + dr)
    minus = (br + di, bi - dr)
    if sign > 0:
        return (ar + cr, ai + ci), plus, (ar - cr, ai - ci), minus
    return (ar + cr, ai + ci), minus, (ar - cr, ai - ci), plus


def _twiddle16(z, n, sign):
    zr, zi = z
    n %= 16
    if n == 0:
        return z
    if n == 4:
        return (-zi, zr) if sign > 0 else (zi, -zr)
    c = math.cos(2 * math.pi * n / 16)
    s = sign * math.sin(2 * math.pi * n / 16)
    if n % 4 == 2:
        if (c > 0) == (s > 0):
            return c * (zr - zi), c * (zr + zi)
        return c * (zr + zi), c * (zi - zr)
    return c * zr - s * zi, c * zi + s * zr


def _radix16(z, sign):
    u = [_radix4(z[a1], z[a1 + 4], z[a1 + 8], z[a1 + 12], sign) for a1 in range(4)]
    out = [None] * 16
    for q1 in range(4):
        t = [_twiddle16(u[a1][q1], a1 * q1, sign) for a1 in range(4)]
        y = _radix4(*t, sign)
        for q2 in range(4):
            out[q1 + 4 * q2] = y[q2]
    return out


def _gelu(x):
    k = math.sqrt(2 / math.pi)
    inner = x * (k + (k * 0.044715) * (x * x))
    hx = 0.5 * x
    return hx + hx * jnp.tanh(inner)


def _colsum(parts):
    acc = parts[0]
    for p in parts[1:]:
        acc = acc + p
    return jnp.sum(acc, axis=0, keepdims=True)


XCH = 4
FC = 512
SC = 256


def _kernel(x_hbm, wr_hbm, wi_hbm, w1_hbm, w2_hbm, wm_hbm, f_hbm, g_hbm, b1_ref, b2_ref, c_ref,
            out_hbm,
            x_v, wr_v, wi_v, w1_v, w2_v, wm_v, f_v, g_v, mod_v, wp_v, t_v, z_v, y_v, q_v, v_v,
            x1_v, h2_v, hid_v, out_v, sem_in, sem_w1, sem_w2, sem_out):
    f32 = jnp.float32
    xw = S // XCH

    def x_copy(i):
        return pltpu.make_async_copy(x_hbm.at[:, pl.ds(i * xw, xw)], x_v.at[:, pl.ds(i * xw, xw)], sem_in.at[i])

    def wm_copy(i):
        return pltpu.make_async_copy(wm_hbm.at[:, pl.ds(i * 1152, 1152)], wm_v.at[:, pl.ds(i * 1152, 1152)],
                                     sem_in.at[XCH + i])

    f_copy = pltpu.make_async_copy(f_hbm, f_v, sem_in.at[XCH + 3])
    g_copy = pltpu.make_async_copy(g_hbm, g_v, sem_in.at[XCH + 4])
    wr_copy = pltpu.make_async_copy(wr_hbm, wr_v, sem_in.at[XCH + 5])
    wi_copy = pltpu.make_async_copy(wi_hbm, wi_v, sem_in.at[XCH + 6])

    def w1_copy(j):
        off = pl.multiple_of(j * FC, FC)
        return pltpu.make_async_copy(w1_hbm.at[:, pl.ds(off, FC)], w1_v.at[j], sem_w1.at[j])

    def w2_copy(j):
        off = pl.multiple_of(j * SC, SC)
        return pltpu.make_async_copy(w2_hbm.at[:, pl.ds(off, SC)], w2_v.at[j], sem_w2.at[j])

    def out_copy(j):
        off = pl.multiple_of(j * SC, SC)
        return pltpu.make_async_copy(out_v.at[j], out_hbm.at[:, pl.ds(off, SC)], sem_out.at[j])

    wm_copy(0).start()
    for i in range(XCH):
        x_copy(i).start()
    f_copy.start()
    wr_copy.start()
    wi_copy.start()
    g_copy.start()
    wm_copy(1).start()
    wm_copy(2).start()
    for j in range(F // FC):
        w1_copy(j).start()
    for j in range(S // SC):
        w2_copy(j).start()

    cc = c_ref[...].astype(f32)
    act = jnp.broadcast_to(cc * jax.nn.sigmoid(cc), (8, D))

    def modulation(i):
        wm_copy(i).wait()
        row = jnp.dot(act, wm_v[:, i * 1152:(i + 1) * 1152], preferred_element_type=f32)
        for t in range(9):
            tile = jnp.broadcast_to(row[0:1, t * 128:(t + 1) * 128], (128, 128))
            mod_v[pl.ds(i * 1152 + t * 128, 128), :] = tile.T

    def mod_col(which, r0, n):
        return mod_v[pl.ds(which * D + r0, n), :]

    modulation(0)
    f_copy.wait()

    def stage1(t):
        cols = pl.ds(pl.multiple_of(t * 128, 128), 128)
        m = _colsum([x_v[pl.ds(16 * i, 16), cols].astype(f32) for i in range(D // 16)]) * (1.0 / D)
        sq = []
        for i in range(D // 16):
            d = x_v[pl.ds(16 * i, 16), cols].astype(f32) - m
            sq.append(d * d)
        rs = lax.rsqrt(_colsum(sq) * (1.0 / D) + EPS)
        for i in range(4):
            h = []
            for a in range(9):
                r0 = 64 * a + 16 * i
                n = (x_v[pl.ds(r0, 16), cols].astype(f32) - m) * rs
                h.append(n * (1.0 + mod_col(1, r0, 16)) + mod_col(0, r0, 16))
            e = [h[a] + h[9 - a] for a in range(1, 5)]
            o = [h[a] - h[9 - a] for a in range(1, 5)]
            te = _radix9_even(h[0], *e)
            to = _radix9_odd(*o)
            t_v[pl.ds(512 + 16 * i, 16), :] = te[0]
            for r in range(4):
                t_v[pl.ds(128 * r + 16 * i, 16), :] = te[r + 1]
                t_v[pl.ds(128 * r + 64 + 16 * i, 16), :] = to[r]
        for r in range(4):
            z_v[pl.ds(128 * r, 128), cols] = jnp.dot(
                f_v[r], t_v[pl.ds(128 * r, 128), :].astype(jnp.bfloat16), preferred_element_type=f32)
        z_v[pl.ds(512, 2 * G0), cols] = jnp.dot(
            f_v[4, 0:2 * G0, 0:64], t_v[pl.ds(512, 64), :].astype(jnp.bfloat16), preferred_element_type=f32)

    for i in range(XCH):
        x_copy(i).wait()
        per = NT // XCH
        lax.fori_loop(i * per, (i + 1) * per, lambda t, _: (stage1(t), 0)[1], 0)

    wr_copy.wait()
    wi_copy.wait()
    lane = lax.broadcasted_iota(jnp.int32, (8, 128), 1)
    grp = lane >> 3

    def permute(tiles, row0):
        a = [None] * NT
        for ct in range(NT):
            idx = ((lane & 7) << 4) + ((grp - ct) & 15)
            a[(-ct) % NT] = jnp.take_along_axis(tiles[ct], idx, axis=1)
        for bit in range(4):
            mask = ((grp >> bit) & 1) == 1
            a = [jnp.where(mask, a[(m - (1 << bit)) % NT], a[m]) for m in range(NT)]
        for k1 in range(NT):
            wp_v[k1, pl.ds(row0, 8), :] = a[k1]

    def wbody(i, _):
        rows = pl.ds(pl.multiple_of(i * 16, 16), 16)
        for src, base in ((wr_v, 0), (wi_v, 144)):
            tiles = [pltpu.bitcast(src[rows, ct * 128:(ct + 1) * 128], jnp.int32) for ct in range(NT)]
            permute(tiles, pl.multiple_of(base + i * 8, 8))
        return 0

    lax.fori_loop(0, 18, wbody, 0)
    tiles = []
    for ct in range(NT):
        lo = pltpu.bitcast(jnp.broadcast_to(wr_v[288:289, ct * 128:(ct + 1) * 128].astype(f32), (8, 128)), jnp.int32)
        hi = pltpu.bitcast(jnp.broadcast_to(wi_v[288:289, ct * 128:(ct + 1) * 128].astype(f32), (8, 128)), jnp.int32)
        tiles.append(lax.shift_right_logical(lo, 16) | hi)
    permute(tiles, 288)

    def butterflies(src, dst, sign):
        def one(re0, im0):
            z = [(src[pl.ds(re0, 8), a * 128:(a + 1) * 128], src[pl.ds(im0, 8), a * 128:(a + 1) * 128])
                 for a in range(NT)]
            y = _radix16(z, sign)
            for k in range(NT):
                dst[pl.ds(re0, 8), k * 128:(k + 1) * 128] = y[k][0]
                dst[pl.ds(im0, 8), k * 128:(k + 1) * 128] = y[k][1]

        def body(i, _):
            re0 = pl.multiple_of((i >> 3) * 128 + (i & 7) * 8, 8)
            one(re0, pl.multiple_of(re0 + 64, 8))
            return 0

        lax.fori_loop(0, 32, body, 0)

        def body0(i, _):
            re0 = pl.multiple_of(512 + i * 8, 8)
            one(re0, pl.multiple_of(re0 + G0, 8))
            return 0

        lax.fori_loop(0, G0 // 8, body0, 0)

    butterflies(z_v, y_v, -1)
    g_copy.wait()

    def unpack(u, half):
        bits = (u << 16) if half == 0 else (u & jnp.int32(-65536))
        return pltpu.bitcast(bits, f32)

    def spectral(k1, _):
        cols = pl.ds(pl.multiple_of(k1 * 128, 128), 128)
        y = y_v[:, cols]
        yc = jnp.dot(y, g_v[k1, 0:128, :], preferred_element_type=f32)
        ys = jnp.dot(y, g_v[k1, 128:256, :], preferred_element_type=f32)
        pieces = {}
        for r in (1, 2, 3, 4, 0):
            base, n = (128 * (r - 1), 64) if r else (512, G0)
            filt = []
            for sg in _sigmas(r):
                wr = unpack(wp_v[k1, pl.ds(sg // 2, 16, stride=9), :], sg % 2)
                wi = unpack(wp_v[k1, pl.ds(144 + sg // 2, 16, stride=9), :], sg % 2)
                filt.append((wr, wi))
            if r == 0:
                u = wp_v[k1, 288:296, :]
                filt.append((unpack(u, 0), unpack(u, 1)))
            o = 0
            for wr, wi in filt:
                h = wr.shape[0]
                re, im = base + o, base + n + o
                xr = yc[re:re + h] - ys[im:im + h]
                xi = ys[re:re + h] + yc[im:im + h]
                pieces[re] = xr * wr - xi * wi
                pieces[im] = xr * wi + xi * wr
                o += h
        fl = jnp.concatenate([pieces[k] for k in sorted(pieces)], axis=0)
        nt = (((1,), (1,)), ((), ()))
        fc = lax.dot_general(fl, g_v[k1, 0:128, :], nt, preferred_element_type=f32)
        fs = lax.dot_general(fl, g_v[k1, 128:256, :], nt, preferred_element_type=f32)
        for r in (1, 2, 3, 4, 0):
            base, n = (128 * (r - 1), 64) if r else (512, G0)
            re, im = base, base + n
            q_v[re:re + n, cols] = fc[re:re + n] + fs[im:im + n]
            q_v[im:im + n, cols] = fc[im:im + n] - fs[re:re + n]
        return 0

    lax.fori_loop(0, NT, spectral, 0)
    butterflies(q_v, v_v, +1)

    modulation(1)
    modulation(2)

    def stage5(t, _):
        cols = pl.ds(pl.multiple_of(t * 128, 128), 128)
        for r in range(4):
            t_v[pl.ds(128 * r, 128), :] = jnp.dot(
                f_v[5 + r], v_v[pl.ds(128 * r, 128), cols].astype(jnp.bfloat16), preferred_element_type=f32)
        t_v[pl.ds(512, 64), :] = jnp.dot(
            f_v[9, 0:64, 0:2 * G0], v_v[pl.ds(512, 2 * G0), cols].astype(jnp.bfloat16), preferred_element_type=f32)
        parts = []
        for i in range(4):
            pe = [t_v[pl.ds(512 + 16 * i, 16), :]] + [t_v[pl.ds(128 * r + 16 * i, 16), :] for r in range(4)]
            po = [t_v[pl.ds(128 * r + 64 + 16 * i, 16), :] for r in range(4)]
            ee = _radix9_even(*pe)
            oo = _radix9_odd(*po)
            ya = [ee[0]] + [ee[a] - oo[a - 1] for a in range(1, 5)] + [ee[a] + oo[a - 1] for a in (4, 3, 2, 1)]
            for a in range(9):
                r0 = 64 * a + 16 * i
                x1 = x_v[pl.ds(r0, 16), cols].astype(f32) + mod_col(2, r0, 16) * ya[a]
                x1_v[pl.ds(r0, 16), cols] = x1
                parts.append(x1)
        m = _colsum(parts) * (1.0 / D)
        sq = []
        for i in range(D // 16):
            d = x1_v[pl.ds(16 * i, 16), cols] - m
            sq.append(d * d)
        rs = lax.rsqrt(_colsum(sq) * (1.0 / D) + EPS)
        parts = []
        for i in range(D // 16):
            n = (x1_v[pl.ds(16 * i, 16), cols] - m) * rs
            h = n * (1.0 + mod_col(4, 16 * i, 16)) + mod_col(3, 16 * i, 16)
            t_v[pl.ds(16 * i, 16), :] = h
            parts.append(h)
        m2 = _colsum(parts) * (1.0 / D)
        sq = []
        for i in range(D // 16):
            d = t_v[pl.ds(16 * i, 16), :] - m2
            sq.append(d * d)
        rs2 = lax.rsqrt(_colsum(sq) * (1.0 / D) + EPS)
        for i in range(D // 16):
            h2_v[pl.ds(16 * i, 16), cols] = ((t_v[pl.ds(16 * i, 16), :] - m2) * rs2).astype(jnp.bfloat16)
        return 0

    lax.fori_loop(0, NT, stage5, 0)

    b1 = b1_ref[...].astype(f32)
    b2 = b2_ref[...].astype(f32)

    for j in range(F // FC):
        w1_copy(j).wait()
        u = jnp.dot(h2_v[...], w1_v[j], preferred_element_type=f32)
        for t in range(FC // 128):
            row = j * (FC // 128) + t
            ut = u[:, t * 128:(t + 1) * 128] + b1[row:row + 1, :]
            hid_v[:, row * 128:(row + 1) * 128] = _gelu(ut).astype(jnp.bfloat16)

    for j in range(S // SC):
        w2_copy(j).wait()
        y = jnp.dot(hid_v[...], w2_v[j], preferred_element_type=f32)
        for t in range(SC // 128):
            row = j * (SC // 128) + t
            yt = y[:, t * 128:(t + 1) * 128] + b2[row:row + 1, :]
            o = x1_v[:, row * 128:(row + 1) * 128] + mod_col(5, 0, D) * yt
            out_v[j, :, t * 128:(t + 1) * 128] = o.astype(jnp.bfloat16)
        out_copy(j).start()
    for j in range(S // SC):
        out_copy(j).wait()


@jax.jit
def pallas_adaLN_cond__spectral_gfnet__mixer_token_mlp__prompt_kernel(A_x, A_w_r, A_w_i, B_x, B_w1, B_b1, B_w2, B_b2, c, w_mod):
    del B_x
    bf, f32 = jnp.bfloat16, jnp.float32
    hbm = pl.BlockSpec(memory_space=pl.ANY)
    vmem = pl.BlockSpec(memory_space=pltpu.VMEM)
    out_t = pl.pallas_call(
        _kernel,
        out_shape=jax.ShapeDtypeStruct((D, S), bf),
        in_specs=[hbm] * 8 + [vmem] * 3,
        out_specs=hbm,
        scratch_shapes=[
            pltpu.VMEM((D, S), bf),
            pltpu.VMEM((DF, S), bf),
            pltpu.VMEM((DF, S), bf),
            pltpu.VMEM((F // FC, S, FC), bf),
            pltpu.VMEM((S // SC, F, SC), bf),
            pltpu.VMEM((D, 6 * D), bf),
            pltpu.VMEM(_FMAT.shape, bf),
            pltpu.VMEM(_GMAT.shape, bf),
            pltpu.VMEM((6 * D, 128), f32),
            pltpu.VMEM((NT, WROWS, 128), jnp.int32),
            pltpu.VMEM((D, 128), f32),
            pltpu.VMEM((ZR, S), f32),
            pltpu.VMEM((ZR, S), f32),
            pltpu.VMEM((ZR, S), f32),
            pltpu.VMEM((ZR, S), f32),
            pltpu.VMEM((D, S), f32),
            pltpu.VMEM((D, S), bf),
            pltpu.VMEM((D, F), bf),
            pltpu.VMEM((S // SC, D, SC), bf),
            pltpu.SemaphoreType.DMA((XCH + 7,)),
            pltpu.SemaphoreType.DMA((F // FC,)),
            pltpu.SemaphoreType.DMA((S // SC,)),
            pltpu.SemaphoreType.DMA((S // SC,)),
        ],
        compiler_params=pltpu.CompilerParams(vmem_limit_bytes=110 * 1024 * 1024),
    )(A_x[0].T, A_w_r.T, A_w_i.T, B_w1, B_w2, w_mod, _FMAT, _GMAT,
      B_b1.reshape(F // 128, 128), B_b2.reshape(S // 128, 128), c)
    return out_t.T[None]
```

```python
import contextlib
import math

import jax
import jax.numpy as jnp
import numpy as np
from jax import lax
import jax.experimental.pallas as pl
import jax.experimental.pallas.tpu as pltpu

S, D, F = 2048, 576, 4608
DF = D // 2 + 1
EPS = 1e-5
NT = S // 128
G0 = 40
NL = 4 * 64 + G0
WROWS = 296
H = D // 2

XCH = 8
FC = 768
SC = 512
SCOPES = False

_C9 = [math.cos(2 * math.pi * j / 9) for j in range(9)]
_S9 = [math.sin(2 * math.pi * j / 9) for j in range(9)]


def _scope(name):
    return jax.named_scope(name) if SCOPES else contextlib.nullcontext()


def _sigmas(r):
    if r == 0:
        return [0, 9]
    return [r, r + 9, 9 - r, 18 - r]


def _pack_rows(m):
    u = m.astype(np.float32).astype(jnp.bfloat16).view(np.uint16).astype(np.uint32)
    return (u[..., 0::2, :] | (u[..., 1::2, :] << 16)).view(np.int32)


def _constants():
    dp = np.arange(64)
    ff = np.zeros((5, 128, 128))
    fi = np.zeros((5, 128, 128))
    scale = 1.0 / (D * S)
    for r in range(1, 5):
        l = np.array([18 * m + sg for sg in _sigmas(r) for m in range(16)])
        th = 2 * np.pi * np.outer(l, dp) / D
        sg = np.where(l % 9 == r, 1.0, -1.0)[:, None]
        co, si = np.cos(th), np.sin(th)
        ff[r - 1] = np.block([[co, -_S9[3] * sg * si], [-si, -_S9[3] * sg * co]])
        fi[r - 1] = 2 * scale * np.block(
            [[co.T, -si.T], [_S9[3] * (sg * si).T, _S9[3] * (sg * co).T]])
    l = np.array([18 * m + sg for sg in _sigmas(0) for m in range(16)] + [D // 2])
    th = 2 * np.pi * np.outer(l, dp) / D
    edge = (l == 0) | (l == D // 2)
    co, si = np.cos(th), np.where(edge[:, None], 0.0, np.sin(th))
    ff[4, :33, :64] = co
    ff[4, G0:G0 + 33, :64] = -si
    cl = np.where(edge, 1.0, 2.0)[None, :]
    fi[4, :64, :33] = scale * cl * co.T
    fi[4, :64, G0:G0 + 33] = -scale * cl * si.T
    b = np.arange(8)[:, None]
    p = np.arange(128)[None, :]
    k0 = 128 * (p // 8) + 16 * (p % 8)
    one = np.ones((8, 128))
    seeds = []
    for z in (np.exp(-2j * np.pi * b * k0 / S), np.exp(-2j * np.pi * 8 * k0 / S) * one,
              np.exp(2j * np.pi * 127 * b / S) * one, np.exp(2j * np.pi * 127 * 8 / S) * one):
        seeds += [z.real, z.imag]
    return _pack_rows(np.concatenate([ff, fi], 0)), np.concatenate(seeds, 0).astype(np.float32)


_FMAT, _SEEDS = _constants()


def _radix9_even(h0, e1, e2, e3, e4):
    p = h0 + e3
    q = e1 + e2 + e4
    t0 = p + q
    t3 = p - 0.5 * q
    g = h0 - 0.5 * e3
    u = e1 - e4
    v = e2 - e4
    a = _C9[1] * u + _C9[2] * v
    b = _C9[2] * u + _C9[4] * v
    return t0, g + a, g + b, t3, g - a - b


def _radix9_odd(o1, o2, o3, o4):
    t3 = o1 - o2 + o4
    u = o1 + o2
    v = o2 + o4
    a = (_S9[1] / _S9[3]) * u + (_S9[4] / _S9[3]) * v
    b = (_S9[2] / _S9[3]) * u - (_S9[1] / _S9[3]) * v
    return a + o3, b - o3, t3, b - a + o3


def _radix4(z0, z1, z2, z3, sign):
    ar, ai = z0[0] + z2[0], z0[1] + z2[1]
    br, bi = z0[0] - z2[0], z0[1] - z2[1]
    cr, ci = z1[0] + z3[0], z1[1] + z3[1]
    dr, di = z1[0] - z3[0], z1[1] - z3[1]
    plus = (br - di, bi + dr)
    minus = (br + di, bi - dr)
    if sign > 0:
        return (ar + cr, ai + ci), plus, (ar - cr, ai - ci), minus
    return (ar + cr, ai + ci), minus, (ar - cr, ai - ci), plus


def _twiddle16(z, n, sign):
    zr, zi = z
    n %= 16
    if n == 0:
        return z
    if n == 4:
        return (-zi, zr) if sign > 0 else (zi, -zr)
    c = math.cos(2 * math.pi * n / 16)
    s = sign * math.sin(2 * math.pi * n / 16)
    if n % 4 == 2:
        if (c > 0) == (s > 0):
            return c * (zr - zi), c * (zr + zi)
        return c * (zr + zi), c * (zi - zr)
    return c * zr - s * zi, c * zi + s * zr


def _radix16(z, sign):
    u = [_radix4(z[a1], z[a1 + 4], z[a1 + 8], z[a1 + 12], sign) for a1 in range(4)]
    out = [None] * 16
    for q1 in range(4):
        t = [_twiddle16(u[a1][q1], a1 * q1, sign) for a1 in range(4)]
        y = _radix4(*t, sign)
        for q2 in range(4):
            out[q1 + 4 * q2] = y[q2]
    return out


def _cmul(a, b):
    return a[0] * b[0] - a[1] * b[1], a[0] * b[1] + a[1] * b[0]


def _gelu(x):
    k = math.sqrt(2 / math.pi)
    inner = x * (k + (k * 0.044715) * (x * x))
    hx = 0.5 * x
    return hx + hx * jnp.tanh(inner)


def _colmean(parts):
    acc = [parts[0], parts[1]]
    for i, p in enumerate(parts[2:]):
        acc[i % 2] = acc[i % 2] + p
    return jnp.sum(acc[0] + acc[1], axis=0, keepdims=True) * (1.0 / D)


def _pack(x):
    return pltpu.bitcast(x.astype(jnp.bfloat16), jnp.int32)


def _unpack(x):
    return pltpu.bitcast(x, jnp.bfloat16)


def _dot(a, b):
    return jnp.dot(a, b, preferred_element_type=jnp.float32)


def _dot_nt(a, b):
    return lax.dot_general(a, b, (((1,), (1,)), ((), ())), preferred_element_type=jnp.float32)


def _strassen_lhs(a11, a12, a21, a22):
    return (a11 + a22, a21 + a22, a11, a22, a11 + a12, a21 - a11, a12 - a22)


def _strassen(lhs, rhs):
    f32, bf = jnp.float32, jnp.bfloat16

    def comb(i, first, second, sign):
        a, b = rhs(*first, i).astype(f32), rhs(*second, i).astype(f32)
        return (a + b if sign > 0 else a - b).astype(bf)

    m3 = _dot(lhs(2), comb(2, (0, 1), (1, 1), -1))
    m5 = _dot(lhs(4), rhs(1, 1, 4))
    yield 0, 1, m3 + m5
    m2 = _dot(lhs(1), rhs(0, 0, 1))
    m4 = _dot(lhs(3), comb(3, (1, 0), (0, 0), -1))
    yield 1, 0, m2 + m4
    m1 = _dot(lhs(0), comb(0, (0, 0), (1, 1), +1))
    m7 = _dot(lhs(6), comb(6, (1, 0), (1, 1), +1))
    yield 0, 0, m1 + m4 - m5 + m7
    m6 = _dot(lhs(5), comb(5, (0, 0), (0, 1), +1))
    yield 1, 1, m1 - m2 + m3 + m6


def _kernel(x_hbm, wr_hbm, wi_hbm, w1_hbm, w2_hbm, wm_hbm, f_hbm, seed_hbm, b1_hbm, b2_hbm, c_hbm,
            out_hbm,
            x_v, wr_v, wi_v, w1_v, w2_v, wm_v, f_v, seed_v, b1_v, b2_v, c_v, g_v, mod_v, wp_v, t_v,
            yr_v, yi_v, xr_v, xi_v, qr_v, qi_v, p_v, zs_v, x1_v, a1_v, a2_v, out_v, zero_s,
            sem_in, sem_x, sem_w1, sem_w2, sem_out):
    f32, bf = jnp.float32, jnp.bfloat16
    xw = S // XCH
    nfc, nsc = F // FC, S // SC
    fct, sct = FC // 128, SC // 128

    def x_copy(i):
        return pltpu.make_async_copy(x_hbm.at[:, pl.ds(i * xw, xw)], x_v.at[:, pl.ds(i * xw, xw)], sem_x.at[i])

    wm_parts = ((512, 1152), (0, 512), (1152, 2944), (2944, 6 * D))

    def wm_copy(i):
        lo, hi = wm_parts[i]
        return pltpu.make_async_copy(wm_hbm.at[:, lo:hi], wm_v.at[:, lo:hi], sem_in.at[i])

    small = [pltpu.make_async_copy(s, d, sem_in.at[4 + i]) for i, (s, d) in enumerate(
        ((seed_hbm, seed_v), (c_hbm, c_v), (f_hbm, f_v), (wr_hbm, wr_v), (wi_hbm, wi_v),
         (b1_hbm, b1_v), (b2_hbm, b2_v)))]
    seed_copy, c_copy, f_copy, wr_copy, wi_copy, b1_copy, b2_copy = small

    def w1_copies(j):
        return [pltpu.make_async_copy(w1_hbm.at[:, pl.ds(pl.multiple_of((j * fct + t) * 128, 128), 128)],
                                      w1_v.at[j * fct + t], sem_w1.at[j]) for t in range(fct)]

    def w2_copies(j):
        return [pltpu.make_async_copy(w2_hbm.at[:, pl.ds(pl.multiple_of((j * sct + t) * 128, 128), 128)],
                                      w2_v.at[j * sct + t], sem_w2.at[j]) for t in range(sct)]

    def out_copy(j, p, q):
        col = pl.multiple_of(j * SC + q * (SC // 2), SC // 2)
        return pltpu.make_async_copy(out_v.at[j, p, q], out_hbm.at[pl.ds(p * H, H), pl.ds(col, SC // 2)],
                                     sem_out.at[j * 4 + p * 2 + q])

    def start(copies):
        for cp in copies:
            cp.start()

    def wait(copies):
        for cp in copies:
            cp.wait()

    start([seed_copy, c_copy, wm_copy(0), x_copy(0)])
    for i in range(8):
        zero_s[i] = 0

    with _scope("twiddle"):
        seed_copy.wait()
        start([x_copy(1)])
        sd = [seed_v[8 * i:8 * i + 8, :] for i in range(8)]
        g0, tau = [(sd[0], sd[1])], [(sd[4], sd[5])]
        for i in range(15):
            g0.append(_cmul(g0[-1], (sd[2], sd[3])))
            tau.append(_cmul(tau[-1], (sd[6], sd[7])))
        for i in range(8):
            g = [g0[2 * i], g0[2 * i + 1]]
            for k1 in range(NT):
                gr = jnp.concatenate([g[0][0], g[1][0]], axis=0)
                gi = jnp.concatenate([g[0][1], g[1][1]], axis=0)
                g_v[k1, 0, 8 * i:8 * i + 8, :] = _pack(gr)
                g_v[k1, 1, 8 * i:8 * i + 8, :] = _pack(gi - gr)
                g_v[k1, 2, 8 * i:8 * i + 8, :] = _pack(gi + gr)
                if k1 + 1 < NT:
                    g = [_cmul(g[0], tau[2 * i]), _cmul(g[1], tau[2 * i + 1])]

    with _scope("mod0"):
        c_copy.wait()
        start([x_copy(2)])
        cc = c_v[...].astype(f32)
        act = jnp.broadcast_to(cc * jax.nn.sigmoid(cc), (8, D))

        def modulation(i):
            lo, hi = wm_parts[i]
            row = _dot(act, wm_v[:, lo:hi])
            for t in range((hi - lo) // 128):
                tile = jnp.broadcast_to(row[0:1, t * 128:(t + 1) * 128], (128, 128))
                mod_v[lo + t * 128:lo + (t + 1) * 128, :] = tile.T

        def mod_col(which, r0, n):
            return mod_v[pl.ds(which * D + r0, n), :]

        wm_copy(0).wait()
        start([x_copy(3)])
        modulation(0)
        mod_v[D:2 * D, :] = 1.0 + mod_v[D:2 * D, :]

    def radix9_fwd(rows):
        for i in range(4):
            h = [rows(64 * a + 16 * i) for a in range(9)]
            e = [h[a] + h[9 - a] for a in range(1, 5)]
            o = [h[a] - h[9 - a] for a in range(1, 5)]
            te = _radix9_even(h[0], *e)
            to = _radix9_odd(*o)
            yield 256 + 8 * i, _pack(te[0])
            for r in range(4):
                yield 64 * r + 8 * i, _pack(te[r + 1])
                yield 64 * r + 32 + 8 * i, _pack(to[r])

    def stage1(t):
        cols = pl.ds(t * 128, 128)
        xs = [x_v[pl.ds(16 * i, 16), cols].astype(f32) for i in range(D // 16)]
        m = _colmean(xs)
        ds = [v - m for v in xs]
        rs = lax.rsqrt(_colmean([d * d for d in ds]) + EPS)
        for r0, piece in radix9_fwd(lambda r0: ds[r0 // 16] * rs * mod_col(1, r0, 16)):
            t_v[pl.ds(r0, 8), cols] = piece

    later = {4: [f_copy], 5: [wr_copy], 6: [wi_copy], 7: [wm_copy(1)]}
    for i in range(XCH):
        with _scope("xwait%d" % i):
            x_copy(i).wait()
            start([x_copy(i + 4)] if i + 4 < XCH else later[i])
        with _scope("stage1_%d" % i):
            for t in range(NT // XCH):
                stage1(i * (NT // XCH) + t)

    def d_forward(r, tmat):
        if r < 4:
            return _dot(_unpack(f_v[r]), _unpack(tmat(64 * r, 64))), 64
        return _dot(_unpack(f_v[4, 0:G0, 0:64]), _unpack(tmat(256, 32))), G0

    def tiles(v, r0):
        return [v[r0:r0 + 8, a * 128:(a + 1) * 128] for a in range(NT)]

    with _scope("fwait"):
        f_copy.wait()
        start([wm_copy(2), b1_copy, b2_copy])
    with _scope("dfwd"):
        for r in range(5):
            z, n = d_forward(r, lambda r0, k: t_v[r0:r0 + k, :])
            for i in range(0, n, 8):
                y = _radix16(list(zip(tiles(z, i), tiles(z, n + i))), -1)
                for k in range(NT):
                    yr_v[k, 64 * r + i:64 * r + i + 8, :] = y[k][0]
                    yi_v[k, 64 * r + i:64 * r + i + 8, :] = y[k][1]

    def s_forward(k1):
        yr, yi = yr_v[k1], yi_v[k1]
        k = _dot(yr + yi, _unpack(g_v[k1, 0]))
        xr_v[k1] = k - _dot(yi, _unpack(g_v[k1, 2]))
        xi_v[k1] = k + _dot(yr, _unpack(g_v[k1, 1]))

    with _scope("sfwd_a"):
        for k1 in range(NT // 2):
            s_forward(k1)

    with _scope("wwait"):
        wr_copy.wait()
        wi_copy.wait()
        start(w1_copies(0))
    lane = lax.broadcasted_iota(jnp.int32, (8, 128), 1)
    grp = lane >> 3

    def permute(src, row0):
        a = [None] * NT
        for ct in range(NT):
            idx = ((lane & 7) << 4) + ((grp - ct) & 15)
            a[(-ct) % NT] = jnp.take_along_axis(src[ct], idx, axis=1)
        for bit in range(4):
            mask = ((grp >> bit) & 1) == 1
            a = [jnp.where(mask, a[(m - (1 << bit)) % NT], a[m]) for m in range(NT)]
        for k1 in range(NT):
            wp_v[k1, pl.ds(row0, 8), :] = a[k1]

    with _scope("sfwd_b_wperm"):
        for k1 in range(NT // 2, NT):
            s_forward(k1)
        for i in range(18):
            for src, base in ((wr_v, 0), (wi_v, 144)):
                permute([pltpu.bitcast(src[16 * i:16 * i + 16, ct * 128:(ct + 1) * 128], jnp.int32)
                         for ct in range(NT)], base + 8 * i)
        last = []
        for ct in range(NT):
            lo, hi = [pltpu.bitcast(jnp.broadcast_to(w[288:289, ct * 128:(ct + 1) * 128].astype(f32), (8, 128)),
                                    jnp.int32) for w in (wr_v, wi_v)]
            last.append(lax.shift_right_logical(lo, 16) | hi)
        permute(last, 288)

    with _scope("sa"):
        wm_copy(1).wait()
        start(w1_copies(1))
        modulation(1)
        for r0, piece in radix9_fwd(lambda r0: mod_col(0, r0, 16)):
            zs_v[pl.ds(r0, 8), :] = piece
        first = lax.broadcasted_iota(jnp.int32, (1, 128), 1) == 0
        for r in range(5):
            z, n = d_forward(r, lambda r0, k: zs_v[r0:r0 + k, :])
            z = jnp.where(first, z * float(S), 0.0)
            xr_v[0, 64 * r:64 * r + n, :] = xr_v[0, 64 * r:64 * r + n, :] + z[0:n]
            xi_v[0, 64 * r:64 * r + n, :] = xi_v[0, 64 * r:64 * r + n, :] + z[n:2 * n]

    def half_f32(u, half):
        bits = (u << 16) if half == 0 else (u & jnp.int32(-65536))
        return pltpu.bitcast(bits, f32)

    def s_inverse(k1):
        wr, wi = [], []
        for r in (1, 2, 3, 4, 0):
            for sg in _sigmas(r):
                wr.append(half_f32(wp_v[k1, pl.ds(sg // 2, 16, stride=9), :], sg % 2))
                wi.append(half_f32(wp_v[k1, pl.ds(144 + sg // 2, 16, stride=9), :], sg % 2))
        u = wp_v[k1, 288:296, :]
        wr = jnp.concatenate(wr + [half_f32(u, 0)], axis=0)
        wi = jnp.concatenate(wi + [half_f32(u, 1)], axis=0)
        xr, xi = xr_v[k1], xi_v[k1]
        fr = xr * wr - xi * wi
        fi = xr * wi + xi * wr
        k = _dot_nt(fr + fi, _unpack(g_v[k1, 0]))
        qr_v[k1] = k + _dot_nt(fi, _unpack(g_v[k1, 1]))
        qi_v[k1] = k - _dot_nt(fr, _unpack(g_v[k1, 2]))

    with _scope("sinv"):
        for k1 in range(NT):
            s_inverse(k1)

    with _scope("dinv"):
        wm_copy(2).wait()
        start(w1_copies(2))
        for r in range(5):
            n = 64 if r < 4 else G0
            vr, vi = [], []
            for i in range(0, n, 8):
                rows = slice(64 * r + i, 64 * r + i + 8)
                v = _radix16([(qr_v[k, rows, :], qi_v[k, rows, :]) for k in range(NT)], +1)
                vr.append(jnp.concatenate([e[0] for e in v], axis=1))
                vi.append(jnp.concatenate([e[1] for e in v], axis=1))
            vmat = jnp.concatenate(vr + vi, axis=0).astype(bf)
            if r < 4:
                p_v[128 * r:128 * r + 128, :] = _dot(_unpack(f_v[5 + r]), vmat)
            else:
                p_v[512:576, :] = _dot(_unpack(f_v[9, 0:32, 0:2 * G0]), vmat)
        modulation(2)
        mod_v[4 * D:5 * D, :] = 1.0 + mod_v[4 * D:5 * D, :]

    def stage5(t):
        cols = pl.ds(pl.multiple_of(t * 128, 128), 128)
        x1 = [None] * (D // 16)
        for i in range(4):
            pe = [p_v[pl.ds(512 + 16 * i, 16), cols]] + [p_v[pl.ds(128 * r + 16 * i, 16), cols] for r in range(4)]
            po = [p_v[pl.ds(128 * r + 64 + 16 * i, 16), cols] for r in range(4)]
            ee = _radix9_even(*pe)
            oo = _radix9_odd(*po)
            ya = [ee[0]] + [ee[a] - oo[a - 1] for a in range(1, 5)] + [ee[a] + oo[a - 1] for a in (4, 3, 2, 1)]
            for a in range(9):
                r0 = 64 * a + 16 * i
                v = x_v[pl.ds(r0, 16), cols].astype(f32) + mod_col(2, r0, 16) * ya[a]
                x1_v[pl.ds(r0, 16), cols] = v
                x1[r0 // 16] = v
        m = _colmean(x1)
        ds = [v - m for v in x1]
        rs = lax.rsqrt(_colmean([d * d for d in ds]) + EPS)
        hs = [d * rs * mod_col(4, 16 * i, 16) + mod_col(3, 16 * i, 16) for i, d in enumerate(ds)]
        m = _colmean(hs)
        ds = [v - m for v in hs]
        rs = lax.rsqrt(_colmean([d * d for d in ds]) + EPS)
        return [d * rs for d in ds]

    def stage5_pair(t, _):
        left, right = stage5(2 * t), stage5(2 * t + 1)
        cols = pl.ds(pl.multiple_of(t * 128, 128), 128)
        for i in range(H // 16):
            ops = _strassen_lhs(left[i], right[i], left[H // 16 + i], right[H // 16 + i])
            for n, op in enumerate(ops):
                a1_v[n, pl.ds(8 * i, 8), cols] = _pack(op)
        return 0

    with _scope("stage5"):
        start(w1_copies(3))
        lax.fori_loop(0, NT // 2, stage5_pair, 0)
        b1_copy.wait()
        b2_copy.wait()

    def mlp_up(j, _):
        wait(w1_copies(j))

        @pl.when(j + 4 < nfc)
        def _():
            start(w1_copies(j + 4))

        @pl.when(j + 4 == nfc)
        def _():
            wm_copy(3).start()

        @pl.when(j + nsc >= nfc)
        def _():
            start(w2_copies(j + nsc - nfc))

        ht = fct // 2

        def rhs(p, q, i):
            base = j * fct + q * ht + zero_s[i]
            return jnp.concatenate(
                [jnp.concatenate([w1_v[base + t, pl.ds(256 * k + 128 * p, 128), :] for k in range(NT // 2)], axis=0)
                 for t in range(ht)], axis=1)

        g = {}
        for p, q, u in _strassen(lambda i: _unpack(a1_v[i]), rhs):
            bias = jnp.concatenate(
                [b1_v[pl.ds(j * fct + q * ht + t, 1), :] for t in range(ht)], axis=1)
            g[p, q] = _gelu(u + bias)
        cols = pl.ds(pl.multiple_of(j * (FC // 2), FC // 2), FC // 2)
        for n, op in enumerate(_strassen_lhs(g[0, 0], g[0, 1], g[1, 0], g[1, 1])):
            a2_v[n, :, cols] = _pack(op)
        return 0

    def mlp_down(j, _):
        wait(w2_copies(j))
        ht = sct // 2

        def rhs(p, q, i):
            base = j * sct + q * ht + zero_s[i]
            return jnp.concatenate(
                [jnp.concatenate([w2_v[base + t, pl.ds(FC * k + (FC // 2) * p, FC // 2), :] for k in range(nfc)],
                                 axis=0) for t in range(ht)], axis=1)

        for p, q, y in _strassen(lambda i: _unpack(a2_v[i]), rhs):
            gate = mod_col(5, p * H, H)
            for t in range(ht):
                tile = j * sct + q * ht + t
                cols = pl.ds(pl.multiple_of(tile * 128, 128), 128)
                yt = y[:, t * 128:(t + 1) * 128] + b2_v[pl.ds(tile, 1), :]
                out_v[j, p, q, :, t * 128:(t + 1) * 128] = (x1_v[pl.ds(p * H, H), cols] + gate * yt).astype(bf)
            out_copy(j, p, q).start()
        return 0

    def widen(ref_bf):
        def inner(ref_f):
            ref_f[...] = ref_bf[...].astype(f32)
            return ref_f
        return inner

    def mlp(b1f, b2f):
        nonlocal b1_v, b2_v
        b1f[...] = b1_v[...].astype(f32)
        b2f[...] = b2_v[...].astype(f32)
        b1_v, b2_v = b1f, b2f
        with _scope("mlp_up"):
            lax.fori_loop(0, nfc, mlp_up, 0)
        with _scope("mod3"):
            wm_copy(3).wait()
            modulation(3)
        with _scope("mlp_down"):
            lax.fori_loop(0, nsc, mlp_down, 0)

    pl.run_scoped(mlp, pltpu.VMEM((F // 128, 128), f32), pltpu.VMEM((NT, 128), f32))
    with _scope("outwait"):
        for j in range(nsc):
            for p in range(2):
                for q in range(2):
                    out_copy(j, p, q).wait()


@jax.jit
def pallas_adaLN_cond__spectral_gfnet__mixer_token_mlp__prompt_kernel(A_x, A_w_r, A_w_i, B_x, B_w1, B_b1, B_w2, B_b2, c, w_mod):
    del B_x
    bf, f32, i32 = jnp.bfloat16, jnp.float32, jnp.int32
    hbm = pl.BlockSpec(memory_space=pl.ANY)
    out_t = pl.pallas_call(
        _kernel,
        out_shape=jax.ShapeDtypeStruct((D, S), bf),
        in_specs=[hbm] * 11,
        out_specs=hbm,
        scratch_shapes=[
            pltpu.VMEM((D, S), bf),
            pltpu.VMEM((DF, S), bf),
            pltpu.VMEM((DF, S), bf),
            pltpu.VMEM((F // 128, S, 128), bf),
            pltpu.VMEM((NT, F, 128), bf),
            pltpu.VMEM((D, 6 * D), bf),
            pltpu.VMEM(_FMAT.shape, i32),
            pltpu.VMEM(_SEEDS.shape, f32),
            pltpu.VMEM((F // 128, 128), bf),
            pltpu.VMEM((NT, 128), bf),
            pltpu.VMEM((1, D), bf),
            pltpu.VMEM((NT, 3, 64, 128), i32),
            pltpu.VMEM((6 * D, 128), f32),
            pltpu.VMEM((NT, WROWS, 128), i32),
            pltpu.VMEM((H, S), i32),
            pltpu.VMEM((NT, NL, 128), f32),
            pltpu.VMEM((NT, NL, 128), f32),
            pltpu.VMEM((NT, NL, 128), f32),
            pltpu.VMEM((NT, NL, 128), f32),
            pltpu.VMEM((NT, NL, 128), f32),
            pltpu.VMEM((NT, NL, 128), f32),
            pltpu.VMEM((D, S), f32),
            pltpu.VMEM((H, 128), i32),
            pltpu.VMEM((D, S), f32),
            pltpu.VMEM((7, H // 2, S // 2), i32),
            pltpu.VMEM((7, H // 2, F // 2), i32),
            pltpu.VMEM((S // SC, 2, 2, H, SC // 2), bf),
            pltpu.SMEM((8,), i32),
            pltpu.SemaphoreType.DMA((11,)),
            pltpu.SemaphoreType.DMA((XCH,)),
            pltpu.SemaphoreType.DMA((F // FC,)),
            pltpu.SemaphoreType.DMA((S // SC,)),
            pltpu.SemaphoreType.DMA((S // SC * 4,)),
        ],
        compiler_params=pltpu.CompilerParams(vmem_limit_bytes=120 * 1024 * 1024),
    )(A_x[0].T, A_w_r.T, A_w_i.T, B_w1, B_w2, w_mod, _FMAT, _SEEDS,
      B_b1.reshape(F // 128, 128), B_b2.reshape(S // 128, 128), c)
    return out_t.T[None]
```

```python
import contextlib
import math

import jax
import jax.numpy as jnp
import numpy as np
from jax import lax
import jax.experimental.pallas as pl
import jax.experimental.pallas.tpu as pltpu

S, D, F = 2048, 576, 4608
DF = D // 2 + 1
EPS = 1e-5
NT = S // 128
G0 = 40
NL = 4 * 64 + G0
WROWS = 296
H = D // 2

XCH = 8
FC = 512
Q = D // 4
UU = 1
UD = 1
KSPLIT = 8
SC = 512
SCOPES = False

_C9 = [math.cos(2 * math.pi * j / 9) for j in range(9)]
_S9 = [math.sin(2 * math.pi * j / 9) for j in range(9)]


def _scope(name):
    return jax.named_scope(name) if SCOPES else contextlib.nullcontext()


def _sigmas(r):
    if r == 0:
        return [0, 9]
    return [r, r + 9, 9 - r, 18 - r]


def _pack_rows(m):
    u = m.astype(np.float32).astype(jnp.bfloat16).view(np.uint16).astype(np.uint32)
    return (u[..., 0::2, :] | (u[..., 1::2, :] << 16)).view(np.int32)


def _constants():
    dp = np.arange(64)
    ff = np.zeros((5, 128, 128))
    fi = np.zeros((5, 128, 128))
    scale = 1.0 / (D * S)

    def by8(re, im):
        return np.stack([re.reshape(-1, 8, re.shape[1]), im.reshape(-1, 8, im.shape[1])], 1).reshape(-1, re.shape[1])

    def by1(a, b):
        return np.stack([a, b], 2).reshape(a.shape[0], -1)

    for r in range(1, 5):
        l = np.array([18 * m + sg for sg in _sigmas(r) for m in range(16)])
        th = 2 * np.pi * np.outer(l, dp) / D
        sg = np.where(l % 9 == r, 1.0, -1.0)[:, None]
        co, si = np.cos(th), np.sin(th)
        ff[r - 1] = by8(by1(co, -_S9[3] * sg * si), by1(-si, -_S9[3] * sg * co))
        fi[r - 1] = 2 * scale * np.concatenate(
            [by1(co.T, -si.T), by1(_S9[3] * (sg * si).T, _S9[3] * (sg * co).T)], 0)
    l = np.array([18 * m + sg for sg in _sigmas(0) for m in range(16)] + [D // 2])
    th = 2 * np.pi * np.outer(l, dp) / D
    edge = (l == 0) | (l == D // 2)
    pad = ((0, G0 - len(l)), (0, 0))
    co, si = np.pad(np.cos(th), pad), np.pad(np.where(edge[:, None], 0.0, np.sin(th)), pad)
    order = np.array([16 * i + j + 8 * h for i in range(4) for j in range(8) for h in range(2)])
    ff[4, :2 * G0, :64] = by8(co[:, order], -si[:, order])
    cl = np.pad(np.where(edge, 1.0, 2.0), pad[0])[None, :]
    fi[4, :64, :2 * G0] = scale * by1(cl * co.T, -cl * si.T)
    b = 2 * np.arange(8)[:, None]
    p = np.arange(128)[None, :]
    k0 = 128 * (p // 8) + 16 * (p % 8)
    one = np.ones((8, 128))
    seeds = []
    for bb in (b, b + 1, 16):
        for z in (np.exp(-2j * np.pi * bb * k0 / S) * one, np.exp(2j * np.pi * 127 * bb / S) * one):
            seeds += [z.real, z.imag]
    return _pack_rows(np.concatenate([ff, fi], 0)), np.concatenate(seeds, 0).astype(np.float32)


_FMAT, _SEEDS = _constants()


def _radix9_even(h0, e1, e2, e3, e4):
    p = h0 + e3
    q = e1 + e2 + e4
    t0 = p + q
    t3 = p - 0.5 * q
    g = h0 - 0.5 * e3
    u = e1 - e4
    v = e2 - e4
    a = _C9[1] * u + _C9[2] * v
    b = _C9[2] * u + _C9[4] * v
    return t0, g + a, g + b, t3, g - a - b


def _radix9_odd(o1, o2, o3, o4):
    t3 = o1 - o2 + o4
    u = o1 + o2
    v = o2 + o4
    a = (_S9[1] / _S9[3]) * u + (_S9[4] / _S9[3]) * v
    b = (_S9[2] / _S9[3]) * u - (_S9[1] / _S9[3]) * v
    return a + o3, b - o3, t3, b - a + o3


def _radix4(z0, z1, z2, z3, sign):
    ar, ai = z0[0] + z2[0], z0[1] + z2[1]
    br, bi = z0[0] - z2[0], z0[1] - z2[1]
    cr, ci = z1[0] + z3[0], z1[1] + z3[1]
    dr, di = z1[0] - z3[0], z1[1] - z3[1]
    plus = (br - di, bi + dr)
    minus = (br + di, bi - dr)
    if sign > 0:
        return (ar + cr, ai + ci), plus, (ar - cr, ai - ci), minus
    return (ar + cr, ai + ci), minus, (ar - cr, ai - ci), plus


def _twiddle16(z, n, sign):
    zr, zi = z
    n %= 16
    if n == 0:
        return z
    if n == 4:
        return (-zi, zr) if sign > 0 else (zi, -zr)
    c = math.cos(2 * math.pi * n / 16)
    s = sign * math.sin(2 * math.pi * n / 16)
    if n % 4 == 2:
        if (c > 0) == (s > 0):
            return c * (zr - zi), c * (zr + zi)
        return c * (zr + zi), c * (zi - zr)
    return c * zr - s * zi, c * zi + s * zr


def _radix16(z, sign):
    u = [_radix4(z[a1], z[a1 + 4], z[a1 + 8], z[a1 + 12], sign) for a1 in range(4)]
    out = [None] * 16
    for q1 in range(4):
        t = [_twiddle16(u[a1][q1], a1 * q1, sign) for a1 in range(4)]
        y = _radix4(*t, sign)
        for q2 in range(4):
            out[q1 + 4 * q2] = y[q2]
    return out


def _cmul(a, b):
    return a[0] * b[0] - a[1] * b[1], a[0] * b[1] + a[1] * b[0]


def _gelu2(x):
    k = math.sqrt(2 / math.pi)
    return x + x * jnp.tanh(x * (k + (k * 0.044715) * (x * x)))


def _colmean(parts):
    acc = [parts[0], parts[1]]
    for i, p in enumerate(parts[2:]):
        acc[i % 2] = acc[i % 2] + p
    return jnp.sum(acc[0] + acc[1], axis=0, keepdims=True) * (1.0 / D)


def _pack(lo, hi):
    return pltpu.pack_elementwise([lo, hi], packed_dtype=jnp.bfloat16).astype(jnp.int32)


def _half(u, index):
    return pltpu.unpack_elementwise(u, index=index, packed_dtype=jnp.bfloat16, unpacked_dtype=jnp.float32)


def _unpack(x):
    return pltpu.bitcast(x, jnp.bfloat16)


def _dot(a, b):
    return jnp.dot(a, b, preferred_element_type=jnp.float32)


def _dot_nt(a, b):
    return lax.dot_general(a, b, (((1,), (1,)), ((), ())), preferred_element_type=jnp.float32)


def _strassen_lhs(a11, a12, a21, a22):
    return (a11 + a22, a21 + a22, a11, a22, a11 + a12, a21 - a11, a12 - a22)


_QUADS = ((0, 0), (0, 1), (1, 0), (1, 1))
_STRASSEN_RHS = (
    (((0, 0), 1), ((1, 1), 1)), (((0, 0), 1),), (((0, 1), 1), ((1, 1), -1)), (((1, 0), 1), ((0, 0), -1)),
    (((1, 1), 1),), (((0, 0), 1), ((0, 1), 1)), (((1, 0), 1), ((1, 1), 1)))


def _signed_sum(terms, get):
    total = get(terms[0][0])
    for block, sign in terms[1:]:
        total = total + get(block) if sign > 0 else total - get(block)
    return total


def _strassen_out(product):
    m3, m5 = product(2), product(4)
    yield 0, 1, lambda f: f(m3) + f(m5)
    m2, m4 = product(1), product(3)
    yield 1, 0, lambda f: f(m2) + f(m4)
    m1, m7 = product(0), product(6)
    yield 0, 0, lambda f: f(m1) + f(m4) - f(m5) + f(m7)
    m6 = product(5)
    yield 1, 1, lambda f: f(m1) - f(m2) + f(m3) + f(m6)


def _strassen2(lhs, words):
    def outer(p):
        def inner(q):
            def block(b, c):
                return words(2 * b[0] + c[0], 2 * b[1] + c[1], p, q)

            rp, rq = _STRASSEN_RHS[p], _STRASSEN_RHS[q]
            if len(rp) == 1 and len(rq) == 1:
                rhs = block(rp[0][0], rq[0][0])
            else:
                rhs = _pack(*[_signed_sum(rq, lambda c: _signed_sum(rp, lambda b: _half(block(b, c), h)))
                              for h in range(2)])
            return _dot(lhs(7 * p + q), _unpack(rhs))

        return {(r, c): f(lambda m: m) for r, c, f in _strassen_out(inner)}

    for r, c, f in _strassen_out(outer):
        yield r, c, {rc: f(lambda m: m[rc]) for rc in _QUADS}


def _kernel(x_hbm, wr_hbm, wi_hbm, w1_hbm, w2_hbm, wm_hbm, f_hbm, seed_hbm, b1_hbm, b2_hbm, c_hbm,
            out_hbm,
            w1_v, w2_v, wm_v, b1_v, b2_v, mod_v, x1_v, a1_v, zero_s, sem_in, sem_x, sem_w1, sem_w2, sem_out):
    f32, bf = jnp.float32, jnp.bfloat16
    xw = S // XCH
    nfc, nsc = F // FC, S // SC
    fct, sct = FC // 128, SC // 128

    wm_parts = ((512, 1152), (0, 512), (1152, 2944), (2944, 6 * D))

    def wm_copy(i):
        lo, hi = wm_parts[i]
        return pltpu.make_async_copy(wm_hbm.at[:, lo:hi], wm_v.at[:, lo:hi], sem_in.at[i])

    b1_copy = pltpu.make_async_copy(b1_hbm, b1_v, sem_in.at[4])
    b2_copy = pltpu.make_async_copy(b2_hbm, b2_v, sem_in.at[5])

    def w1_copies(j):
        return [pltpu.make_async_copy(w1_hbm.at[:, pl.ds(pl.multiple_of((j * fct + t) * 128, 128), 128)],
                                      w1_v.at[j * fct + t], sem_w1.at[j]) for t in range(fct)]

    def w2_copies(j):
        return [pltpu.make_async_copy(w2_hbm.at[:, pl.ds(pl.multiple_of((j * sct + t) * 128, 128), 128)],
                                      w2_v.at[j * sct + t], sem_w2.at[j]) for t in range(sct)]

    def out_copy(out_v, j, p, q):
        col = pl.multiple_of(j * SC + q * (SC // 2), SC // 2)
        return pltpu.make_async_copy(out_v.at[j, p, q], out_hbm.at[pl.ds(p * H, H), pl.ds(col, SC // 2)],
                                     sem_out.at[j * 4 + p * 2 + q])

    def start(copies):
        for cp in copies:
            cp.start()

    def wait(copies):
        for cp in copies:
            cp.wait()

    def modulation(act, i):
        lo, hi = wm_parts[i]
        row = _dot(act, wm_v[:, lo:hi])
        for t in range((hi - lo) // 128):
            tile = jnp.broadcast_to(row[0:1, t * 128:(t + 1) * 128], (128, 128))
            mod_v[lo + t * 128:lo + (t + 1) * 128, :] = tile.T

    def mod_col(which, r0, n):
        return mod_v[pl.ds(which * D + r0, n), :]

    def front(act_v, x_v, wr_v, wi_v, f_v, seed_v, c_v, g_v, wp_v, t_v, yr_v, yi_v, xr_v, xi_v, qr_v, qi_v,
              p_v, zs_v, h_v, *u_v):
        def x_copy(i):
            return pltpu.make_async_copy(x_hbm.at[:, pl.ds(i * xw, xw)], x_v.at[:, pl.ds(i * xw, xw)], sem_x.at[i])

        seed_copy, c_copy, f_copy, wr_copy, wi_copy = [
            pltpu.make_async_copy(src, dst, sem_in.at[6 + i]) for i, (src, dst) in enumerate(
                ((seed_hbm, seed_v), (c_hbm, c_v), (f_hbm, f_v), (wr_hbm, wr_v), (wi_hbm, wi_v)))]

        start([seed_copy, c_copy, wm_copy(0), x_copy(0)])
        for i in range(49):
            zero_s[i] = 0

        with _scope("twiddle"):
            seed_copy.wait()
            start([x_copy(1)])
            sd = [(seed_v[16 * i:16 * i + 8, :], seed_v[16 * i + 8:16 * i + 16, :]) for i in range(6)]
            g0, tau = [sd[0], sd[2]], [sd[1], sd[3]]
            for i in range(8):
                g = g0
                for k1 in range(NT):
                    g_v[k1, 0, 8 * i:8 * i + 8, :] = _pack(g[0][0], g[1][0])
                    g_v[k1, 1, 8 * i:8 * i + 8, :] = _pack(g[0][1] - g[0][0], g[1][1] - g[1][0])
                    g_v[k1, 2, 8 * i:8 * i + 8, :] = _pack(g[0][1] + g[0][0], g[1][1] + g[1][0])
                    if k1 + 1 < NT:
                        g = [_cmul(g[0], tau[0]), _cmul(g[1], tau[1])]
                if i < 7:
                    g0 = [_cmul(z, sd[4]) for z in g0]
                    tau = [_cmul(z, sd[5]) for z in tau]

        with _scope("mod0"):
            c_copy.wait()
            start([x_copy(2)])
            cc = c_v[...].astype(f32)
            act_v[...] = jnp.broadcast_to(cc * jax.nn.sigmoid(cc), (8, D))
            wm_copy(0).wait()
            start([x_copy(3)])
            modulation(act_v[...], 0)
            mod_v[D:2 * D, :] = 1.0 + mod_v[D:2 * D, :]

        def radix9_fwd(rows):
            for i in range(4):
                h = [rows(64 * a + 16 * i) for a in range(9)]
                e = [h[a] + h[9 - a] for a in range(1, 5)]
                o = [h[a] - h[9 - a] for a in range(1, 5)]
                te = _radix9_even(h[0], *e)
                to = _radix9_odd(*o)
                yield 256 + 8 * i, _pack(te[0][0:8], te[0][8:16])
                for r in range(4):
                    yield 64 * r + 16 * i, _pack(te[r + 1], to[r])

        def stage1(t):
            cols = pl.ds(t * 128, 128)
            xs = [x_v[pl.ds(16 * i, 16), cols].astype(f32) for i in range(D // 16)]
            m = _colmean(xs)
            ds = [v - m for v in xs]
            rs = lax.rsqrt(_colmean([d * d for d in ds]) + EPS)
            for r0, piece in radix9_fwd(lambda r0: ds[r0 // 16] * rs * mod_col(1, r0, 16)):
                t_v[pl.ds(r0, piece.shape[0]), cols] = piece

        later = {4: [f_copy], 5: [wr_copy], 6: [wi_copy], 7: [wm_copy(1)]}
        for i in range(XCH):
            with _scope("xwait%d" % i):
                x_copy(i).wait()
                start([x_copy(i + 4)] if i + 4 < XCH else later[i])
            with _scope("stage1_%d" % i):
                for t in range(NT // XCH):
                    stage1(i * (NT // XCH) + t)

        def d_forward(r, tmat):
            if r < 4:
                return _dot(_unpack(f_v[r]), _unpack(tmat(64 * r, 64)))
            return _dot(_unpack(f_v[4, 0:G0, 0:64]), _unpack(tmat(256, 32)))

        def group_rows(r):
            return range(0, 64 if r < 4 else G0, 8)

        with _scope("fwait"):
            f_copy.wait()
            start([wm_copy(2), b1_copy, b2_copy])
        with _scope("dfwd"):
            for r in range(5):
                for a1 in range(4):
                    z = d_forward(r, lambda r0, k: jnp.concatenate(
                        [t_v[r0:r0 + k, (a1 + 4 * a2) * 128:(a1 + 4 * a2 + 1) * 128] for a2 in range(4)], axis=1))
                    for i in group_rows(r):
                        u = _radix4(*[(z[2 * i:2 * i + 8, a2 * 128:(a2 + 1) * 128],
                                       z[2 * i + 8:2 * i + 16, a2 * 128:(a2 + 1) * 128]) for a2 in range(4)], -1)
                        for q1 in range(4):
                            u_v[r][a1, q1, 0, i:i + 8, :], u_v[r][a1, q1, 1, i:i + 8, :] = _twiddle16(
                                u[q1], a1 * q1, -1)
                for i in group_rows(r):
                    rows = slice(64 * r + i, 64 * r + i + 8)
                    for q1 in range(4):
                        y = _radix4(*[(u_v[r][a1, q1, 0, i:i + 8, :], u_v[r][a1, q1, 1, i:i + 8, :])
                                      for a1 in range(4)], -1)
                        for q2 in range(4):
                            yr_v[q1 + 4 * q2, rows, :], yi_v[q1 + 4 * q2, rows, :] = y[q2]

        def s_forward(k1):
            yr, yi = yr_v[k1], yi_v[k1]
            k = _dot(yr + yi, _unpack(g_v[k1, 0]))
            xr_v[k1] = k - _dot(yi, _unpack(g_v[k1, 2]))
            xi_v[k1] = k + _dot(yr, _unpack(g_v[k1, 1]))

        with _scope("sfwd_a"):
            for k1 in range(KSPLIT):
                s_forward(k1)

        with _scope("wwait"):
            wr_copy.wait()
            wi_copy.wait()
            wm_copy(1).wait()
            start(w1_copies(0))
        lane = lax.broadcasted_iota(jnp.int32, (8, 128), 1)
        grp = lane >> 3

        def permute(src, row0):
            a = [None] * NT
            for ct in range(NT):
                idx = ((lane & 7) << 4) + ((grp - ct) & 15)
                a[(-ct) % NT] = jnp.take_along_axis(src[ct], idx, axis=1)
            for bit in range(4):
                mask = ((grp >> bit) & 1) == 1
                a = [jnp.where(mask, a[(m - (1 << bit)) % NT], a[m]) for m in range(NT)]
            for k1 in range(NT):
                wp_v[k1, pl.ds(row0, 8), :] = a[k1]

        with _scope("sfwd_b_wperm"):
            for k1 in range(KSPLIT, NT):
                s_forward(k1)
            for i in range(18):
                for src, base in ((wr_v, 0), (wi_v, 144)):
                    permute([pltpu.bitcast(src[16 * i:16 * i + 16, ct * 128:(ct + 1) * 128], jnp.int32)
                             for ct in range(NT)], base + 8 * i)
            permute([_pack(*[jnp.broadcast_to(w[288:289, ct * 128:(ct + 1) * 128].astype(f32), (8, 128))
                             for w in (wr_v, wi_v)]) for ct in range(NT)], 288)

            modulation(act_v[...], 1)
            for r0, piece in radix9_fwd(lambda r0: mod_col(0, r0, 16)):
                zs_v[pl.ds(r0, piece.shape[0]), :] = piece
            first = lane == 0
            for r in range(5):
                z = d_forward(r, lambda r0, k: zs_v[r0:r0 + k, :])
                for i in group_rows(r):
                    rows = slice(64 * r + i, 64 * r + i + 8)
                    for dst, r0 in ((xr_v, 2 * i), (xi_v, 2 * i + 8)):
                        dst[0, rows, :] = dst[0, rows, :] + jnp.where(first, z[r0:r0 + 8] * float(S), 0.0)

        def s_inverse(k1):
            wr, wi = [], []
            for r in (1, 2, 3, 4, 0):
                for sg in _sigmas(r):
                    wr.append(_half(wp_v[k1, pl.ds(sg // 2, 16, stride=9), :], sg % 2))
                    wi.append(_half(wp_v[k1, pl.ds(144 + sg // 2, 16, stride=9), :], sg % 2))
            u = wp_v[k1, 288:296, :]
            wr = jnp.concatenate(wr + [_half(u, 0)], axis=0)
            wi = jnp.concatenate(wi + [_half(u, 1)], axis=0)
            xr, xi = xr_v[k1], xi_v[k1]
            fr = xr * wr - xi * wi
            fi = xr * wi + xi * wr
            k = _dot_nt(fr + fi, _unpack(g_v[k1, 0]))
            qr_v[k1] = k + _dot_nt(fi, _unpack(g_v[k1, 1]))
            qi_v[k1] = k - _dot_nt(fr, _unpack(g_v[k1, 2]))

        with _scope("sinv"):
            start(w1_copies(1))
            for k1 in range(NT):
                s_inverse(k1)

        with _scope("dinv"):
            wm_copy(2).wait()
            start(w1_copies(2))
            for r in range(5):
                for i in group_rows(r):
                    rows = slice(64 * r + i, 64 * r + i + 8)
                    for q1 in range(4):
                        u = _radix4(*[(qr_v[q1 + 4 * q2, rows, :], qi_v[q1 + 4 * q2, rows, :])
                                      for q2 in range(4)], +1)
                        for a1 in range(4):
                            u_v[r][a1, q1, 0, i:i + 8, :], u_v[r][a1, q1, 1, i:i + 8, :] = _twiddle16(
                                u[a1], a1 * q1, +1)
                for a1 in range(4):
                    v = _radix4(*[(u_v[r][a1, q1, 0], u_v[r][a1, q1, 1]) for q1 in range(4)], +1)
                    vmat = _unpack(jnp.concatenate([_pack(*e) for e in v], axis=1))
                    if r < 4:
                        pr, r0 = _dot(_unpack(f_v[5 + r]), vmat), 128 * r
                    else:
                        pr, r0 = _dot(_unpack(f_v[9, 0:32, 0:2 * G0]), vmat), 512
                    for a2 in range(4):
                        p_v[a1 + 4 * a2, r0:r0 + pr.shape[0], :] = pr[:, a2 * 128:(a2 + 1) * 128]
            modulation(act_v[...], 2)
            mod_v[4 * D:5 * D, :] = 1.0 + mod_v[4 * D:5 * D, :]

        def stage5(t, slot):
            cols = pl.ds(pl.multiple_of(t * 128, 128), 128)
            parts = []
            for i in range(4):
                pe = [p_v[t, pl.ds(512 + 16 * i, 16), :]] + [p_v[t, pl.ds(128 * r + 16 * i, 16), :] for r in range(4)]
                po = [p_v[t, pl.ds(128 * r + 64 + 16 * i, 16), :] for r in range(4)]
                ee = _radix9_even(*pe)
                oo = _radix9_odd(*po)
                ya = [ee[0]] + [ee[a] - oo[a - 1] for a in range(1, 5)] + [ee[a] + oo[a - 1] for a in (4, 3, 2, 1)]
                for a in range(9):
                    r0 = 64 * a + 16 * i
                    v = x_v[pl.ds(r0, 16), cols].astype(f32) + mod_col(2, r0, 16) * ya[a]
                    x1_v[t, pl.ds(r0, 16), :] = v
                    parts.append(v)
            pieces = [pl.ds(16 * i, 16) for i in range(D // 16)]
            m = _colmean(parts)
            ds = [x1_v[t, rows, :] - m for rows in pieces]
            rs = lax.rsqrt(_colmean([d * d for d in ds]) + EPS)
            parts = []
            for i, rows in enumerate(pieces):
                v = (x1_v[t + zero_s[0], rows, :] - m) * rs * mod_col(4, 16 * i, 16) + mod_col(3, 16 * i, 16)
                h_v[slot, rows, :] = v
                parts.append(v)
            m = _colmean(parts)
            ds = [h_v[slot, rows, :] - m for rows in pieces]
            return m, lax.rsqrt(_colmean([d * d for d in ds]) + EPS)

        def stage5_quad(t, _):
            stats = [stage5(4 * t + k, k) for k in range(4)]
            cols = pl.ds(pl.multiple_of(t * 128, 128), 128)
            for i in range(0, Q, 8):
                def block(mq, kq):
                    return (h_v[kq + zero_s[0], pl.ds(mq * Q + i, 8), :] - stats[kq][0]) * stats[kq][1]

                inner = [_strassen_lhs(*[block(2 * r + r2, 2 * c + c2) for r2, c2 in _QUADS]) for r, c in _QUADS]
                for q in range(7):
                    for p, op in enumerate(_strassen_lhs(*[ops[q] for ops in inner])):
                        a1_v[7 * p + q, pl.ds(i, 8), cols] = op
            return 0

        with _scope("stage5"):
            start(w1_copies(3))
            lax.fori_loop(0, NT // 4, stage5_quad, 0)

    def mlp(act_v, a2_v, out_v, b1_f, b2_f):
        def up(j):
            def words(kq, nq, p, q):
                tile = 4 * j + nq + zero_s[7 * p + q]
                return jnp.concatenate([w1_i[tile, pl.ds(64 * (4 * k + kq), 64), :] for k in range(NT // 4)], axis=0)

            inner = {}
            for r, c, u in _strassen2(lambda n: a1_v[n], words):
                inner[r, c] = _strassen_lhs(*[
                    _gelu2(u[r2, c2] + b1_f[pl.ds(4 * j + 2 * c + c2, 1), :]) for r2, c2 in _QUADS])
            cols = pl.ds(pl.multiple_of(j * 128, 128), 128)
            for q in range(7):
                for p, op in enumerate(_strassen_lhs(*[inner[rc][q] for rc in _QUADS])):
                    a2_v[7 * p + q, :, cols] = op

        def up_block(jb, _):
            for u in range(UU):
                wait(w1_copies(jb * UU + u))
            for u in range(UU):
                up(jb * UU + u)
            return 0

        def down(j):
            def words(kq, nq, p, q):
                tile = 4 * j + nq + zero_s[7 * p]
                return jnp.concatenate([w2_i[tile, pl.ds(64 * (4 * k + kq), 64), :] for k in range(nfc)], axis=0)

            for r, c, y in _strassen2(lambda n: a2_v[n], words):
                for r2 in range(2):
                    r0 = (2 * r + r2) * Q
                    gate = mod_col(5, r0, Q)
                    halves = []
                    for c2 in range(2):
                        tile = 4 * j + 2 * c + c2
                        yt = 0.5 * y[r2, c2] + b2_f[pl.ds(tile, 1), :]
                        halves.append(x1_v[tile, pl.ds(r0, Q), :] + gate * yt)
                    out_v[j, r, c, pl.ds(r2 * Q, Q), :] = jnp.concatenate(halves, axis=1).astype(bf)
                out_copy(out_v, j, r, c).start()

        def down_block(jb, _):
            for u in range(UD):
                wait(w2_copies(jb * UD + u))
            for u in range(UD):
                down(jb * UD + u)
            return 0

        w1_i, w2_i = w1_v.bitcast(jnp.int32), w2_v.bitcast(jnp.int32)
        for j in range(4, nfc):
            start(w1_copies(j))
        wm_copy(3).start()
        b1_copy.wait()
        b2_copy.wait()
        b1_f[...] = b1_v[...].astype(f32)
        b2_f[...] = b2_v[...].astype(f32)
        with _scope("mlp_up"):
            def up_loop(jb, _):
                @pl.when(jb == 1)
                def _():
                    for j in range(nsc):
                        start(w2_copies(j))
                return up_block(jb, 0)

            lax.fori_loop(0, nfc // UU, up_loop, 0)
        with _scope("mod3"):
            wm_copy(3).wait()
            modulation(act_v[...], 3)
        with _scope("mlp_down"):
            lax.fori_loop(0, nsc // UD, down_block, 0)
        with _scope("outwait"):
            for j in range(nsc):
                for r, c in _QUADS:
                    out_copy(out_v, j, r, c).wait()

    def body(act_v):
        vmem = pltpu.VMEM
        i32 = jnp.int32
        pl.run_scoped(
            lambda *refs: front(act_v, *refs),
            vmem((D, S), bf), vmem((DF, S), bf), vmem((DF, S), bf), vmem(_FMAT.shape, i32),
            vmem(_SEEDS.shape, f32), vmem((1, D), bf), vmem((NT, 3, 64, 128), i32), vmem((NT, WROWS, 128), i32),
            vmem((H, S), i32), *[vmem((NT, NL, 128), f32)] * 6, vmem((NT, D, 128), f32), vmem((H, 128), i32),
            vmem((4, D, 128), f32), *[vmem((4, 4, 2, n, 128), f32) for n in (64, 64, 64, 64, G0)])
        pl.run_scoped(
            lambda *refs: mlp(act_v, *refs),
            vmem((49, Q, F // 4), f32), vmem((nsc, 2, 2, H, SC // 2), bf), vmem((F // 128, 128), f32),
            vmem((NT, 128), f32))

    pl.run_scoped(body, pltpu.VMEM((8, D), f32))


@jax.jit
def pallas_adaLN_cond__spectral_gfnet__mixer_token_mlp__prompt_kernel(A_x, A_w_r, A_w_i, B_x, B_w1, B_b1, B_w2, B_b2, c, w_mod):
    del B_x
    bf, f32, i32 = jnp.bfloat16, jnp.float32, jnp.int32
    hbm = pl.BlockSpec(memory_space=pl.ANY)
    out_t = pl.pallas_call(
        _kernel,
        out_shape=jax.ShapeDtypeStruct((D, S), bf),
        in_specs=[hbm] * 11,
        out_specs=hbm,
        scratch_shapes=[
            pltpu.VMEM((F // 128, S, 128), bf),
            pltpu.VMEM((NT, F, 128), bf),
            pltpu.VMEM((D, 6 * D), bf),
            pltpu.VMEM((F // 128, 128), bf),
            pltpu.VMEM((NT, 128), bf),
            pltpu.VMEM((6 * D, 128), f32),
            pltpu.VMEM((NT, D, 128), f32),
            pltpu.VMEM((49, Q, S // 4), f32),
            pltpu.SMEM((49,), i32),
            pltpu.SemaphoreType.DMA((11,)),
            pltpu.SemaphoreType.DMA((XCH,)),
            pltpu.SemaphoreType.DMA((F // FC,)),
            pltpu.SemaphoreType.DMA((S // SC,)),
            pltpu.SemaphoreType.DMA((S // SC * 4,)),
        ],
        compiler_params=pltpu.CompilerParams(vmem_limit_bytes=120 * 1024 * 1024),
    )(A_x[0].T, A_w_r.T, A_w_i.T, B_w1, B_w2, w_mod, _FMAT, _SEEDS,
      B_b1.reshape(F // 128, 128), B_b2.reshape(S // 128, 128), c)
    return out_t.T[None]
```

```python
import contextlib
import math

import jax
import jax.numpy as jnp
import numpy as np
from jax import lax
import jax.experimental.pallas as pl
import jax.experimental.pallas.tpu as pltpu

S, D, F = 2048, 576, 4608
DF = D // 2 + 1
EPS = 1e-5
NT = S // 128
G0 = 40
NL = 4 * 64 + G0
WROWS = 296
H = D // 2

XCH = 8
FC = 512
Q = D // 4
UU = 1
UD = 1
KSPLIT = 8
A2_F32 = False
ORDER_UP = (2, 4, 1, 3, 0, 6, 5)
ORDER_DOWN = (2, 4, 1, 3, 0, 6, 5)
ORDER_IN = (2, 4, 1, 3, 0, 6, 5)
SHARE_UP = ()
SHARE_DOWN = (0, 1, 2, 3, 4, 5, 6)
SC = 512
SCOPES = False

_C9 = [math.cos(2 * math.pi * j / 9) for j in range(9)]
_S9 = [math.sin(2 * math.pi * j / 9) for j in range(9)]


def _scope(name):
    return jax.named_scope(name) if SCOPES else contextlib.nullcontext()


def _sigmas(r):
    if r == 0:
        return [0, 9]
    return [r, r + 9, 9 - r, 18 - r]


def _pack_rows(m):
    u = m.astype(np.float32).astype(jnp.bfloat16).view(np.uint16).astype(np.uint32)
    return (u[..., 0::2, :] | (u[..., 1::2, :] << 16)).view(np.int32)


def _constants():
    dp = np.arange(64)
    ff = np.zeros((5, 128, 128))
    fi = np.zeros((5, 128, 128))
    scale = 1.0 / (D * S)

    def by8(re, im):
        return np.stack([re.reshape(-1, 8, re.shape[1]), im.reshape(-1, 8, im.shape[1])], 1).reshape(-1, re.shape[1])

    def even_odd(m):
        n = m.shape[0] // 16 * 16
        head = m[:n].reshape(-1, 8, 2, m.shape[1]).transpose(0, 2, 1, 3).reshape(n, m.shape[1])
        return np.concatenate([head, m[n:]], 0)

    def by1(a, b):
        return np.stack([a, b], 2).reshape(a.shape[0], -1)

    for r in range(1, 5):
        l = np.array([18 * m + sg for sg in _sigmas(r) for m in range(16)])
        th = 2 * np.pi * np.outer(l, dp) / D
        sg = np.where(l % 9 == r, 1.0, -1.0)[:, None]
        co, si = np.cos(th), np.sin(th)
        ff[r - 1] = by8(even_odd(by1(co, -_S9[3] * sg * si)), even_odd(by1(-si, -_S9[3] * sg * co)))
        fi[r - 1] = 2 * scale * even_odd(np.concatenate(
            [by1(co.T, -si.T), by1(_S9[3] * (sg * si).T, _S9[3] * (sg * co).T)], 0))
    l = np.array([18 * m + sg for sg in _sigmas(0) for m in range(16)] + [D // 2])
    th = 2 * np.pi * np.outer(l, dp) / D
    edge = (l == 0) | (l == D // 2)
    pad = ((0, G0 - len(l)), (0, 0))
    co, si = np.pad(np.cos(th), pad), np.pad(np.where(edge[:, None], 0.0, np.sin(th)), pad)
    order = np.array([16 * i + j + 8 * h for i in range(4) for j in range(8) for h in range(2)])
    ff[4, :2 * G0, :64] = by8(even_odd(co[:, order]), even_odd(-si[:, order]))
    cl = np.pad(np.where(edge, 1.0, 2.0), pad[0])[None, :]
    fi[4, :64, :2 * G0] = scale * even_odd(by1(cl * co.T, -cl * si.T))
    b = 2 * np.arange(8)[:, None]
    p = np.arange(128)[None, :]
    k0 = 128 * (p % 16) + 16 * (p // 16)
    step = -127 + 0 * p
    wrap = step + np.where(p < 16, 112, -16)
    seeds = []
    for bb in (b, b + 1, 16 + 0 * b):
        for k in (k0, step, wrap):
            z = np.exp(-2j * np.pi * bb * k / S)
            seeds += [z.real, z.imag]
    return _pack_rows(np.concatenate([ff, fi], 0)), np.concatenate(seeds, 0).astype(np.float32)


_FMAT, _SEEDS = _constants()


def _radix9_even(h0, e1, e2, e3, e4):
    p = h0 + e3
    q = e1 + e2 + e4
    t0 = p + q
    t3 = p - 0.5 * q
    g = h0 - 0.5 * e3
    u = e1 - e4
    v = e2 - e4
    a = _C9[1] * u + _C9[2] * v
    b = _C9[2] * u + _C9[4] * v
    return t0, g + a, g + b, t3, g - a - b


def _radix9_odd(o1, o2, o3, o4):
    t3 = o1 - o2 + o4
    u = o1 + o2
    v = o2 + o4
    a = (_S9[1] / _S9[3]) * u + (_S9[4] / _S9[3]) * v
    b = (_S9[2] / _S9[3]) * u - (_S9[1] / _S9[3]) * v
    return a + o3, b - o3, t3, b - a + o3


def _radix4(z0, z1, z2, z3, sign):
    ar, ai = z0[0] + z2[0], z0[1] + z2[1]
    br, bi = z0[0] - z2[0], z0[1] - z2[1]
    cr, ci = z1[0] + z3[0], z1[1] + z3[1]
    dr, di = z1[0] - z3[0], z1[1] - z3[1]
    plus = (br - di, bi + dr)
    minus = (br + di, bi - dr)
    if sign > 0:
        return (ar + cr, ai + ci), plus, (ar - cr, ai - ci), minus
    return (ar + cr, ai + ci), minus, (ar - cr, ai - ci), plus


def _twiddle16(z, n, sign):
    zr, zi = z
    n %= 16
    if n == 0:
        return z
    if n == 4:
        return (-zi, zr) if sign > 0 else (zi, -zr)
    c = math.cos(2 * math.pi * n / 16)
    s = sign * math.sin(2 * math.pi * n / 16)
    if n % 4 == 2:
        if (c > 0) == (s > 0):
            return c * (zr - zi), c * (zr + zi)
        return c * (zr + zi), c * (zi - zr)
    return c * zr - s * zi, c * zi + s * zr


def _radix16(z, sign):
    u = [_radix4(z[a1], z[a1 + 4], z[a1 + 8], z[a1 + 12], sign) for a1 in range(4)]
    out = [None] * 16
    for q1 in range(4):
        t = [_twiddle16(u[a1][q1], a1 * q1, sign) for a1 in range(4)]
        y = _radix4(*t, sign)
        for q2 in range(4):
            out[q1 + 4 * q2] = y[q2]
    return out


def _cmul(a, b):
    return a[0] * b[0] - a[1] * b[1], a[0] * b[1] + a[1] * b[0]


def _gelu2(x):
    k = math.sqrt(2 / math.pi)
    return x + x * jnp.tanh(x * (k + (k * 0.044715) * (x * x)))


def _colmean(parts):
    acc = [parts[0], parts[1]]
    for i, p in enumerate(parts[2:]):
        acc[i % 2] = acc[i % 2] + p
    return jnp.sum(acc[0] + acc[1], axis=0, keepdims=True) * (1.0 / D)


def _pack(lo, hi):
    return pltpu.pack_elementwise([lo, hi], packed_dtype=jnp.bfloat16).astype(jnp.int32)


def _half(u, index):
    return pltpu.unpack_elementwise(u, index=index, packed_dtype=jnp.bfloat16, unpacked_dtype=jnp.float32)


def _unpack(x):
    return pltpu.bitcast(x, jnp.bfloat16)


def _dot(a, b):
    return jnp.dot(a, b, preferred_element_type=jnp.float32)


def _dot_nt(a, b):
    return lax.dot_general(a, b, (((1,), (1,)), ((), ())), preferred_element_type=jnp.float32)


def _strassen_lhs(a11, a12, a21, a22):
    return (a11 + a22, a21 + a22, a11, a22, a11 + a12, a21 - a11, a12 - a22)


_QUADS = ((0, 0), (0, 1), (1, 0), (1, 1))
_STRASSEN_RHS = (
    (((0, 0), 1), ((1, 1), 1)), (((0, 0), 1),), (((0, 1), 1), ((1, 1), -1)), (((1, 0), 1), ((0, 0), -1)),
    (((1, 1), 1),), (((0, 0), 1), ((0, 1), 1)), (((1, 0), 1), ((1, 1), 1)))


def _signed_sum(terms, get):
    total = get(terms[0][0])
    for block, sign in terms[1:]:
        total = total + get(block) if sign > 0 else total - get(block)
    return total


_STRASSEN_OUT = {
    (0, 0): ((0, 1), (3, 1), (4, -1), (6, 1)), (0, 1): ((2, 1), (4, 1)),
    (1, 0): ((1, 1), (3, 1)), (1, 1): ((0, 1), (1, -1), (2, 1), (5, 1))}


def _strassen_out(product, order):
    done = {}
    for n in order:
        done[n] = product(n)
        for (r, c), terms in _STRASSEN_OUT.items():
            if n in dict(terms) and all(k in done for k, _ in terms):
                yield r, c, lambda f, terms=terms: _signed_sum(terms, lambda k: f(done[k]))


def _strassen2(lhs, words, order):
    def outer(p):
        def inner(q):
            def block(b, c):
                return words(2 * b[0] + c[0], 2 * b[1] + c[1], p, q)

            rp, rq = _STRASSEN_RHS[p], _STRASSEN_RHS[q]
            if len(rp) == 1 and len(rq) == 1:
                rhs = block(rp[0][0], rq[0][0])
            else:
                rhs = _pack(*[_signed_sum(rq, lambda c: _signed_sum(rp, lambda b: _half(block(b, c), h)))
                              for h in range(2)])
            return _dot(lhs(7 * p + q), _unpack(rhs))

        return {(r, c): f(lambda m: m) for r, c, f in _strassen_out(inner, ORDER_IN)}

    for r, c, f in _strassen_out(outer, order):
        yield r, c, {rc: f(lambda m: m[rc]) for rc in _QUADS}


def _kernel(x_hbm, wr_hbm, wi_hbm, w1_hbm, w2_hbm, wm_hbm, f_hbm, seed_hbm, b1_hbm, b2_hbm, c_hbm,
            out_hbm,
            w1_v, w2_v, wm_v, b1_v, b2_v, mod_v, x1_v, a1_v, zero_s, sem_in, sem_x, sem_w1, sem_w2, sem_out):
    f32, bf = jnp.float32, jnp.bfloat16
    xw = S // XCH
    nfc, nsc = F // FC, S // SC
    fct, sct = FC // 128, SC // 128

    wm_parts = ((512, 1152), (0, 512), (1152, 6 * D))

    def wm_copy(i):
        lo, hi = wm_parts[i]
        return pltpu.make_async_copy(wm_hbm.at[:, lo:hi], wm_v.at[:, lo:hi], sem_in.at[i])

    b1_copy = pltpu.make_async_copy(b1_hbm, b1_v, sem_in.at[4])
    b2_copy = pltpu.make_async_copy(b2_hbm, b2_v, sem_in.at[5])

    def w1_copies(j):
        return [pltpu.make_async_copy(w1_hbm.at[:, pl.ds(pl.multiple_of((j * fct + t) * 128, 128), 128)],
                                      w1_v.at[j * fct + t], sem_w1.at[j]) for t in range(fct)]

    def w2_copies(j):
        return [pltpu.make_async_copy(w2_hbm.at[:, pl.ds(pl.multiple_of((j * sct + t) * 128, 128), 128)],
                                      w2_v.at[j * sct + t], sem_w2.at[j]) for t in range(sct)]

    def out_copy(out_v, j, p, q):
        col = pl.multiple_of(j * SC + q * (SC // 2), SC // 2)
        return pltpu.make_async_copy(out_v.at[j, p, q], out_hbm.at[pl.ds(p * H, H), pl.ds(col, SC // 2)],
                                     sem_out.at[j * 4 + p * 2 + q])

    def start(copies):
        for cp in copies:
            cp.start()

    def wait(copies):
        for cp in copies:
            cp.wait()

    def modulation(act, i):
        lo, hi = wm_parts[i]
        row = _dot(act, wm_v[:, lo:hi])
        for t in range((hi - lo) // 128):
            tile = jnp.broadcast_to(row[0:1, t * 128:(t + 1) * 128], (128, 128))
            mod_v[lo + t * 128:lo + (t + 1) * 128, :] = tile.T

    def mod_col(which, r0, n):
        return mod_v[pl.ds(which * D + r0, n), :]

    def front(act_v, x_v, wr_v, wi_v, f_v, seed_v, c_v, g_v, wp_v, t_v, y_v, xr_v, xi_v, qr_v, qi_v,
              p_v, zs_v, sh_v, e_v, h_v, *u_v):
        def x_copy(i):
            cols = pl.ds(pl.multiple_of(i * xw, xw), xw)
            return pltpu.make_async_copy(x_hbm.at[:, cols], x_v.at[:, cols], sem_x.at[i])

        seed_copy, c_copy, f_copy, wr_copy, wi_copy = [
            pltpu.make_async_copy(src, dst, sem_in.at[6 + i]) for i, (src, dst) in enumerate(
                ((seed_hbm, seed_v), (c_hbm, c_v), (f_hbm, f_v), (wr_hbm, wr_v), (wi_hbm, wi_v)))]

        start([seed_copy, c_copy, wm_copy(0), x_copy(0)])
        for i in range(49):
            zero_s[i] = 0

        lane = lax.broadcasted_iota(jnp.int32, (8, 128), 1)
        with _scope("twiddle"):
            seed_copy.wait()
            start([x_copy(1)])
            sd = [(seed_v[16 * i:16 * i + 8, :], seed_v[16 * i + 8:16 * i + 16, :]) for i in range(9)]
            rows = [sd[0:3], sd[3:6]]
            for i in range(8):
                g = [row[0] for row in rows]
                for k1 in range(NT):
                    g_v[k1, 0, 8 * i:8 * i + 8, :] = _pack(g[0][0], g[1][0])
                    g_v[k1, 1, 8 * i:8 * i + 8, :] = _pack(g[0][1] - g[0][0], g[1][1] - g[1][0])
                    g_v[k1, 2, 8 * i:8 * i + 8, :] = _pack(g[0][1] + g[0][0], g[1][1] + g[1][0])
                    if k1 + 1 < NT:
                        at = (lane & 15) == k1
                        g = [_cmul(z, (jnp.where(at, row[2][0], row[1][0]), jnp.where(at, row[2][1], row[1][1])))
                             for z, row in zip(g, rows)]
                if i < 7:
                    rows = [[_cmul(z, w) for z, w in zip(row, sd[6:9])] for row in rows]

        with _scope("mod0"):
            c_copy.wait()
            start([x_copy(2)])
            cc = c_v[...].astype(f32)
            act_v[...] = jnp.broadcast_to(cc * jax.nn.sigmoid(cc), (8, D))
            wm_copy(0).wait()
            start([x_copy(3)])
            modulation(act_v[...], 0)
            mod_v[D:2 * D, :] = 1.0 + mod_v[D:2 * D, :]

        def radix9_fwd(rows):
            for i in range(4):
                h = [rows(64 * a + 16 * i) for a in range(9)]
                e = [h[a] + h[9 - a] for a in range(1, 5)]
                o = [h[a] - h[9 - a] for a in range(1, 5)]
                te = _radix9_even(h[0], *e)
                to = _radix9_odd(*o)
                yield 256 + 8 * i, _pack(te[0][0:8], te[0][8:16])
                for r in range(4):
                    yield 64 * r + 16 * i, _pack(te[r + 1], to[r])

        def stage1(t):
            cols = pl.ds(pl.multiple_of(t * 128, 128), 128)
            xs = [x_v[pl.ds(16 * i, 16), cols].astype(f32) for i in range(D // 16)]
            m = _colmean(xs)
            ds = [v - m for v in xs]
            rs = lax.rsqrt(_colmean([d * d for d in ds]) + EPS)
            for r0, piece in radix9_fwd(lambda r0: ds[r0 // 16] * rs * mod_col(1, r0, 16)):
                t_v[pl.ds(r0, piece.shape[0]), cols] = piece

        def stage1_chunk(i, _):
            x_copy(i).wait()
            pl.when(i + 4 < XCH)(lambda: x_copy(i + 4).start())
            for n, cp in enumerate((f_copy, wr_copy, wi_copy, wm_copy(1))):
                pl.when(i == XCH - 4 + n)(cp.start)
            for t in range(NT // XCH):
                stage1(i * (NT // XCH) + t)
            return 0

        with _scope("stage1"):
            lax.fori_loop(0, XCH, stage1_chunk, 0)

        def d_forward(r, tmat):
            if r < 4:
                return _dot(_unpack(f_v[r]), _unpack(tmat(64 * r, 64)))
            return _dot(_unpack(f_v[4, 0:G0, 0:64]), _unpack(tmat(256, 32)))

        def group_rows(r):
            return range(0, 64 if r < 4 else G0, 8)

        with _scope("fwait"):
            f_copy.wait()
            start([wm_copy(2), b1_copy, b2_copy])
        with _scope("dfwd"):
            for r in range(5):
                for a1 in range(4):
                    z = d_forward(r, lambda r0, k: jnp.concatenate(
                        [t_v[r0:r0 + k, (a1 + 4 * a2) * 128:(a1 + 4 * a2 + 1) * 128] for a2 in range(4)], axis=1))
                    for i in group_rows(r):
                        u = _radix4(*[(z[2 * i:2 * i + 8, a2 * 128:(a2 + 1) * 128],
                                       z[2 * i + 8:2 * i + 16, a2 * 128:(a2 + 1) * 128]) for a2 in range(4)], -1)
                        for q1 in range(4):
                            u_v[r][a1, q1, 0, i:i + 8, :], u_v[r][a1, q1, 1, i:i + 8, :] = _twiddle16(
                                u[q1], a1 * q1, -1)
                for i in group_rows(r)[::2]:
                    rows = slice(32 * r + i // 2, 32 * r + i // 2 + 8)
                    for q1 in range(4):
                        y = [_radix4(*[(u_v[r][a1, q1, 0, j:j + 8, :], u_v[r][a1, q1, 1, j:j + 8, :])
                                       for a1 in range(4)], -1) for j in (i, i + 8) if j in group_rows(r)]
                        for q2 in range(4):
                            lo = y[0][q2]
                            hi = y[1][q2] if len(y) == 2 else (jnp.zeros_like(lo[0]),) * 2
                            y_v[q1 + 4 * q2, 0, rows, :] = _pack(lo[0] + lo[1], hi[0] + hi[1])
                            y_v[q1 + 4 * q2, 1, rows, :] = _pack(lo[0], hi[0])
                            y_v[q1 + 4 * q2, 2, rows, :] = _pack(lo[1], hi[1])

        def s_forward(k1, shift=None):
            k, kr, ki = [_dot(_unpack(y_v[k1, n]), _unpack(g_v[k1, n]))[0:NL] for n in range(3)]
            xr, xi = k - ki, k + kr
            xr_v[k1], xi_v[k1] = (xr, xi) if shift is None else (xr + shift[0], xi + shift[1])

        with _scope("sfwd_a"):
            for k1 in range(NT - 1, NT - 1 - KSPLIT, -1):
                s_forward(k1)

        with _scope("wwait"):
            wr_copy.wait()
            wi_copy.wait()
            wm_copy(1).wait()
            start(w1_copies(0))

        def permute(src, row0):
            a = [None] * NT
            for ct in range(NT):
                a[(-ct) % NT] = pltpu.roll(src[ct], ct, 1) if ct else src[ct]
            for bit in range(4):
                mask = ((lane >> bit) & 1) == 1
                a = [jnp.where(mask, a[(m - (1 << bit)) % NT], a[m]) for m in range(NT)]
            for k1 in range(NT):
                wp_v[k1, pl.ds(row0, 8), :] = a[k1]

        with _scope("sfwd_b_wperm"):
            modulation(act_v[...], 1)
            for i in range(18):
                for src, base in ((wr_v, 0), (wi_v, 144)):
                    permute([pltpu.bitcast(src[16 * i:16 * i + 16, ct * 128:(ct + 1) * 128], jnp.int32)
                             for ct in range(NT)], base + 8 * i)
            permute([_pack(*[jnp.broadcast_to(w[288:289, ct * 128:(ct + 1) * 128].astype(f32), (8, 128))
                             for w in (wr_v, wi_v)]) for ct in range(NT)], 288)
            for k1 in range(NT - 1 - KSPLIT, 2, -1):
                s_forward(k1)
            for r0, piece in radix9_fwd(lambda r0: mod_col(0, r0, 16)):
                zs_v[pl.ds(r0, piece.shape[0]), :] = piece
            for r in range(5):
                z = d_forward(r, lambda r0, k: zs_v[r0:r0 + k, :])
                for i in group_rows(r):
                    rows = pl.ds(64 * r + i // 16 * 16 + i // 8 % 2, 8, stride=2)
                    for n in range(2):
                        sh_v[n, rows, :] = jnp.where(lane == 0, z[2 * i + 8 * n:2 * i + 8 * n + 8] * float(S), 0.0)
            s_forward(2)
            s_forward(1)
            sh_v[:, pl.ds(4 * 64 + 33, 8, stride=2), :] = jnp.zeros((2, 8, 128), f32)
            s_forward(0, (sh_v[0, 0:NL, :], sh_v[1, 0:NL, :]))

        def s_inverse(k1):
            wr, wi = [], []
            for r in (1, 2, 3, 4, 0):
                for sg in _sigmas(r):
                    wr.append(_half(wp_v[k1, pl.ds(sg // 2, 16, stride=9), :], sg % 2))
                    wi.append(_half(wp_v[k1, pl.ds(144 + sg // 2, 16, stride=9), :], sg % 2))
            u = wp_v[k1, 288:296, :]
            wr = jnp.concatenate(wr + [_half(u, 0)], axis=0)
            wi = jnp.concatenate(wi + [_half(u, 1)], axis=0)
            xr, xi = xr_v[k1], xi_v[k1]
            fr = xr * wr - xi * wi
            fi = xr * wi + xi * wr
            k = _dot_nt(fr + fi, _unpack(g_v[k1, 0]))
            qr_v[k1] = k + _dot_nt(fi, _unpack(g_v[k1, 1]))
            qi_v[k1] = k - _dot_nt(fr, _unpack(g_v[k1, 2]))

        with _scope("sinv"):
            start(w1_copies(1))
            for k1 in range(NT):
                s_inverse(k1)

        with _scope("dinv"):
            wm_copy(2).wait()
            start(w1_copies(2))
            modulation(act_v[...], 2)
            for r in range(5):
                for i in group_rows(r):
                    rows = slice(64 * r + i, 64 * r + i + 8)
                    for q1 in range(4):
                        u = _radix4(*[(qr_v[q1 + 4 * q2, rows, :], qi_v[q1 + 4 * q2, rows, :])
                                      for q2 in range(4)], +1)
                        for a1 in range(4):
                            u_v[r][a1, q1, 0, i:i + 8, :], u_v[r][a1, q1, 1, i:i + 8, :] = _twiddle16(
                                u[a1], a1 * q1, +1)
                for a1 in range(4):
                    v = _radix4(*[(u_v[r][a1, q1, 0], u_v[r][a1, q1, 1]) for q1 in range(4)], +1)
                    vmat = _unpack(jnp.concatenate([_pack(*e) for e in v], axis=1))
                    if r < 4:
                        pr, r0 = _dot(_unpack(f_v[5 + r]), vmat), 128 * r
                    else:
                        pr, r0 = _dot(_unpack(f_v[9, 0:32, 0:2 * G0]), vmat), 512
                    for a2 in range(4):
                        p_v[a1 + 4 * a2, r0:r0 + pr.shape[0], :] = pr[:, a2 * 128:(a2 + 1) * 128]
            mod_v[4 * D:5 * D, :] = 1.0 + mod_v[4 * D:5 * D, :]
            sb = [mod_col(3, 16 * i, 16) for i in range(D // 16)]
            mean_sb = _colmean(sb)
            for i, v in enumerate(sb):
                mod_v[pl.ds(3 * D + 16 * i, 16), :] = v - mean_sb

        def split(ref, lead, r0):
            return jnp.concatenate([ref[(*lead, pl.ds(r0 + h, 8, stride=2), slice(None))] for h in range(2)], axis=0)

        def stage5(t, slot):
            cols = pl.ds(pl.multiple_of(t * 128, 128), 128)
            parts = []
            for i in range(4):
                pe = [p_v[t, pl.ds(512 + 16 * i, 16), :]] + [p_v[t, pl.ds(128 * r + 16 * i, 16), :] for r in range(4)]
                po = [p_v[t, pl.ds(128 * r + 64 + 16 * i, 16), :] for r in range(4)]
                ee = _radix9_even(*pe)
                oo = _radix9_odd(*po)
                ya = [ee[0]] + [ee[a] - oo[a - 1] for a in range(1, 5)] + [ee[a] + oo[a - 1] for a in (4, 3, 2, 1)]
                for a in range(9):
                    r0 = 64 * a + 16 * i
                    u = pltpu.bitcast(x_v[pl.ds(r0, 16), cols], jnp.int32)
                    v = jnp.concatenate([_half(u, 0), _half(u, 1)], axis=0) + split(mod_v, (), 2 * D + r0) * ya[a]
                    for h in range(2):
                        x1_v[t, pl.ds(r0 + h, 8, stride=2), :] = v[8 * h:8 * h + 8]
                    parts.append(v)
            m = _colmean(parts)
            squares, parts = [], []
            for i in range(D // 16):
                d = split(x1_v, (t,), 16 * i) - m
                e = d * split(mod_v, (), 4 * D + 16 * i)
                e_v[slot, pl.ds(16 * i, 16), :] = e
                squares.append(d * d)
                parts.append(e)
            rs = lax.rsqrt(_colmean(squares) + EPS)
            m = _colmean(parts)
            squares = []
            for i in range(D // 16):
                d = (e_v[slot, pl.ds(16 * i, 16), :] - m) * rs + split(mod_v, (), 3 * D + 16 * i)
                h_v[slot, pl.ds(16 * i, 16), :] = d
                squares.append(d * d)
            return lax.rsqrt(_colmean(squares) + EPS)

        def stage5_quad(t, _):
            scale = [stage5(4 * t + k, k) for k in range(4)]
            cols = pl.ds(pl.multiple_of(t * 128, 128), 128)
            for i in range(0, Q, 16):
                def block(mq, kq):
                    return h_v[kq, pl.ds(mq * Q + i, 16), :] * scale[kq]

                inner = [_strassen_lhs(*[block(2 * r + r2, 2 * c + c2) for r2, c2 in _QUADS]) for r, c in _QUADS]
                for q in range(7):
                    for p, op in enumerate(_strassen_lhs(*[ops[q] for ops in inner])):
                        a1_v[7 * p + q, pl.ds(i // 2, 8), cols] = _pack(op[0:8], op[8:16])
            return 0

        with _scope("stage5"):
            start(w1_copies(3))
            lax.fori_loop(0, NT // 4, stage5_quad, 0)

    def mlp(act_v, a2_v, out_v, b1_f, b2_f):
        def up(j):
            def words(kq, nq, p, q):
                tile = 4 * j + nq + zero_s[7 * p + (0 if p in SHARE_UP else q)]
                return jnp.concatenate([w1_i[tile, pl.ds(64 * (4 * k + kq), 64), :] for k in range(NT // 4)], axis=0)

            inner = {}
            for r, c, u in _strassen2(lambda n: _unpack(a1_v[n]), words, ORDER_UP):
                inner[r, c] = _strassen_lhs(*[
                    _gelu2(u[r2, c2] + b1_f[pl.ds(4 * j + 2 * c + c2, 1), :]) for r2, c2 in _QUADS])
            ops = [op for q in range(7) for op in _strassen_lhs(*[inner[rc][q] for rc in _QUADS])]
            if A2_F32:
                cols = pl.ds(pl.multiple_of(j * 128, 128), 128)
                for n in range(49):
                    a2_v[n, :, cols] = ops[n]
            else:
                cols = pl.ds(pl.multiple_of(j * 256, 256), 256)
                for n in range(25):
                    a2_v[n, :, cols] = jnp.concatenate([ops[2 * n], ops[min(2 * n + 1, 48)]], axis=1).astype(bf)

        def hidden(n):
            n = n % 7 * 7 + n // 7
            if A2_F32:
                return a2_v[n]
            return jnp.concatenate(
                [a2_v[n // 2, :, pl.ds(256 * k + 128 * (n % 2), 128)] for k in range(nfc)], axis=1)

        def up_block(jb, _):
            for u in range(UU):
                wait(w1_copies(jb * UU + u))
            for u in range(UU):
                up(jb * UU + u)
            return 0

        def down(j):
            def words(kq, nq, p, q):
                tile = 4 * j + nq + zero_s[7 * p + (0 if p in SHARE_DOWN else q)]
                return jnp.concatenate([w2_i[tile, pl.ds(64 * (4 * k + kq), 64), :] for k in range(nfc)], axis=0)

            for r, c, y in _strassen2(hidden, words, ORDER_DOWN):
                for r2 in range(2):
                    r0 = (2 * r + r2) * Q
                    gate = mod_col(5, r0, Q)
                    halves = []
                    for c2 in range(2):
                        tile = 4 * j + 2 * c + c2
                        yt = 0.5 * y[r2, c2] + b2_f[pl.ds(tile, 1), :]
                        halves.append(x1_v[tile, pl.ds(r0, Q), :] + gate * yt)
                    out_v[j, r, c, pl.ds(r2 * Q, Q), :] = jnp.concatenate(halves, axis=1).astype(bf)
                out_copy(out_v, j, r, c).start()

        def down_block(jb, _):
            for u in range(UD):
                wait(w2_copies(jb * UD + u))
            for u in range(UD):
                down(jb * UD + u)
            return 0

        w1_i, w2_i = w1_v.bitcast(jnp.int32), w2_v.bitcast(jnp.int32)
        for j in range(4, nfc):
            start(w1_copies(j))
        b1_copy.wait()
        b2_copy.wait()
        b1_f[...] = b1_v[...].astype(f32)
        b2_f[...] = b2_v[...].astype(f32)
        with _scope("mlp_up"):
            def up_loop(jb, _):
                @pl.when(jb == 1)
                def _():
                    for j in range(nsc):
                        start(w2_copies(j))
                return up_block(jb, 0)

            lax.fori_loop(0, nfc // UU, up_loop, 0)
        with _scope("mlp_down"):
            lax.fori_loop(0, nsc // UD, down_block, 0)
        with _scope("outwait"):
            for j in range(nsc):
                for r, c in _QUADS:
                    out_copy(out_v, j, r, c).wait()

    def body(act_v):
        vmem = pltpu.VMEM
        i32 = jnp.int32
        pl.run_scoped(
            lambda *refs: front(act_v, *refs),
            vmem((D, S), bf), vmem((DF, S), bf), vmem((DF, S), bf), vmem(_FMAT.shape, i32),
            vmem(_SEEDS.shape, f32), vmem((1, D), bf), vmem((NT, 3, 64, 128), i32), vmem((NT, WROWS, 128), i32),
            vmem((H, S), i32), vmem((NT, 3, NL // 2 + 4, 128), i32), *[vmem((NT, NL, 128), f32)] * 4,
            vmem((NT, D, 128), f32), vmem((H, 128), i32), vmem((2, NL + 8, 128), f32),
            vmem((4, D, 128), f32), vmem((4, D, 128), f32), *[vmem((4, 4, 2, n, 128), f32) for n in (64, 64, 64, 64, G0)])
        pl.run_scoped(
            lambda *refs: mlp(act_v, *refs),
            vmem((49, Q, F // 4), f32) if A2_F32 else vmem((25, Q, F // 2), bf), vmem((nsc, 2, 2, H, SC // 2), bf), vmem((F // 128, 128), f32),
            vmem((NT, 128), f32))

    pl.run_scoped(body, pltpu.VMEM((8, D), f32))


@jax.jit
def pallas_adaLN_cond__spectral_gfnet__mixer_token_mlp__prompt_kernel(A_x, A_w_r, A_w_i, B_x, B_w1, B_b1, B_w2, B_b2, c, w_mod):
    del B_x
    bf, f32, i32 = jnp.bfloat16, jnp.float32, jnp.int32
    hbm = pl.BlockSpec(memory_space=pl.ANY)
    out_t = pl.pallas_call(
        _kernel,
        out_shape=jax.ShapeDtypeStruct((D, S), bf),
        in_specs=[hbm] * 11,
        out_specs=hbm,
        scratch_shapes=[
            pltpu.VMEM((F // 128, S, 128), bf),
            pltpu.VMEM((NT, F, 128), bf),
            pltpu.VMEM((D, 6 * D), bf),
            pltpu.VMEM((F // 128, 128), bf),
            pltpu.VMEM((NT, 128), bf),
            pltpu.VMEM((6 * D, 128), f32),
            pltpu.VMEM((NT, D, 128), f32),
            pltpu.VMEM((49, Q // 2, S // 4), i32),
            pltpu.SMEM((49,), i32),
            pltpu.SemaphoreType.DMA((11,)),
            pltpu.SemaphoreType.DMA((XCH,)),
            pltpu.SemaphoreType.DMA((F // FC,)),
            pltpu.SemaphoreType.DMA((S // SC,)),
            pltpu.SemaphoreType.DMA((S // SC * 4,)),
        ],
        compiler_params=pltpu.CompilerParams(vmem_limit_bytes=120 * 1024 * 1024),
    )(A_x[0].T, A_w_r.T, A_w_i.T, B_w1, B_w2, w_mod, _FMAT, _SEEDS,
      B_b1.reshape(F // 128, 128), B_b2.reshape(S // 128, 128), c)
    return out_t.T[None]
```

```python
import contextlib
import math

import jax
import jax.numpy as jnp
import numpy as np
from jax import lax
import jax.experimental.pallas as pl
import jax.experimental.pallas.tpu as pltpu

S, D, F = 2048, 576, 4608
DF = D // 2 + 1
EPS = 1e-5
NT = S // 128
G0 = 40
NL = 4 * 64 + G0
WROWS = 296
H = D // 2

XCH = 8
FC = 512
Q = D // 4
UU = 1
UD = 1
KSPLIT = 8
SA_AT = 6
ORDER_UP = (2, 4, 1, 3, 0, 6, 5)
ORDER_DOWN = (2, 4, 1, 3, 0, 6, 5)
ORDER_IN = (4, 2, 1, 3, 0, 6, 5)
SHARE_UP = (0, 6, 5)
SHARE_DOWN = (0, 1, 2, 3, 4, 5, 6)
SC = 512
SCOPES = False

_C9 = [math.cos(2 * math.pi * j / 9) for j in range(9)]
_S9 = [math.sin(2 * math.pi * j / 9) for j in range(9)]


def _scope(name):
    return jax.named_scope(name) if SCOPES else contextlib.nullcontext()


def _sigmas(r):
    if r == 0:
        return [0, 9]
    return [r, r + 9, 9 - r, 18 - r]


def _pack_rows(m):
    u = m.astype(np.float32).astype(jnp.bfloat16).view(np.uint16).astype(np.uint32)
    return (u[..., 0::2, :] | (u[..., 1::2, :] << 16)).view(np.int32)


def _constants():
    dp = np.arange(64)
    ff = np.zeros((5, 128, 128))
    fi = np.zeros((5, 128, 128))
    scale = 1.0 / (D * S)

    def by8(re, im):
        return np.stack([re.reshape(-1, 8, re.shape[1]), im.reshape(-1, 8, im.shape[1])], 1).reshape(-1, re.shape[1])

    def even_odd(m):
        n = m.shape[0] // 16 * 16
        head = m[:n].reshape(-1, 8, 2, m.shape[1]).transpose(0, 2, 1, 3).reshape(n, m.shape[1])
        return np.concatenate([head, m[n:]], 0)

    def by1(a, b):
        return np.stack([a, b], 2).reshape(a.shape[0], -1)

    for r in range(1, 5):
        l = np.array([18 * m + sg for sg in _sigmas(r) for m in range(16)])
        th = 2 * np.pi * np.outer(l, dp) / D
        sg = np.where(l % 9 == r, 1.0, -1.0)[:, None]
        co, si = np.cos(th), np.sin(th)
        ff[r - 1] = by8(by1(co, -_S9[3] * sg * si), by1(-si, -_S9[3] * sg * co))
        fi[r - 1] = 2 * scale * even_odd(np.concatenate(
            [by1(co.T, -si.T), by1(_S9[3] * (sg * si).T, _S9[3] * (sg * co).T)], 0))
    l = np.array([18 * m + sg for sg in _sigmas(0) for m in range(16)] + [D // 2])
    th = 2 * np.pi * np.outer(l, dp) / D
    edge = (l == 0) | (l == D // 2)
    pad = ((0, G0 - len(l)), (0, 0))
    co, si = np.pad(np.cos(th), pad), np.pad(np.where(edge[:, None], 0.0, np.sin(th)), pad)
    order = np.array([16 * i + j + 8 * h for i in range(4) for j in range(8) for h in range(2)])
    ff[4, :2 * G0, :64] = by8(co[:, order], -si[:, order])
    cl = np.pad(np.where(edge, 1.0, 2.0), pad[0])[None, :]
    fi[4, :64, :2 * G0] = scale * even_odd(by1(cl * co.T, -cl * si.T))
    b = 2 * np.arange(8)[:, None]
    p = np.arange(128)[None, :]
    k0 = 128 * (p % 16) + 16 * (p // 16)
    step = -127 + 0 * p
    wrap = step + np.where(p < 16, 112, -16)
    seeds = []
    for bb in (b, b + 1, 16 + 0 * b):
        for k in (k0, step, wrap):
            z = np.exp(-2j * np.pi * bb * k / S)
            seeds += [z.real, z.imag]
    return _pack_rows(np.concatenate([ff, fi], 0)), np.concatenate(seeds, 0).astype(np.float32)


_FMAT, _SEEDS = _constants()


def _radix9_even(h0, e1, e2, e3, e4):
    p = h0 + e3
    q = e1 + e2 + e4
    t0 = p + q
    t3 = p - 0.5 * q
    g = h0 - 0.5 * e3
    u = e1 - e4
    v = e2 - e4
    a = _C9[1] * u + _C9[2] * v
    b = _C9[2] * u + _C9[4] * v
    return t0, g + a, g + b, t3, g - a - b


def _radix9_odd(o1, o2, o3, o4):
    t3 = o1 - o2 + o4
    u = o1 + o2
    v = o2 + o4
    a = (_S9[1] / _S9[3]) * u + (_S9[4] / _S9[3]) * v
    b = (_S9[2] / _S9[3]) * u - (_S9[1] / _S9[3]) * v
    return a + o3, b - o3, t3, b - a + o3


def _radix4(z0, z1, z2, z3, sign):
    ar, ai = z0[0] + z2[0], z0[1] + z2[1]
    br, bi = z0[0] - z2[0], z0[1] - z2[1]
    cr, ci = z1[0] + z3[0], z1[1] + z3[1]
    dr, di = z1[0] - z3[0], z1[1] - z3[1]
    plus = (br - di, bi + dr)
    minus = (br + di, bi - dr)
    if sign > 0:
        return (ar + cr, ai + ci), plus, (ar - cr, ai - ci), minus
    return (ar + cr, ai + ci), minus, (ar - cr, ai - ci), plus


def _twiddle16(z, n, sign):
    zr, zi = z
    n %= 16
    if n == 0:
        return z
    if n == 4:
        return (-zi, zr) if sign > 0 else (zi, -zr)
    c = math.cos(2 * math.pi * n / 16)
    s = sign * math.sin(2 * math.pi * n / 16)
    if n % 4 == 2:
        if (c > 0) == (s > 0):
            return c * (zr - zi), c * (zr + zi)
        return c * (zr + zi), c * (zi - zr)
    return c * zr - s * zi, c * zi + s * zr


def _radix16(z, sign):
    u = [_radix4(z[a1], z[a1 + 4], z[a1 + 8], z[a1 + 12], sign) for a1 in range(4)]
    out = [None] * 16
    for q1 in range(4):
        t = [_twiddle16(u[a1][q1], a1 * q1, sign) for a1 in range(4)]
        y = _radix4(*t, sign)
        for q2 in range(4):
            out[q1 + 4 * q2] = y[q2]
    return out


def _cmul(a, b):
    return a[0] * b[0] - a[1] * b[1], a[0] * b[1] + a[1] * b[0]


def _gelu2(x):
    k = math.sqrt(2 / math.pi)
    return x + x * jnp.tanh(x * (k + (k * 0.044715) * (x * x)))


def _colmean(parts):
    acc = [parts[0], parts[1]]
    for i, p in enumerate(parts[2:]):
        acc[i % 2] = acc[i % 2] + p
    return jnp.sum(acc[0] + acc[1], axis=0, keepdims=True) * (1.0 / D)


def _pack(lo, hi):
    return pltpu.pack_elementwise([lo, hi], packed_dtype=jnp.bfloat16).astype(jnp.int32)


def _half(u, index):
    return pltpu.unpack_elementwise(u, index=index, packed_dtype=jnp.bfloat16, unpacked_dtype=jnp.float32)


def _unpack(x):
    return pltpu.bitcast(x, jnp.bfloat16)


def _dot(a, b):
    return jnp.dot(a, b, preferred_element_type=jnp.float32)


def _dot_nt(a, b):
    return lax.dot_general(a, b, (((1,), (1,)), ((), ())), preferred_element_type=jnp.float32)


def _strassen_lhs(a11, a12, a21, a22):
    return (a11 + a22, a21 + a22, a11, a22, a11 + a12, a21 - a11, a12 - a22)


_QUADS = ((0, 0), (0, 1), (1, 0), (1, 1))
_STRASSEN_RHS = (
    (((0, 0), 1), ((1, 1), 1)), (((0, 0), 1),), (((0, 1), 1), ((1, 1), -1)), (((1, 0), 1), ((0, 0), -1)),
    (((1, 1), 1),), (((0, 0), 1), ((0, 1), 1)), (((1, 0), 1), ((1, 1), 1)))


def _signed_sum(terms, get):
    total = get(terms[0][0])
    for block, sign in terms[1:]:
        total = total + get(block) if sign > 0 else total - get(block)
    return total


_STRASSEN_OUT = {
    (0, 0): ((0, 1), (3, 1), (4, -1), (6, 1)), (0, 1): ((2, 1), (4, 1)),
    (1, 0): ((1, 1), (3, 1)), (1, 1): ((0, 1), (1, -1), (2, 1), (5, 1))}


def _strassen_out(product, order):
    done = {}
    for n in order:
        done[n] = product(n)
        for (r, c), terms in _STRASSEN_OUT.items():
            if n in dict(terms) and all(k in done for k, _ in terms):
                yield r, c, lambda f, terms=terms: _signed_sum(terms, lambda k: f(done[k]))


def _strassen2(lhs, words, order):
    def outer(p):
        def inner(q):
            def block(b, c):
                return words(2 * b[0] + c[0], 2 * b[1] + c[1], p, q)

            rp, rq = _STRASSEN_RHS[p], _STRASSEN_RHS[q]
            if len(rp) == 1 and len(rq) == 1:
                rhs = block(rp[0][0], rq[0][0])
            else:
                rhs = _pack(*[_signed_sum(rq, lambda c: _signed_sum(rp, lambda b: _half(block(b, c), h)))
                              for h in range(2)])
            return _dot(lhs(7 * p + q), _unpack(rhs))

        return {(r, c): f(lambda m: m) for r, c, f in _strassen_out(inner, ORDER_IN)}

    for r, c, f in _strassen_out(outer, order):
        yield r, c, {rc: f(lambda m: m[rc]) for rc in _QUADS}


def _kernel(x_hbm, wr_hbm, wi_hbm, w1_hbm, w2_hbm, wm_hbm, f_hbm, seed_hbm, b1_hbm, b2_hbm, c_hbm,
            out_hbm,
            w1_v, w2_v, wm_v, b1_v, b2_v, mod_v, x1_v, a1_v, zero_s, sem_in, sem_x, sem_w1, sem_w2, sem_out):
    f32, bf = jnp.float32, jnp.bfloat16
    xw = S // XCH
    nfc, nsc = F // FC, S // SC
    fct, sct = FC // 128, SC // 128

    wm_parts = ((512, 1152), (0, 512), (1152, 6 * D))

    def wm_copy(i):
        lo, hi = wm_parts[i]
        return pltpu.make_async_copy(wm_hbm.at[:, lo:hi], wm_v.at[:, lo:hi], sem_in.at[i])

    b1_copy = pltpu.make_async_copy(b1_hbm, b1_v, sem_in.at[4])
    b2_copy = pltpu.make_async_copy(b2_hbm, b2_v, sem_in.at[5])

    def w1_copies(j):
        return [pltpu.make_async_copy(w1_hbm.at[:, pl.ds(pl.multiple_of((j * fct + t) * 128, 128), 128)],
                                      w1_v.at[j * fct + t], sem_w1.at[j]) for t in range(fct)]

    def w2_copies(j):
        return [pltpu.make_async_copy(w2_hbm.at[:, pl.ds(pl.multiple_of((j * sct + t) * 128, 128), 128)],
                                      w2_v.at[j * sct + t], sem_w2.at[j]) for t in range(sct)]

    def out_copy(out_v, j, p, q):
        col = pl.multiple_of(j * SC + q * (SC // 2), SC // 2)
        return pltpu.make_async_copy(out_v.at[j, p, q], out_hbm.at[pl.ds(p * H, H), pl.ds(col, SC // 2)],
                                     sem_out.at[j * 4 + p * 2 + q])

    w1_i, w2_i = w1_v.bitcast(jnp.int32), w2_v.bitcast(jnp.int32)

    def start(copies):
        for cp in copies:
            cp.start()

    def wait(copies):
        for cp in copies:
            cp.wait()

    def modulation(act, lo, tiles):
        row = _dot(act, wm_v[:, pl.ds(lo, tiles * 128)])
        for t in range(tiles):
            tile = jnp.broadcast_to(row[0:1, t * 128:(t + 1) * 128], (128, 128))
            mod_v[pl.ds(lo + t * 128, 128), :] = tile.T

    def mod_col(which, r0, n):
        return mod_v[pl.ds(which * D + r0, n), :]

    def front(act_v, x_v, wr_v, wi_v, f_v, seed_v, c_v, g_v, wp_v, t_v, yr_v, yi_v, xr_v, xi_v, qr_v, qi_v,
              p_v, zs_v, e_v, h_v, *u_v):
        def x_copy(i):
            cols = pl.ds(pl.multiple_of(i * xw, xw), xw)
            return pltpu.make_async_copy(x_hbm.at[:, cols], x_v.at[:, cols], sem_x.at[i])

        seed_copy, c_copy, f_copy, wr_copy, wi_copy = [
            pltpu.make_async_copy(src, dst, sem_in.at[6 + i]) for i, (src, dst) in enumerate(
                ((seed_hbm, seed_v), (c_hbm, c_v), (f_hbm, f_v), (wr_hbm, wr_v), (wi_hbm, wi_v)))]

        start([seed_copy, c_copy, wm_copy(0), x_copy(0)])
        for i in range(49):
            zero_s[i] = 0

        lane = lax.broadcasted_iota(jnp.int32, (8, 128), 1)
        with _scope("twiddle"):
            seed_copy.wait()
            start([x_copy(1)])
            sd = [(seed_v[16 * i:16 * i + 8, :], seed_v[16 * i + 8:16 * i + 16, :]) for i in range(9)]
            rows = [sd[0:3], sd[3:6]]
            for i in range(8):
                g = [row[0] for row in rows]
                for k1 in range(NT):
                    g_v[k1, 0, 8 * i:8 * i + 8, :] = _pack(g[0][0], g[1][0])
                    g_v[k1, 1, 8 * i:8 * i + 8, :] = _pack(g[0][1] - g[0][0], g[1][1] - g[1][0])
                    g_v[k1, 2, 8 * i:8 * i + 8, :] = _pack(g[0][1] + g[0][0], g[1][1] + g[1][0])
                    if k1 + 1 < NT:
                        at = (lane & 15) == k1
                        g = [_cmul(z, (jnp.where(at, row[2][0], row[1][0]), jnp.where(at, row[2][1], row[1][1])))
                             for z, row in zip(g, rows)]
                if i < 7:
                    rows = [[_cmul(z, w) for z, w in zip(row, sd[6:9])] for row in rows]

        with _scope("mod0"):
            c_copy.wait()
            start([x_copy(2)])
            cc = c_v[...].astype(f32)
            act_v[...] = jnp.broadcast_to(cc * jax.nn.sigmoid(cc), (8, D))
            wm_copy(0).wait()
            start([x_copy(3)])
            modulation(act_v[...], 512, 5)
            mod_v[D:2 * D, :] = 1.0 + mod_v[D:2 * D, :]

        def radix9_fwd(rows):
            for i in range(4):
                h = [rows(64 * a + 16 * i) for a in range(9)]
                e = [h[a] + h[9 - a] for a in range(1, 5)]
                o = [h[a] - h[9 - a] for a in range(1, 5)]
                te = _radix9_even(h[0], *e)
                to = _radix9_odd(*o)
                yield 256 + 8 * i, _pack(te[0][0:8], te[0][8:16])
                for r in range(4):
                    yield 64 * r + 16 * i, _pack(te[r + 1], to[r])

        def stage1(t):
            cols = pl.ds(pl.multiple_of(t * 128, 128), 128)
            xs = [x_v[pl.ds(16 * i, 16), cols].astype(f32) for i in range(D // 16)]
            m = _colmean(xs)
            ds = [v - m for v in xs]
            rs = lax.rsqrt(_colmean([d * d for d in ds]) + EPS)
            for r0, piece in radix9_fwd(lambda r0: ds[r0 // 16] * rs * mod_col(1, r0, 16)):
                t_v[pl.ds(r0, piece.shape[0]), cols] = piece

        def stage1_chunk(i, _):
            x_copy(i).wait()
            pl.when(i + 4 < XCH)(lambda: x_copy(i + 4).start())
            for n, cp in enumerate((f_copy, wr_copy, wi_copy, wm_copy(1))):
                pl.when(i == XCH - 4 + n)(cp.start)
            for t in range(NT // XCH):
                stage1(i * (NT // XCH) + t)
            return 0

        with _scope("stage1"):
            lax.fori_loop(0, XCH, stage1_chunk, 0)

        def d_forward(r, tmat):
            if r < 4:
                return _dot(_unpack(f_v[r]), _unpack(tmat(64 * r, 64)))
            return _dot(_unpack(f_v[4, 0:G0, 0:64]), _unpack(tmat(256, 32)))

        def group_rows(r):
            return range(0, 64 if r < 4 else G0, 8)

        with _scope("fwait"):
            f_copy.wait()
            start([wm_copy(2), b1_copy, b2_copy])
        with _scope("dfwd"):
            for r in range(5):
                for a1 in range(4):
                    z = d_forward(r, lambda r0, k: jnp.concatenate(
                        [t_v[r0:r0 + k, (a1 + 4 * a2) * 128:(a1 + 4 * a2 + 1) * 128] for a2 in range(4)], axis=1))
                    for i in group_rows(r):
                        u = _radix4(*[(z[2 * i:2 * i + 8, a2 * 128:(a2 + 1) * 128],
                                       z[2 * i + 8:2 * i + 16, a2 * 128:(a2 + 1) * 128]) for a2 in range(4)], -1)
                        for q1 in range(4):
                            u_v[r][a1, q1, 0, i:i + 8, :], u_v[r][a1, q1, 1, i:i + 8, :] = _twiddle16(
                                u[q1], a1 * q1, -1)
                for i in group_rows(r):
                    rows = slice(64 * r + i, 64 * r + i + 8)
                    for q1 in range(4):
                        y = _radix4(*[(u_v[r][a1, q1, 0, i:i + 8, :], u_v[r][a1, q1, 1, i:i + 8, :])
                                      for a1 in range(4)], -1)
                        for q2 in range(4):
                            yr_v[q1 + 4 * q2, rows, :], yi_v[q1 + 4 * q2, rows, :] = y[q2]

        def s_forward(k1):
            yr, yi = yr_v[k1], yi_v[k1]
            k, kr, ki = [_dot(y, _unpack(g_v[k1, n])) for n, y in enumerate((yr + yi, yr, yi))]
            xr_v[k1], xi_v[k1] = k - ki, k + kr

        with _scope("sfwd_a"):
            for k1 in range(NT - 1, NT - 1 - KSPLIT, -1):
                s_forward(k1)

        with _scope("wwait"):
            wr_copy.wait()
            wi_copy.wait()
            start(w1_copies(0))

        def permute(src, row0):
            a = [None] * NT
            for ct in range(NT):
                a[(-ct) % NT] = pltpu.roll(src[ct], ct, 1) if ct else src[ct]
            for bit in range(4):
                mask = ((lane >> bit) & 1) == 1
                a = [jnp.where(mask, a[(m - (1 << bit)) % NT], a[m]) for m in range(NT)]
            for k1 in range(NT):
                wp_v[k1, pl.ds(row0, 8), :] = a[k1]

        with _scope("sfwd_b_wperm"):
            for i in range(18):
                for src, base in ((wr_v, 0), (wi_v, 144)):
                    permute([pltpu.bitcast(src[16 * i:16 * i + 16, ct * 128:(ct + 1) * 128], jnp.int32)
                             for ct in range(NT)], base + 8 * i)
            permute([_pack(*[jnp.broadcast_to(w[288:289, ct * 128:(ct + 1) * 128].astype(f32), (8, 128))
                             for w in (wr_v, wi_v)]) for ct in range(NT)], 288)
            for k1 in range(NT - 1 - KSPLIT, -1, -1):
                s_forward(k1)

        def s_inverse(k1, shift=None):
            wr, wi = [], []
            for r in (1, 2, 3, 4, 0):
                for sg in _sigmas(r):
                    wr.append(_half(wp_v[k1, pl.ds(sg // 2, 16, stride=9), :], sg % 2))
                    wi.append(_half(wp_v[k1, pl.ds(144 + sg // 2, 16, stride=9), :], sg % 2))
            u = wp_v[k1, 288:296, :]
            wr = jnp.concatenate(wr + [_half(u, 0)], axis=0)
            wi = jnp.concatenate(wi + [_half(u, 1)], axis=0)
            xr, xi = xr_v[k1], xi_v[k1]
            if shift:
                xr, xi = xr + shift[0], xi + shift[1]
            fr = xr * wr - xi * wi
            fi = xr * wi + xi * wr
            k = _dot_nt(fr + fi, _unpack(g_v[k1, 0]))
            qr_v[k1] = k + _dot_nt(fi, _unpack(g_v[k1, 1]))
            qi_v[k1] = k - _dot_nt(fr, _unpack(g_v[k1, 2]))

        with _scope("sinv"):
            wm_copy(1).wait()
            start(w1_copies(1))
            modulation(act_v[...], 0, 4)
            for k1 in range(NT - 1, SA_AT, -1):
                s_inverse(k1)
            for r0, piece in radix9_fwd(lambda r0: mod_col(0, r0, 16)):
                zs_v[pl.ds(r0, piece.shape[0]), :] = piece
            shift = ([], [])
            for r in range(5):
                z = d_forward(r, lambda r0, k: zs_v[r0:r0 + k, :])
                for i in group_rows(r):
                    for n in range(2):
                        shift[n].append(jnp.where(lane == 0, z[2 * i + 8 * n:2 * i + 8 * n + 8] * float(S), 0.0))
            for k1 in range(SA_AT, 0, -1):
                s_inverse(k1)
            s_inverse(0, [jnp.concatenate(v, axis=0) for v in shift])

        with _scope("dinv"):
            wm_copy(2).wait()
            start(w1_copies(2))
            modulation(act_v[...], 1152, 18)
            for r in range(5):
                for i in group_rows(r):
                    rows = slice(64 * r + i, 64 * r + i + 8)
                    for q1 in range(4):
                        u = _radix4(*[(qr_v[q1 + 4 * q2, rows, :], qi_v[q1 + 4 * q2, rows, :])
                                      for q2 in range(4)], +1)
                        for a1 in range(4):
                            u_v[r][a1, q1, 0, i:i + 8, :], u_v[r][a1, q1, 1, i:i + 8, :] = _twiddle16(
                                u[a1], a1 * q1, +1)
                for a1 in range(4):
                    v = _radix4(*[(u_v[r][a1, q1, 0], u_v[r][a1, q1, 1]) for q1 in range(4)], +1)
                    vmat = _unpack(jnp.concatenate([_pack(*e) for e in v], axis=1))
                    if r < 4:
                        pr, r0 = _dot(_unpack(f_v[5 + r]), vmat), 128 * r
                    else:
                        pr, r0 = _dot(_unpack(f_v[9, 0:32, 0:2 * G0]), vmat), 512
                    for a2 in range(4):
                        p_v[a1 + 4 * a2, r0:r0 + pr.shape[0], :] = pr[:, a2 * 128:(a2 + 1) * 128]
            mod_v[4 * D:5 * D, :] = 1.0 + mod_v[4 * D:5 * D, :]
            sb = [mod_col(3, 16 * i, 16) for i in range(D // 16)]
            mean_sb = _colmean(sb)
            for i, v in enumerate(sb):
                mod_v[pl.ds(3 * D + 16 * i, 16), :] = v - mean_sb

        def split(ref, lead, r0):
            return jnp.concatenate([ref[(*lead, pl.ds(r0 + h, 8, stride=2), slice(None))] for h in range(2)], axis=0)

        def stage5(t, slot):
            cols = pl.ds(pl.multiple_of(t * 128, 128), 128)
            parts = []
            for i in range(4):
                pe = [p_v[t, pl.ds(512 + 16 * i, 16), :]] + [p_v[t, pl.ds(128 * r + 16 * i, 16), :] for r in range(4)]
                po = [p_v[t, pl.ds(128 * r + 64 + 16 * i, 16), :] for r in range(4)]
                ee = _radix9_even(*pe)
                oo = _radix9_odd(*po)
                ya = [ee[0]] + [ee[a] - oo[a - 1] for a in range(1, 5)] + [ee[a] + oo[a - 1] for a in (4, 3, 2, 1)]
                for a in range(9):
                    r0 = 64 * a + 16 * i
                    u = pltpu.bitcast(x_v[pl.ds(r0, 16), cols], jnp.int32)
                    v = jnp.concatenate([_half(u, 0), _half(u, 1)], axis=0) + split(mod_v, (), 2 * D + r0) * ya[a]
                    for h in range(2):
                        x1_v[t, pl.ds(r0 + h, 8, stride=2), :] = v[8 * h:8 * h + 8]
                    parts.append(v)
            m = _colmean(parts)
            squares, parts = [], []
            for i in range(D // 16):
                d = split(x1_v, (t,), 16 * i) - m
                e = d * split(mod_v, (), 4 * D + 16 * i)
                e_v[slot, pl.ds(16 * i, 16), :] = e
                squares.append(d * d)
                parts.append(e)
            rs = lax.rsqrt(_colmean(squares) + EPS)
            m = _colmean(parts)
            squares = []
            for i in range(D // 16):
                d = (e_v[slot, pl.ds(16 * i, 16), :] - m) * rs + split(mod_v, (), 3 * D + 16 * i)
                h_v[slot, pl.ds(16 * i, 16), :] = d
                squares.append(d * d)
            return lax.rsqrt(_colmean(squares) + EPS)

        def stage5_quad(t, _):
            scale = [stage5(4 * t + k, k) for k in range(4)]
            cols = pl.ds(pl.multiple_of(t * 128, 128), 128)
            for i in range(0, Q, 16):
                def block(mq, kq):
                    return h_v[kq, pl.ds(mq * Q + i, 16), :] * scale[kq]

                inner = [_strassen_lhs(*[block(2 * r + r2, 2 * c + c2) for r2, c2 in _QUADS]) for r, c in _QUADS]
                for q in range(7):
                    for p, op in enumerate(_strassen_lhs(*[ops[q] for ops in inner])):
                        a1_v[7 * p + q, pl.ds(i // 2, 8), cols] = _pack(op[0:8], op[8:16])
            return 0

        with _scope("stage5"):
            start(w1_copies(3))
            lax.fori_loop(0, NT // 4, stage5_quad, 0)

    def mlp(act_v, a2_v, out_v, b1_f, b2_f):
        def emit(inner, tile0):
            ops = [op for q in range(7) for op in _strassen_lhs(*[inner[rc][q] for rc in _QUADS])]
            for t in range(ops[0].shape[1] // 128):
                cols = pl.ds(pl.multiple_of((tile0 + t) * 256, 256), 256)
                for n in range(25):
                    a2_v[n, :, cols] = jnp.concatenate(
                        [ops[m][:, t * 128:(t + 1) * 128] for m in (2 * n, min(2 * n + 1, 48))], axis=1).astype(bf)

        def up(j):
            nt = fct // 4

            def tile(nq, t):
                return j * fct + 4 * t + nq

            def words(kq, nq, p, q):
                shift = zero_s[7 * p + (0 if p in SHARE_UP else q)]
                return jnp.concatenate([jnp.concatenate(
                    [w1_i[tile(nq, t) + shift, pl.ds(64 * (4 * k + kq), 64), :] for k in range(NT // 4)], axis=0)
                    for t in range(nt)], axis=1)

            inner = {}
            for r, c, u in _strassen2(lambda n: _unpack(a1_v[n]), words, ORDER_UP):
                inner[r, c] = _strassen_lhs(*[_gelu2(u[r2, c2] + jnp.concatenate(
                    [b1_f[pl.ds(tile(2 * c + c2, t), 1), :] for t in range(nt)], axis=1)) for r2, c2 in _QUADS])
            emit(inner, j * nt)

        def hidden(n):
            n = n % 7 * 7 + n // 7
            return jnp.concatenate(
                [a2_v[n // 2, :, pl.ds(256 * k + 128 * (n % 2), 128)] for k in range(F // 512)], axis=1)

        def up_block(jb, _):
            for u in range(UU):
                wait(w1_copies(jb * UU + u))
            for u in range(UU):
                up(jb * UU + u)
            return 0

        def down(j):
            def words(kq, nq, p, q):
                tile = 4 * j + nq + zero_s[7 * p + (0 if p in SHARE_DOWN else q)]
                return jnp.concatenate([w2_i[tile, pl.ds(64 * (4 * k + kq), 64), :] for k in range(F // 512)], axis=0)

            for r, c, y in _strassen2(hidden, words, ORDER_DOWN):
                for r2 in range(2):
                    r0 = (2 * r + r2) * Q
                    gate = mod_col(5, r0, Q)
                    halves = []
                    for c2 in range(2):
                        tile = 4 * j + 2 * c + c2
                        yt = 0.5 * y[r2, c2] + b2_f[pl.ds(tile, 1), :]
                        halves.append(x1_v[tile, pl.ds(r0, Q), :] + gate * yt)
                    out_v[j, r, c, pl.ds(r2 * Q, Q), :] = jnp.concatenate(halves, axis=1).astype(bf)
                out_copy(out_v, j, r, c).start()

        def down_block(jb, _):
            for u in range(UD):
                wait(w2_copies(jb * UD + u))
            for u in range(UD):
                down(jb * UD + u)
            return 0

        for j in range(4, nfc):
            start(w1_copies(j))
        b1_copy.wait()
        b2_copy.wait()
        b1_f[...] = b1_v[...].astype(f32)
        b2_f[...] = b2_v[...].astype(f32)
        with _scope("mlp_up"):
            def up_loop(jb, _):
                @pl.when(jb == 1)
                def _():
                    for j in range(nsc):
                        start(w2_copies(j))
                return up_block(jb, 0)

            lax.fori_loop(0, nfc // UU, up_loop, 0)
        with _scope("mlp_down"):
            lax.fori_loop(0, nsc // UD, down_block, 0)
        with _scope("outwait"):
            for j in range(nsc):
                for r, c in _QUADS:
                    out_copy(out_v, j, r, c).wait()

    def body(act_v):
        vmem = pltpu.VMEM
        i32 = jnp.int32
        pl.run_scoped(
            lambda *refs: front(act_v, *refs),
            vmem((D, S), bf), vmem((DF, S), bf), vmem((DF, S), bf), vmem(_FMAT.shape, i32),
            vmem(_SEEDS.shape, f32), vmem((1, D), bf), vmem((NT, 3, 64, 128), i32), vmem((NT, WROWS, 128), i32),
            vmem((H, S), i32), *[vmem((NT, NL, 128), f32)] * 6,
            vmem((NT, D, 128), f32), vmem((H, 128), i32),
            vmem((4, D, 128), f32), vmem((4, D, 128), f32), *[vmem((4, 4, 2, n, 128), f32) for n in (64, 64, 64, 64, G0)])
        pl.run_scoped(
            lambda *refs: mlp(act_v, *refs),
            vmem((25, Q, F // 2), bf), vmem((nsc, 2, 2, H, SC // 2), bf), vmem((F // 128, 128), f32),
            vmem((NT, 128), f32))

    pl.run_scoped(body, pltpu.VMEM((8, D), f32))


@jax.jit
def pallas_adaLN_cond__spectral_gfnet__mixer_token_mlp__prompt_kernel(A_x, A_w_r, A_w_i, B_x, B_w1, B_b1, B_w2, B_b2, c, w_mod):
    del B_x
    bf, f32, i32 = jnp.bfloat16, jnp.float32, jnp.int32
    hbm = pl.BlockSpec(memory_space=pl.ANY)
    out_t = pl.pallas_call(
        _kernel,
        out_shape=jax.ShapeDtypeStruct((D, S), bf),
        in_specs=[hbm] * 11,
        out_specs=hbm,
        scratch_shapes=[
            pltpu.VMEM((F // 128, S, 128), bf),
            pltpu.VMEM((NT, F, 128), bf),
            pltpu.VMEM((D, 6 * D), bf),
            pltpu.VMEM((F // 128, 128), bf),
            pltpu.VMEM((NT, 128), bf),
            pltpu.VMEM((6 * D, 128), f32),
            pltpu.VMEM((NT, D, 128), f32),
            pltpu.VMEM((49, Q // 2, S // 4), i32),
            pltpu.SMEM((49,), i32),
            pltpu.SemaphoreType.DMA((11,)),
            pltpu.SemaphoreType.DMA((XCH,)),
            pltpu.SemaphoreType.DMA((F // FC,)),
            pltpu.SemaphoreType.DMA((S // SC,)),
            pltpu.SemaphoreType.DMA((S // SC * 4,)),
        ],
        compiler_params=pltpu.CompilerParams(vmem_limit_bytes=120 * 1024 * 1024),
    )(A_x[0].T, A_w_r.T, A_w_i.T, B_w1, B_w2, w_mod, _FMAT, _SEEDS,
      B_b1.reshape(F // 128, 128), B_b2.reshape(S // 128, 128), c)
    return out_t.T[None]
```

```python
import contextlib
import math

import jax
import jax.numpy as jnp
import numpy as np
from jax import lax
import jax.experimental.pallas as pl
import jax.experimental.pallas.tpu as pltpu

S, D, F = 2048, 576, 4608
DF = D // 2 + 1
EPS = 1e-5
NT = S // 128
G0 = 40
NL = 4 * 64 + G0
WROWS = 296
H = D // 2

XCH = 8
FC = 512
Q = D // 4
UU = 1
UD = 1
KSPLIT = 2
SA_AT = 1
GROUP5 = 4
ORDER_UP = (2, 4, 1, 3, 0, 6, 5)
ORDER_DOWN = (2, 4, 1, 3, 0, 6, 5)
ORDER_IN = (4, 2, 1, 3, 0, 6, 5)
SHARE_UP = (0, 6, 5)
SHARE_DOWN = (0, 1, 2, 3, 4, 5, 6)
SC = 512
SCOPES = False

_C9 = [math.cos(2 * math.pi * j / 9) for j in range(9)]
_S9 = [math.sin(2 * math.pi * j / 9) for j in range(9)]


def _scope(name):
    return jax.named_scope(name) if SCOPES else contextlib.nullcontext()


def _sigmas(r):
    if r == 0:
        return [0, 9]
    return [r, r + 9, 9 - r, 18 - r]


def _pack_rows(m):
    u = m.astype(np.float32).astype(jnp.bfloat16).view(np.uint16).astype(np.uint32)
    return (u[..., 0::2, :] | (u[..., 1::2, :] << 16)).view(np.int32)


def _constants():
    dp = np.arange(64)
    ff = np.zeros((5, 128, 128))
    fi = np.zeros((5, 128, 128))
    scale = 1.0 / (D * S)

    def by8(re, im):
        return np.stack([re.reshape(-1, 8, re.shape[1]), im.reshape(-1, 8, im.shape[1])], 1).reshape(-1, re.shape[1])

    def even_odd(m):
        n = m.shape[0] // 16 * 16
        head = m[:n].reshape(-1, 8, 2, m.shape[1]).transpose(0, 2, 1, 3).reshape(n, m.shape[1])
        return np.concatenate([head, m[n:]], 0)

    def by1(a, b):
        return np.stack([a, b], 2).reshape(a.shape[0], -1)

    for r in range(1, 5):
        l = np.array([18 * m + sg for sg in _sigmas(r) for m in range(16)])
        th = 2 * np.pi * np.outer(l, dp) / D
        sg = np.where(l % 9 == r, 1.0, -1.0)[:, None]
        co, si = np.cos(th), np.sin(th)
        ff[r - 1] = by8(by1(co, -_S9[3] * sg * si), by1(-si, -_S9[3] * sg * co))
        fi[r - 1] = 2 * scale * even_odd(np.concatenate(
            [by1(co.T, -si.T), by1(_S9[3] * (sg * si).T, _S9[3] * (sg * co).T)], 0))
    l = np.array([18 * m + sg for sg in _sigmas(0) for m in range(16)] + [D // 2])
    th = 2 * np.pi * np.outer(l, dp) / D
    edge = (l == 0) | (l == D // 2)
    pad = ((0, G0 - len(l)), (0, 0))
    co, si = np.pad(np.cos(th), pad), np.pad(np.where(edge[:, None], 0.0, np.sin(th)), pad)
    order = np.array([16 * i + j + 8 * h for i in range(4) for j in range(8) for h in range(2)])
    ff[4, :2 * G0, :64] = by8(co[:, order], -si[:, order])
    cl = np.pad(np.where(edge, 1.0, 2.0), pad[0])[None, :]
    fi[4, :64, :2 * G0] = scale * even_odd(by1(cl * co.T, -cl * si.T))
    b = 2 * np.arange(8)[:, None]
    p = np.arange(128)[None, :]
    k0 = 128 * (p % 16) + 16 * (p // 16)
    step = -127 + 0 * p
    wrap = step + np.where(p < 16, 112, -16)
    seeds = []
    for bb in (b, b + 1, 16 + 0 * b):
        for k in (k0, step, wrap):
            z = np.exp(-2j * np.pi * bb * k / S)
            seeds += [z.real, z.imag]
    return _pack_rows(np.concatenate([ff, fi], 0)), np.concatenate(seeds, 0).astype(np.float32)


_FMAT, _SEEDS = _constants()


def _radix9_even(h0, e1, e2, e3, e4):
    p = h0 + e3
    q = e1 + e2 + e4
    t0 = p + q
    t3 = p - 0.5 * q
    g = h0 - 0.5 * e3
    u = e1 - e4
    v = e2 - e4
    a = _C9[1] * u + _C9[2] * v
    b = _C9[2] * u + _C9[4] * v
    return t0, g + a, g + b, t3, g - a - b


def _radix9_odd(o1, o2, o3, o4):
    t3 = o1 - o2 + o4
    u = o1 + o2
    v = o2 + o4
    a = (_S9[1] / _S9[3]) * u + (_S9[4] / _S9[3]) * v
    b = (_S9[2] / _S9[3]) * u - (_S9[1] / _S9[3]) * v
    return a + o3, b - o3, t3, b - a + o3


def _radix4(z0, z1, z2, z3, sign):
    ar, ai = z0[0] + z2[0], z0[1] + z2[1]
    br, bi = z0[0] - z2[0], z0[1] - z2[1]
    cr, ci = z1[0] + z3[0], z1[1] + z3[1]
    dr, di = z1[0] - z3[0], z1[1] - z3[1]
    plus = (br - di, bi + dr)
    minus = (br + di, bi - dr)
    if sign > 0:
        return (ar + cr, ai + ci), plus, (ar - cr, ai - ci), minus
    return (ar + cr, ai + ci), minus, (ar - cr, ai - ci), plus


def _twiddle16(z, n, sign):
    zr, zi = z
    n %= 16
    if n == 0:
        return z
    if n == 4:
        return (-zi, zr) if sign > 0 else (zi, -zr)
    c = math.cos(2 * math.pi * n / 16)
    s = sign * math.sin(2 * math.pi * n / 16)
    if n % 4 == 2:
        if (c > 0) == (s > 0):
            return c * (zr - zi), c * (zr + zi)
        return c * (zr + zi), c * (zi - zr)
    return c * zr - s * zi, c * zi + s * zr


def _radix16(z, sign):
    u = [_radix4(z[a1], z[a1 + 4], z[a1 + 8], z[a1 + 12], sign) for a1 in range(4)]
    out = [None] * 16
    for q1 in range(4):
        t = [_twiddle16(u[a1][q1], a1 * q1, sign) for a1 in range(4)]
        y = _radix4(*t, sign)
        for q2 in range(4):
            out[q1 + 4 * q2] = y[q2]
    return out


def _cmul(a, b):
    return a[0] * b[0] - a[1] * b[1], a[0] * b[1] + a[1] * b[0]


def _gelu2(x):
    k = math.sqrt(2 / math.pi)
    return x + x * jnp.tanh(x * (k + (k * 0.044715) * (x * x)))


class _Mean:
    def __init__(self):
        self.total = None

    def add(self, piece):
        self.total = piece if self.total is None else self.total + piece

    def value(self):
        return jnp.sum(self.total[0:8] + self.total[8:16], axis=0, keepdims=True) * (1.0 / D)


def _pack(lo, hi):
    return pltpu.pack_elementwise([lo, hi], packed_dtype=jnp.bfloat16).astype(jnp.int32)


def _half(u, index):
    return pltpu.unpack_elementwise(u, index=index, packed_dtype=jnp.bfloat16, unpacked_dtype=jnp.float32)


def _unpack(x):
    return pltpu.bitcast(x, jnp.bfloat16)


def _dot(a, b):
    return jnp.dot(a, b, preferred_element_type=jnp.float32)


def _dot_nt(a, b):
    return lax.dot_general(a, b, (((1,), (1,)), ((), ())), preferred_element_type=jnp.float32)


def _strassen_lhs(a11, a12, a21, a22):
    return (a11 + a22, a21 + a22, a11, a22, a11 + a12, a21 - a11, a12 - a22)


_QUADS = ((0, 0), (0, 1), (1, 0), (1, 1))
_STRASSEN_RHS = (
    (((0, 0), 1), ((1, 1), 1)), (((0, 0), 1),), (((0, 1), 1), ((1, 1), -1)), (((1, 0), 1), ((0, 0), -1)),
    (((1, 1), 1),), (((0, 0), 1), ((0, 1), 1)), (((1, 0), 1), ((1, 1), 1)))


def _signed_sum(terms, get):
    total = get(terms[0][0])
    for block, sign in terms[1:]:
        total = total + get(block) if sign > 0 else total - get(block)
    return total


_STRASSEN_OUT = {
    (0, 0): ((0, 1), (3, 1), (4, -1), (6, 1)), (0, 1): ((2, 1), (4, 1)),
    (1, 0): ((1, 1), (3, 1)), (1, 1): ((0, 1), (1, -1), (2, 1), (5, 1))}


def _strassen_out(product, order):
    done = {}
    for n in order:
        done[n] = product(n)
        for (r, c), terms in _STRASSEN_OUT.items():
            if n in dict(terms) and all(k in done for k, _ in terms):
                yield r, c, lambda f, terms=terms: _signed_sum(terms, lambda k: f(done[k]))


def _strassen2(lhs, words, order):
    def outer(p):
        def inner(q):
            def block(b, c):
                return words(2 * b[0] + c[0], 2 * b[1] + c[1], p, q)

            rp, rq = _STRASSEN_RHS[p], _STRASSEN_RHS[q]
            if len(rp) == 1 and len(rq) == 1:
                rhs = block(rp[0][0], rq[0][0])
            else:
                rhs = _pack(*[_signed_sum(rq, lambda c: _signed_sum(rp, lambda b: _half(block(b, c), h)))
                              for h in range(2)])
            return _dot(lhs(7 * p + q), _unpack(rhs))

        return {(r, c): f(lambda m: m) for r, c, f in _strassen_out(inner, ORDER_IN)}

    for r, c, f in _strassen_out(outer, order):
        yield r, c, {rc: f(lambda m: m[rc]) for rc in _QUADS}


def _kernel(x_hbm, wr_hbm, wi_hbm, w1_hbm, w2_hbm, wm_hbm, f_hbm, seed_hbm, b1_hbm, b2_hbm, c_hbm,
            out_hbm,
            w1_v, w2_v, wm_v, b1_v, b2_v, mod_v, x1_v, a1_v, zero_s, sem_in, sem_x, sem_w1, sem_w2, sem_out):
    f32, bf = jnp.float32, jnp.bfloat16
    xw = S // XCH
    nfc, nsc = F // FC, S // SC
    fct, sct = FC // 128, SC // 128

    wm_parts = ((512, 1152), (0, 512), (1152, 6 * D))

    def wm_copy(i):
        lo, hi = wm_parts[i]
        return pltpu.make_async_copy(wm_hbm.at[:, lo:hi], wm_v.at[:, lo:hi], sem_in.at[i])

    b1_copy = pltpu.make_async_copy(b1_hbm, b1_v, sem_in.at[4])
    b2_copy = pltpu.make_async_copy(b2_hbm, b2_v, sem_in.at[5])

    def w1_copies(j):
        return [pltpu.make_async_copy(w1_hbm.at[:, pl.ds(pl.multiple_of((j * fct + t) * 128, 128), 128)],
                                      w1_v.at[j * fct + t], sem_w1.at[j]) for t in range(fct)]

    def w2_copies(j):
        return [pltpu.make_async_copy(w2_hbm.at[:, pl.ds(pl.multiple_of((j * sct + t) * 128, 128), 128)],
                                      w2_v.at[j * sct + t], sem_w2.at[j]) for t in range(sct)]

    def out_copy(out_v, j, p, q):
        col = pl.multiple_of(j * SC + q * (SC // 2), SC // 2)
        return pltpu.make_async_copy(out_v.at[j, p, q], out_hbm.at[pl.ds(p * H, H), pl.ds(col, SC // 2)],
                                     sem_out.at[j * 4 + p * 2 + q])

    w1_i, w2_i = w1_v.bitcast(jnp.int32), w2_v.bitcast(jnp.int32)

    def start(copies):
        for cp in copies:
            cp.start()

    def wait(copies):
        for cp in copies:
            cp.wait()

    def modulation(act, lo, tiles):
        row = _dot(act, wm_v[:, pl.ds(lo, tiles * 128)])
        for t in range(tiles):
            tile = jnp.broadcast_to(row[0:1, t * 128:(t + 1) * 128], (128, 128))
            mod_v[pl.ds(lo + t * 128, 128), :] = tile.T

    def mod_col(which, r0, n):
        return mod_v[pl.ds(which * D + r0, n), :]

    def front(act_v, x_v, wr_v, wi_v, f_v, seed_v, c_v, g_v, wp_v, t_v, xr_v, xi_v, u_v, v_v,
              p_v, zs_v, e_v, h_v):
        def x_copy(i):
            cols = pl.ds(pl.multiple_of(i * xw, xw), xw)
            return pltpu.make_async_copy(x_hbm.at[:, cols], x_v.at[:, cols], sem_x.at[i])

        seed_copy, c_copy, f_copy, wr_copy, wi_copy = [
            pltpu.make_async_copy(src, dst, sem_in.at[6 + i]) for i, (src, dst) in enumerate(
                ((seed_hbm, seed_v), (c_hbm, c_v), (f_hbm, f_v), (wr_hbm, wr_v), (wi_hbm, wi_v)))]

        start([seed_copy, c_copy, wm_copy(0), x_copy(0)])
        for i in range(49):
            zero_s[i] = 0

        lane = lax.broadcasted_iota(jnp.int32, (8, 128), 1)
        with _scope("twiddle"):
            seed_copy.wait()
            start([x_copy(1)])
            sd = [(seed_v[16 * i:16 * i + 8, :], seed_v[16 * i + 8:16 * i + 16, :]) for i in range(9)]
            rows = [sd[0:3], sd[3:6]]
            for i in range(8):
                g = [row[0] for row in rows]
                for k1 in range(NT):
                    g_v[k1, 0, 8 * i:8 * i + 8, :] = _pack(g[0][0], g[1][0])
                    g_v[k1, 1, 8 * i:8 * i + 8, :] = _pack(g[0][1] - g[0][0], g[1][1] - g[1][0])
                    g_v[k1, 2, 8 * i:8 * i + 8, :] = _pack(g[0][1] + g[0][0], g[1][1] + g[1][0])
                    if k1 + 1 < NT:
                        at = (lane & 15) == k1
                        g = [_cmul(z, (jnp.where(at, row[2][0], row[1][0]), jnp.where(at, row[2][1], row[1][1])))
                             for z, row in zip(g, rows)]
                if i < 7:
                    rows = [[_cmul(z, w) for z, w in zip(row, sd[6:9])] for row in rows]

        with _scope("mod0"):
            c_copy.wait()
            start([x_copy(2)])
            cc = c_v[...].astype(f32)
            act_v[...] = jnp.broadcast_to(cc * jax.nn.sigmoid(cc), (8, D))
            wm_copy(0).wait()
            start([x_copy(3)])
            modulation(act_v[...], 512, 5)
            mod_v[D:2 * D, :] = 1.0 + mod_v[D:2 * D, :]

        def radix9_fwd(rows):
            for i in range(4):
                h = [rows(64 * a + 16 * i) for a in range(9)]
                e = [h[a] + h[9 - a] for a in range(1, 5)]
                o = [h[a] - h[9 - a] for a in range(1, 5)]
                te = _radix9_even(h[0], *e)
                to = _radix9_odd(*o)
                yield 256 + 8 * i, _pack(te[0][0:8], te[0][8:16])
                for r in range(4):
                    yield 64 * r + 16 * i, _pack(te[r + 1], to[r])

        def stage1(tiles):
            cols = [pl.ds(pl.multiple_of(t * 128, 128), 128) for t in tiles]
            mean, var = [_Mean() for _ in tiles], [_Mean() for _ in tiles]
            for n in range(len(tiles)):
                for i in range(0, D, 16):
                    mean[n].add(x_v[pl.ds(i, 16), cols[n]].astype(f32))
            for n in range(len(tiles)):
                m = mean[n].value()
                for i in range(0, D, 16):
                    d = x_v[pl.ds(i, 16), cols[n]].astype(f32) - m
                    e_v[n, pl.ds(i, 16), :] = d
                    var[n].add(d * d)
            for n in range(len(tiles)):
                rs = lax.rsqrt(var[n].value() + EPS)
                for r0, piece in radix9_fwd(lambda r0: e_v[n, pl.ds(r0, 16), :] * rs * mod_col(1, r0, 16)):
                    t_v[pl.ds(r0, piece.shape[0]), cols[n]] = piece

        def stage1_chunk(i, _):
            x_copy(i).wait()
            pl.when(i + 4 < XCH)(lambda: x_copy(i + 4).start())
            for n, cp in enumerate((f_copy, wr_copy, wi_copy, wm_copy(1))):
                pl.when(i == XCH - 4 + n)(cp.start)
            stage1([i * (NT // XCH) + t for t in range(NT // XCH)])
            return 0

        with _scope("stage1"):
            lax.fori_loop(0, XCH, stage1_chunk, 0)

        def d_forward(r, tmat):
            if r < 4:
                return _dot(_unpack(f_v[r]), _unpack(tmat(64 * r, 64)))
            return _dot(_unpack(f_v[4, 0:G0, 0:64]), _unpack(tmat(256, 32)))

        def group_rows(r):
            return range(0, 64 if r < 4 else G0, 8)

        with _scope("fwait"):
            f_copy.wait()
            start([wm_copy(2), b1_copy, b2_copy])
        with _scope("dfwd"):
            for r in range(5):
                for a1 in range(4):
                    z = d_forward(r, lambda r0, k: jnp.concatenate(
                        [t_v[r0:r0 + k, (a1 + 4 * a2) * 128:(a1 + 4 * a2 + 1) * 128] for a2 in range(4)], axis=1))
                    for i in group_rows(r):
                        u = _radix4(*[(z[2 * i:2 * i + 8, a2 * 128:(a2 + 1) * 128],
                                       z[2 * i + 8:2 * i + 16, a2 * 128:(a2 + 1) * 128]) for a2 in range(4)], -1)
                        for q1 in range(4):
                            rows = slice(64 * r + i, 64 * r + i + 8)
                            u_v[a1, q1, 0, rows, :], u_v[a1, q1, 1, rows, :] = _twiddle16(u[q1], a1 * q1, -1)

        def s_forward(q1):
            y = _radix4(*[(u_v[a1, q1, 0], u_v[a1, q1, 1]) for a1 in range(4)], -1)
            for q2, (yr, yi) in enumerate(y):
                k1 = q1 + 4 * q2
                k, kr, ki = [_dot(e, _unpack(g_v[k1, n])) for n, e in enumerate((yr + yi, yr, yi))]
                xr_v[k1], xi_v[k1] = k - ki, k + kr

        with _scope("sfwd_a"):
            for q1 in range(KSPLIT):
                s_forward(q1)

        with _scope("wwait"):
            wr_copy.wait()
            wi_copy.wait()
            start(w1_copies(0))

        def permute(src, row0):
            a = [None] * NT
            for ct in range(NT):
                a[(-ct) % NT] = pltpu.roll(src[ct], ct, 1) if ct else src[ct]
            for bit in range(4):
                mask = ((lane >> bit) & 1) == 1
                a = [jnp.where(mask, a[(m - (1 << bit)) % NT], a[m]) for m in range(NT)]
            for k1 in range(NT):
                wp_v[k1, pl.ds(row0, 8), :] = a[k1]

        with _scope("sfwd_b_wperm"):
            for i in range(18):
                for src, base in ((wr_v, 0), (wi_v, 144)):
                    permute([pltpu.bitcast(src[16 * i:16 * i + 16, ct * 128:(ct + 1) * 128], jnp.int32)
                             for ct in range(NT)], base + 8 * i)
            permute([_pack(*[jnp.broadcast_to(w[288:289, ct * 128:(ct + 1) * 128].astype(f32), (8, 128))
                             for w in (wr_v, wi_v)]) for ct in range(NT)], 288)
            for q1 in range(KSPLIT, 4):
                s_forward(q1)

        def s_inverse(k1, shift=None):
            wr, wi = [], []
            for r in (1, 2, 3, 4, 0):
                for sg in _sigmas(r):
                    wr.append(_half(wp_v[k1, pl.ds(sg // 2, 16, stride=9), :], sg % 2))
                    wi.append(_half(wp_v[k1, pl.ds(144 + sg // 2, 16, stride=9), :], sg % 2))
            u = wp_v[k1, 288:296, :]
            wr = jnp.concatenate(wr + [_half(u, 0)], axis=0)
            wi = jnp.concatenate(wi + [_half(u, 1)], axis=0)
            xr, xi = xr_v[k1], xi_v[k1]
            if shift:
                xr, xi = xr + shift[0], xi + shift[1]
            fr = xr * wr - xi * wi
            fi = xr * wi + xi * wr
            k = _dot_nt(fr + fi, _unpack(g_v[k1, 0]))
            return k + _dot_nt(fi, _unpack(g_v[k1, 1])), k - _dot_nt(fr, _unpack(g_v[k1, 2]))

        def s_inverse4(q1, shift=None):
            u = _radix4(*[s_inverse(q1 + 4 * q2, None if q2 else shift) for q2 in range(4)], +1)
            for a1 in range(4):
                v_v[a1, q1, 0], v_v[a1, q1, 1] = _twiddle16(u[a1], a1 * q1, +1)

        with _scope("sinv"):
            wm_copy(1).wait()
            start(w1_copies(1))
            modulation(act_v[...], 0, 4)
            for q1 in range(3, SA_AT, -1):
                s_inverse4(q1)
            for r0, piece in radix9_fwd(lambda r0: mod_col(0, r0, 16)):
                zs_v[pl.ds(r0, piece.shape[0]), :] = piece
            shift = ([], [])
            for r in range(5):
                z = d_forward(r, lambda r0, k: zs_v[r0:r0 + k, :])
                for i in group_rows(r):
                    for n in range(2):
                        shift[n].append(jnp.where(lane == 0, z[2 * i + 8 * n:2 * i + 8 * n + 8] * float(S), 0.0))
            for q1 in range(SA_AT, 0, -1):
                s_inverse4(q1)
            s_inverse4(0, [jnp.concatenate(v, axis=0) for v in shift])

        with _scope("dinv"):
            wm_copy(2).wait()
            start(w1_copies(2))
            modulation(act_v[...], 1152, 18)
            for r in range(5):
                rows = slice(64 * r, 64 * r + 64 if r < 4 else NL)
                for a1 in range(4):
                    v = _radix4(*[(v_v[a1, q1, 0, rows, :], v_v[a1, q1, 1, rows, :]) for q1 in range(4)], +1)
                    vmat = _unpack(jnp.concatenate([_pack(*e) for e in v], axis=1))
                    if r < 4:
                        pr, r0 = _dot(_unpack(f_v[5 + r]), vmat), 128 * r
                    else:
                        pr, r0 = _dot(_unpack(f_v[9, 0:32, 0:2 * G0]), vmat), 512
                    for a2 in range(4):
                        p_v[a1 + 4 * a2, r0:r0 + pr.shape[0], :] = pr[:, a2 * 128:(a2 + 1) * 128]
            mod_v[4 * D:5 * D, :] = 1.0 + mod_v[4 * D:5 * D, :]
            sb = [mod_col(3, 16 * i, 16) for i in range(D // 16)]
            mean_sb = _Mean()
            for v in sb:
                mean_sb.add(v)
            mean_sb = mean_sb.value()
            for i, v in enumerate(sb):
                mod_v[pl.ds(3 * D + 16 * i, 16), :] = v - mean_sb

        def split(ref, lead, r0):
            return jnp.concatenate([ref[(*lead, pl.ds(r0 + h, 8, stride=2), slice(None))] for h in range(2)], axis=0)

        def residual(t):
            cols = pl.ds(pl.multiple_of(t * 128, 128), 128)
            mean = _Mean()
            for i in range(4):
                pe = [p_v[t, pl.ds(512 + 16 * i, 16), :]] + [p_v[t, pl.ds(128 * r + 16 * i, 16), :] for r in range(4)]
                po = [p_v[t, pl.ds(128 * r + 64 + 16 * i, 16), :] for r in range(4)]
                ee = _radix9_even(*pe)
                oo = _radix9_odd(*po)
                for a in range(9):
                    ya = ee[0] if a == 0 else ee[a] - oo[a - 1] if a < 5 else ee[9 - a] + oo[8 - a]
                    r0 = 64 * a + 16 * i
                    u = pltpu.bitcast(x_v[pl.ds(r0, 16), cols], jnp.int32)
                    v = jnp.concatenate([_half(u, 0), _half(u, 1)], axis=0) + split(mod_v, (), 2 * D + r0) * ya
                    for h in range(2):
                        x1_v[t, pl.ds(r0 + h, 8, stride=2), :] = v[8 * h:8 * h + 8]
                    mean.add(v)
            return mean

        def norm_first(t, slot, m):
            var, mean = _Mean(), _Mean()
            for i in range(0, D, 16):
                d = split(x1_v, (t,), i) - m
                e = d * split(mod_v, (), 4 * D + i)
                e_v[slot, pl.ds(i, 16), :] = e
                var.add(d * d)
                mean.add(e)
            return var, mean

        def norm_second(slot, rs, m):
            var = _Mean()
            for i in range(0, D, 16):
                d = (e_v[slot, pl.ds(i, 16), :] - m) * rs + split(mod_v, (), 3 * D + i)
                h_v[slot, pl.ds(i, 16), :] = d
                var.add(d * d)
            return var

        def stage5_quad(t, _):
            scale = []
            for k0 in range(0, 4, GROUP5):
                slots = range(k0, k0 + GROUP5)
                means = [residual(4 * t + k) for k in slots]
                stats = [norm_first(4 * t + k, k, m.value()) for k, m in zip(slots, means)]
                spread = [norm_second(k, lax.rsqrt(v.value() + EPS), m.value()) for k, (v, m) in zip(slots, stats)]
                scale += [lax.rsqrt(v.value() + EPS) for v in spread]
            cols = pl.ds(pl.multiple_of(t * 128, 128), 128)
            for i in range(0, Q, 16):
                def block(mq, kq):
                    return h_v[kq, pl.ds(mq * Q + i, 16), :] * scale[kq]

                inner = [_strassen_lhs(*[block(2 * r + r2, 2 * c + c2) for r2, c2 in _QUADS]) for r, c in _QUADS]
                for q in range(7):
                    for p, op in enumerate(_strassen_lhs(*[ops[q] for ops in inner])):
                        a1_v[7 * p + q, pl.ds(i // 2, 8), cols] = _pack(op[0:8], op[8:16])
            return 0

        with _scope("stage5"):
            start(w1_copies(3))
            lax.fori_loop(0, NT // 4, stage5_quad, 0)

    def mlp(act_v, a2_v, out_v, b1_f, b2_f):
        def emit(inner, tile0):
            ops = [op for q in range(7) for op in _strassen_lhs(*[inner[rc][q] for rc in _QUADS])]
            for t in range(ops[0].shape[1] // 128):
                cols = pl.ds(pl.multiple_of((tile0 + t) * 256, 256), 256)
                for n in range(25):
                    a2_v[n, :, cols] = jnp.concatenate(
                        [ops[m][:, t * 128:(t + 1) * 128] for m in (2 * n, min(2 * n + 1, 48))], axis=1).astype(bf)

        def up(j):
            nt = fct // 4

            def tile(nq, t):
                return j * fct + 4 * t + nq

            def words(kq, nq, p, q):
                shift = zero_s[7 * p + (0 if p in SHARE_UP else q)]
                return jnp.concatenate([jnp.concatenate(
                    [w1_i[tile(nq, t) + shift, pl.ds(64 * (4 * k + kq), 64), :] for k in range(NT // 4)], axis=0)
                    for t in range(nt)], axis=1)

            inner = {}
            for r, c, u in _strassen2(lambda n: _unpack(a1_v[n]), words, ORDER_UP):
                inner[r, c] = _strassen_lhs(*[_gelu2(u[r2, c2] + jnp.concatenate(
                    [b1_f[pl.ds(tile(2 * c + c2, t), 1), :] for t in range(nt)], axis=1)) for r2, c2 in _QUADS])
            emit(inner, j * nt)

        def hidden(n):
            n = n % 7 * 7 + n // 7
            return jnp.concatenate(
                [a2_v[n // 2, :, pl.ds(256 * k + 128 * (n % 2), 128)] for k in range(F // 512)], axis=1)

        def up_block(jb, _):
            for u in range(UU):
                wait(w1_copies(jb * UU + u))
            for u in range(UU):
                up(jb * UU + u)
            return 0

        def down(j):
            def words(kq, nq, p, q):
                tile = 4 * j + nq + zero_s[7 * p + (0 if p in SHARE_DOWN else q)]
                return jnp.concatenate([w2_i[tile, pl.ds(64 * (4 * k + kq), 64), :] for k in range(F // 512)], axis=0)

            for r, c, y in _strassen2(hidden, words, ORDER_DOWN):
                for r2 in range(2):
                    r0 = (2 * r + r2) * Q
                    gate = mod_col(5, r0, Q)
                    halves = []
                    for c2 in range(2):
                        tile = 4 * j + 2 * c + c2
                        yt = 0.5 * y[r2, c2] + b2_f[pl.ds(tile, 1), :]
                        halves.append(x1_v[tile, pl.ds(r0, Q), :] + gate * yt)
                    out_v[j, r, c, pl.ds(r2 * Q, Q), :] = jnp.concatenate(halves, axis=1).astype(bf)
                out_copy(out_v, j, r, c).start()

        def down_block(jb, _):
            for u in range(UD):
                wait(w2_copies(jb * UD + u))
            for u in range(UD):
                down(jb * UD + u)
            return 0

        for j in range(4, nfc):
            start(w1_copies(j))
        b1_copy.wait()
        b2_copy.wait()
        b1_f[...] = b1_v[...].astype(f32)
        b2_f[...] = b2_v[...].astype(f32)
        with _scope("mlp_up"):
            def up_loop(jb, _):
                @pl.when(jb == 1)
                def _():
                    for j in range(nsc):
                        start(w2_copies(j))
                return up_block(jb, 0)

            lax.fori_loop(0, nfc // UU, up_loop, 0)
        with _scope("mlp_down"):
            lax.fori_loop(0, nsc // UD, down_block, 0)
        with _scope("outwait"):
            for j in range(nsc):
                for r, c in _QUADS:
                    out_copy(out_v, j, r, c).wait()

    def body(act_v):
        vmem = pltpu.VMEM
        i32 = jnp.int32
        pl.run_scoped(
            lambda *refs: front(act_v, *refs),
            vmem((D, S), bf), vmem((DF, S), bf), vmem((DF, S), bf), vmem(_FMAT.shape, i32),
            vmem(_SEEDS.shape, f32), vmem((1, D), bf), vmem((NT, 3, 64, 128), i32), vmem((NT, WROWS, 128), i32),
            vmem((H, S), i32), *[vmem((NT, NL, 128), f32)] * 2, *[vmem((4, 4, 2, NL, 128), f32)] * 2,
            vmem((NT, D, 128), f32), vmem((H, 128), i32), vmem((4, D, 128), f32), vmem((4, D, 128), f32))
        pl.run_scoped(
            lambda *refs: mlp(act_v, *refs),
            vmem((25, Q, F // 2), bf), vmem((nsc, 2, 2, H, SC // 2), bf), vmem((F // 128, 128), f32),
            vmem((NT, 128), f32))

    pl.run_scoped(body, pltpu.VMEM((8, D), f32))


@jax.jit
def pallas_adaLN_cond__spectral_gfnet__mixer_token_mlp__prompt_kernel(A_x, A_w_r, A_w_i, B_x, B_w1, B_b1, B_w2, B_b2, c, w_mod):
    del B_x
    bf, f32, i32 = jnp.bfloat16, jnp.float32, jnp.int32
    hbm = pl.BlockSpec(memory_space=pl.ANY)
    out_t = pl.pallas_call(
        _kernel,
        out_shape=jax.ShapeDtypeStruct((D, S), bf),
        in_specs=[hbm] * 11,
        out_specs=hbm,
        scratch_shapes=[
            pltpu.VMEM((F // 128, S, 128), bf),
            pltpu.VMEM((NT, F, 128), bf),
            pltpu.VMEM((D, 6 * D), bf),
            pltpu.VMEM((F // 128, 128), bf),
            pltpu.VMEM((NT, 128), bf),
            pltpu.VMEM((6 * D, 128), f32),
            pltpu.VMEM((NT, D, 128), f32),
            pltpu.VMEM((49, Q // 2, S // 4), i32),
            pltpu.SMEM((49,), i32),
            pltpu.SemaphoreType.DMA((11,)),
            pltpu.SemaphoreType.DMA((XCH,)),
            pltpu.SemaphoreType.DMA((F // FC,)),
            pltpu.SemaphoreType.DMA((S // SC,)),
            pltpu.SemaphoreType.DMA((S // SC * 4,)),
        ],
        compiler_params=pltpu.CompilerParams(vmem_limit_bytes=120 * 1024 * 1024),
    )(A_x[0].T, A_w_r.T, A_w_i.T, B_w1, B_w2, w_mod, _FMAT, _SEEDS,
      B_b1.reshape(F // 128, 128), B_b2.reshape(S // 128, 128), c)
    return out_t.T[None]
```

```python
import contextlib
import math

import jax
import jax.numpy as jnp
import numpy as np
from jax import lax
import jax.experimental.pallas as pl
import jax.experimental.pallas.tpu as pltpu

S, D, F = 2048, 576, 4608
DF = D // 2 + 1
EPS = 1e-5
NT = S // 128
G0 = 40
NL = 4 * 64 + G0
WROWS = 296
H = D // 2

XCH = 8
FC = 512
Q = D // 4
UU = 3
UD = 1
KSPLIT = 2
SA_AT = 2
GROUP5 = 2
KEEP_UP = False
KEEP_DOWN = False
EAGER = True
ORDER_UP = (4, 2, 1, 3, 0, 6, 5)
ORDER_DOWN = (2, 4, 1, 3, 0, 6, 5)
IN_UP = (4, 2, 1, 3, 0, 6, 5)
IN_DOWN = (4, 2, 1, 3, 0, 6, 5)
SHARE_UP = (0, 1, 2, 3, 4, 5, 6)
FLAGS = None
SHARE_DOWN = (0, 1, 2, 3, 4, 5, 6)
SC = 512
SCOPES = False

_C9 = [math.cos(2 * math.pi * j / 9) for j in range(9)]
_S9 = [math.sin(2 * math.pi * j / 9) for j in range(9)]


def _scope(name):
    return jax.named_scope(name) if SCOPES else contextlib.nullcontext()


def _sigmas(r):
    if r == 0:
        return [0, 9]
    return [r, r + 9, 9 - r, 18 - r]


def _pack_rows(m):
    u = m.astype(np.float32).astype(jnp.bfloat16).view(np.uint16).astype(np.uint32)
    return (u[..., 0::2, :] | (u[..., 1::2, :] << 16)).view(np.int32)


def _constants():
    dp = np.arange(64)
    ff = np.zeros((5, 128, 128))
    fi = np.zeros((5, 128, 128))
    scale = 1.0 / (D * S)

    def by8(re, im):
        return np.stack([re.reshape(-1, 8, re.shape[1]), im.reshape(-1, 8, im.shape[1])], 1).reshape(-1, re.shape[1])

    def even_odd(m):
        n = m.shape[0] // 16 * 16
        head = m[:n].reshape(-1, 8, 2, m.shape[1]).transpose(0, 2, 1, 3).reshape(n, m.shape[1])
        return np.concatenate([head, m[n:]], 0)

    def by1(a, b):
        return np.stack([a, b], 2).reshape(a.shape[0], -1)

    for r in range(1, 5):
        l = np.array([18 * m + sg for sg in _sigmas(r) for m in range(16)])
        th = 2 * np.pi * np.outer(l, dp) / D
        sg = np.where(l % 9 == r, 1.0, -1.0)[:, None]
        co, si = np.cos(th), np.sin(th)
        ff[r - 1] = by8(by1(co, -_S9[3] * sg * si), by1(-si, -_S9[3] * sg * co))
        fi[r - 1] = 2 * scale * even_odd(np.concatenate(
            [by1(co.T, -si.T), by1(_S9[3] * (sg * si).T, _S9[3] * (sg * co).T)], 0))
    l = np.array([18 * m + sg for sg in _sigmas(0) for m in range(16)] + [D // 2])
    th = 2 * np.pi * np.outer(l, dp) / D
    edge = (l == 0) | (l == D // 2)
    pad = ((0, G0 - len(l)), (0, 0))
    co, si = np.pad(np.cos(th), pad), np.pad(np.where(edge[:, None], 0.0, np.sin(th)), pad)
    order = np.array([16 * i + j + 8 * h for i in range(4) for j in range(8) for h in range(2)])
    ff[4, :2 * G0, :64] = by8(co[:, order], -si[:, order])
    cl = np.pad(np.where(edge, 1.0, 2.0), pad[0])[None, :]
    fi[4, :64, :2 * G0] = scale * even_odd(by1(cl * co.T, -cl * si.T))
    b = 2 * np.arange(8)[:, None]
    p = np.arange(128)[None, :]
    k0 = 128 * (p % 16) + 16 * (p // 16)
    step = -127 + 0 * p
    wrap = step + np.where(p < 16, 112, -16)
    seeds = []
    for bb in (b, b + 1, 16 + 0 * b):
        for k in (k0, step, wrap):
            z = np.exp(-2j * np.pi * bb * k / S)
            seeds += [z.real, z.imag]
    return _pack_rows(np.concatenate([ff, fi], 0)), np.concatenate(seeds, 0).astype(np.float32)


_FMAT, _SEEDS = _constants()


def _radix9_even(h0, e1, e2, e3, e4):
    p = h0 + e3
    q = e1 + e2 + e4
    t0 = p + q
    t3 = p - 0.5 * q
    g = h0 - 0.5 * e3
    u = e1 - e4
    v = e2 - e4
    a = _C9[1] * u + _C9[2] * v
    b = _C9[2] * u + _C9[4] * v
    return t0, g + a, g + b, t3, g - a - b


def _radix9_odd(o1, o2, o3, o4):
    t3 = o1 - o2 + o4
    u = o1 + o2
    v = o2 + o4
    a = (_S9[1] / _S9[3]) * u + (_S9[4] / _S9[3]) * v
    b = (_S9[2] / _S9[3]) * u - (_S9[1] / _S9[3]) * v
    return a + o3, b - o3, t3, b - a + o3


def _radix4(z0, z1, z2, z3, sign):
    ar, ai = z0[0] + z2[0], z0[1] + z2[1]
    br, bi = z0[0] - z2[0], z0[1] - z2[1]
    cr, ci = z1[0] + z3[0], z1[1] + z3[1]
    dr, di = z1[0] - z3[0], z1[1] - z3[1]
    plus = (br - di, bi + dr)
    minus = (br + di, bi - dr)
    if sign > 0:
        return (ar + cr, ai + ci), plus, (ar - cr, ai - ci), minus
    return (ar + cr, ai + ci), minus, (ar - cr, ai - ci), plus


def _twiddle16(z, n, sign):
    zr, zi = z
    n %= 16
    if n == 0:
        return z
    if n == 4:
        return (-zi, zr) if sign > 0 else (zi, -zr)
    c = math.cos(2 * math.pi * n / 16)
    s = sign * math.sin(2 * math.pi * n / 16)
    if n % 4 == 2:
        if (c > 0) == (s > 0):
            return c * (zr - zi), c * (zr + zi)
        return c * (zr + zi), c * (zi - zr)
    return c * zr - s * zi, c * zi + s * zr


def _radix16(z, sign):
    u = [_radix4(z[a1], z[a1 + 4], z[a1 + 8], z[a1 + 12], sign) for a1 in range(4)]
    out = [None] * 16
    for q1 in range(4):
        t = [_twiddle16(u[a1][q1], a1 * q1, sign) for a1 in range(4)]
        y = _radix4(*t, sign)
        for q2 in range(4):
            out[q1 + 4 * q2] = y[q2]
    return out


def _cmul(a, b):
    return a[0] * b[0] - a[1] * b[1], a[0] * b[1] + a[1] * b[0]


def _gelu2(x):
    k = math.sqrt(2 / math.pi)
    return x + x * jnp.tanh(x * (k + (k * 0.044715) * (x * x)))


class _Mean:
    def __init__(self):
        self.total = None

    def add(self, piece):
        self.total = piece if self.total is None else self.total + piece

    def value(self):
        return jnp.sum(self.total[0:8] + self.total[8:16], axis=0, keepdims=True) * (1.0 / D)


def _pack(lo, hi):
    return pltpu.pack_elementwise([lo, hi], packed_dtype=jnp.bfloat16).astype(jnp.int32)


def _half(u, index):
    return pltpu.unpack_elementwise(u, index=index, packed_dtype=jnp.bfloat16, unpacked_dtype=jnp.float32)


def _unpack(x):
    return pltpu.bitcast(x, jnp.bfloat16)


def _dot(a, b):
    return jnp.dot(a, b, preferred_element_type=jnp.float32)


def _dot_nt(a, b):
    return lax.dot_general(a, b, (((1,), (1,)), ((), ())), preferred_element_type=jnp.float32)


def _strassen_lhs(a11, a12, a21, a22):
    return (a11 + a22, a21 + a22, a11, a22, a11 + a12, a21 - a11, a12 - a22)


_QUADS = ((0, 0), (0, 1), (1, 0), (1, 1))
_STRASSEN_LHS = (
    (((0, 0), 1), ((1, 1), 1)), (((1, 0), 1), ((1, 1), 1)), (((0, 0), 1),), (((1, 1), 1),),
    (((0, 0), 1), ((0, 1), 1)), (((1, 0), 1), ((0, 0), -1)), (((0, 1), 1), ((1, 1), -1)))
_STRASSEN_RHS = (
    (((0, 0), 1), ((1, 1), 1)), (((0, 0), 1),), (((0, 1), 1), ((1, 1), -1)), (((1, 0), 1), ((0, 0), -1)),
    (((1, 1), 1),), (((0, 0), 1), ((0, 1), 1)), (((1, 0), 1), ((1, 1), 1)))


def _signed_sum(terms, get):
    total = get(terms[0][0])
    for block, sign in terms[1:]:
        total = total + get(block) if sign > 0 else total - get(block)
    return total


_STRASSEN_OUT = {
    (0, 0): ((0, 1), (3, 1), (4, -1), (6, 1)), (0, 1): ((2, 1), (4, 1)),
    (1, 0): ((1, 1), (3, 1)), (1, 1): ((0, 1), (1, -1), (2, 1), (5, 1))}


def _strassen_out(product, order):
    done = {}
    for n in order:
        done[n] = product(n)
        for (r, c), terms in _STRASSEN_OUT.items():
            if n in dict(terms) and all(k in done for k, _ in terms):
                yield r, c, lambda f, terms=terms: _signed_sum(terms, lambda k: f(done[k]))


def _strassen2(lhs, words, order, order_in, keep=None):
    def outer(p):
        def inner(q):
            def block(b, c):
                return words(2 * b[0] + c[0], 2 * b[1] + c[1], p, q)

            rp, rq = _STRASSEN_RHS[p], _STRASSEN_RHS[q]
            if len(rp) == 1 and len(rq) == 1:
                rhs = block(rp[0][0], rq[0][0])
            else:
                rhs = _pack(*[_signed_sum(rq, lambda c: _signed_sum(rp, lambda b: _half(block(b, c), h)))
                              for h in range(2)])
            return _dot(lhs(7 * p + q), _unpack(rhs))

        blocks = {}
        for r, c, f in _strassen_out(inner, order_in):
            blocks[r, c] = f(lambda m: m)
            if keep is not None:
                keep[p, r, c] = blocks[r, c]
        if keep is not None:
            return lambda rc: keep[p, rc[0], rc[1]]
        return lambda rc: blocks[rc]

    for r, c, f in _strassen_out(outer, order):
        yield r, c, {rc: f(lambda m: m(rc)) for rc in _QUADS}


def _kernel(x_hbm, wr_hbm, wi_hbm, w1_hbm, w2_hbm, wm_hbm, f_hbm, seed_hbm, b1_hbm, b2_hbm, c_hbm,
            out_hbm,
            w1_v, w2_v, wm_v, b1_v, b2_v, mod_v, x1_v, a1_v, zero_s, sem_in, sem_x, sem_w1, sem_w2, sem_out):
    f32, bf = jnp.float32, jnp.bfloat16
    xw = S // XCH
    nfc, nsc = F // FC, S // SC
    fct, sct = FC // 128, SC // 128

    wm_parts = ((512, 1152), (0, 512), (1152, 6 * D))

    def wm_copy(i):
        lo, hi = wm_parts[i]
        return pltpu.make_async_copy(wm_hbm.at[:, lo:hi], wm_v.at[:, lo:hi], sem_in.at[i])

    b1_copy = pltpu.make_async_copy(b1_hbm, b1_v, sem_in.at[4])
    b2_copy = pltpu.make_async_copy(b2_hbm, b2_v, sem_in.at[5])

    def w1_copies(j):
        return [pltpu.make_async_copy(w1_hbm.at[:, pl.ds(pl.multiple_of((j * fct + t) * 128, 128), 128)],
                                      w1_v.at[j * fct + t], sem_w1.at[j]) for t in range(fct)]

    def w2_copies(j):
        return [pltpu.make_async_copy(w2_hbm.at[:, pl.ds(pl.multiple_of((j * sct + t) * 128, 128), 128)],
                                      w2_v.at[j * sct + t], sem_w2.at[j]) for t in range(sct)]

    def out_copy(out_v, j, p, q):
        col = pl.multiple_of(j * SC + q * (SC // 2), SC // 2)
        return pltpu.make_async_copy(out_v.at[j, p, q], out_hbm.at[pl.ds(p * H, H), pl.ds(col, SC // 2)],
                                     sem_out.at[j * 4 + p * 2 + q])

    w1_i, w2_i = w1_v.bitcast(jnp.int32), w2_v.bitcast(jnp.int32)

    def start(copies):
        for cp in copies:
            cp.start()

    def wait(copies):
        for cp in copies:
            cp.wait()

    def modulation(act, lo, tiles):
        row = _dot(act, wm_v[:, pl.ds(lo, tiles * 128)])
        for t in range(tiles):
            tile = jnp.broadcast_to(row[0:1, t * 128:(t + 1) * 128], (128, 128))
            mod_v[pl.ds(lo + t * 128, 128), :] = tile.T

    def mod_col(which, r0, n):
        return mod_v[pl.ds(which * D + r0, n), :]

    def front(act_v, x_v, wr_v, wi_v, f_v, seed_v, c_v, g_v, wp_v, t_v, xr_v, xi_v, u_v, v_v,
              p_v, zs_v, e_v, h_v):
        def x_copy(i):
            cols = pl.ds(pl.multiple_of(i * xw, xw), xw)
            return pltpu.make_async_copy(x_hbm.at[:, cols], x_v.at[:, cols], sem_x.at[i])

        seed_copy, c_copy, f_copy, wr_copy, wi_copy = [
            pltpu.make_async_copy(src, dst, sem_in.at[6 + i]) for i, (src, dst) in enumerate(
                ((seed_hbm, seed_v), (c_hbm, c_v), (f_hbm, f_v), (wr_hbm, wr_v), (wi_hbm, wi_v)))]

        start([seed_copy, c_copy, wm_copy(0), x_copy(0)])
        for i in range(49):
            zero_s[i] = 0

        lane = lax.broadcasted_iota(jnp.int32, (8, 128), 1)
        with _scope("twiddle"):
            seed_copy.wait()
            start([x_copy(1)])
            sd = [(seed_v[16 * i:16 * i + 8, :], seed_v[16 * i + 8:16 * i + 16, :]) for i in range(9)]
            rows = [sd[0:3], sd[3:6]]
            for i in range(8):
                g = [row[0] for row in rows]
                for k1 in range(NT):
                    g_v[k1, 0, 8 * i:8 * i + 8, :] = _pack(g[0][0], g[1][0])
                    g_v[k1, 1, 8 * i:8 * i + 8, :] = _pack(g[0][1] - g[0][0], g[1][1] - g[1][0])
                    g_v[k1, 2, 8 * i:8 * i + 8, :] = _pack(g[0][1] + g[0][0], g[1][1] + g[1][0])
                    if k1 + 1 < NT:
                        at = (lane & 15) == k1
                        g = [_cmul(z, (jnp.where(at, row[2][0], row[1][0]), jnp.where(at, row[2][1], row[1][1])))
                             for z, row in zip(g, rows)]
                if i < 7:
                    rows = [[_cmul(z, w) for z, w in zip(row, sd[6:9])] for row in rows]

        with _scope("mod0"):
            c_copy.wait()
            start([x_copy(2)])
            cc = c_v[...].astype(f32)
            act_v[...] = jnp.broadcast_to(cc * jax.nn.sigmoid(cc), (8, D))
            wm_copy(0).wait()
            start([x_copy(3)])
            modulation(act_v[...], 512, 5)
            mod_v[D:2 * D, :] = 1.0 + mod_v[D:2 * D, :]

        def radix9_fwd(rows):
            for i in range(4):
                h = [rows(64 * a + 16 * i) for a in range(9)]
                e = [h[a] + h[9 - a] for a in range(1, 5)]
                o = [h[a] - h[9 - a] for a in range(1, 5)]
                te = _radix9_even(h[0], *e)
                to = _radix9_odd(*o)
                yield 256 + 8 * i, _pack(te[0][0:8], te[0][8:16])
                for r in range(4):
                    yield 64 * r + 16 * i, _pack(te[r + 1], to[r])

        def stage1(tiles):
            cols = [pl.ds(pl.multiple_of(t * 128, 128), 128) for t in tiles]
            mean, var = [_Mean() for _ in tiles], [_Mean() for _ in tiles]
            for n in range(len(tiles)):
                for i in range(0, D, 16):
                    mean[n].add(x_v[pl.ds(i, 16), cols[n]].astype(f32))
            for n in range(len(tiles)):
                m = mean[n].value()
                for i in range(0, D, 16):
                    d = x_v[pl.ds(i, 16), cols[n]].astype(f32) - m
                    e_v[n, pl.ds(i, 16), :] = d
                    var[n].add(d * d)
            for n in range(len(tiles)):
                rs = lax.rsqrt(var[n].value() + EPS)
                for r0, piece in radix9_fwd(lambda r0: e_v[n, pl.ds(r0, 16), :] * rs * mod_col(1, r0, 16)):
                    t_v[pl.ds(r0, piece.shape[0]), cols[n]] = piece

        def stage1_chunk(i, _):
            x_copy(i).wait()
            pl.when(i + 4 < XCH)(lambda: x_copy(i + 4).start())
            for n, cp in enumerate((f_copy, wr_copy, wi_copy, wm_copy(1))):
                pl.when(i == XCH - 4 + n)(cp.start)
            stage1([i * (NT // XCH) + t for t in range(NT // XCH)])
            return 0

        with _scope("stage1"):
            lax.fori_loop(0, XCH, stage1_chunk, 0)

        def d_forward(r, tmat):
            if r < 4:
                return _dot(_unpack(f_v[r]), _unpack(tmat(64 * r, 64)))
            return _dot(_unpack(f_v[4, 0:G0, 0:64]), _unpack(tmat(256, 32)))

        def group_rows(r):
            return range(0, 64 if r < 4 else G0, 8)

        with _scope("fwait"):
            f_copy.wait()
            start([wm_copy(2), b1_copy, b2_copy])
        with _scope("dfwd"):
            for r in range(5):
                for a1 in range(4):
                    z = d_forward(r, lambda r0, k: jnp.concatenate(
                        [t_v[r0:r0 + k, (a1 + 4 * a2) * 128:(a1 + 4 * a2 + 1) * 128] for a2 in range(4)], axis=1))
                    for i in group_rows(r):
                        u = _radix4(*[(z[2 * i:2 * i + 8, a2 * 128:(a2 + 1) * 128],
                                       z[2 * i + 8:2 * i + 16, a2 * 128:(a2 + 1) * 128]) for a2 in range(4)], -1)
                        for q1 in range(4):
                            rows = slice(64 * r + i, 64 * r + i + 8)
                            u_v[a1, q1, 0, rows, :], u_v[a1, q1, 1, rows, :] = _twiddle16(u[q1], a1 * q1, -1)

        def s_forward(q1):
            y = _radix4(*[(u_v[a1, q1, 0], u_v[a1, q1, 1]) for a1 in range(4)], -1)
            for q2, (yr, yi) in enumerate(y):
                k1 = q1 + 4 * q2
                k, kr, ki = [_dot(e, _unpack(g_v[k1, n])) for n, e in enumerate((yr + yi, yr, yi))]
                xr_v[k1], xi_v[k1] = k - ki, k + kr

        with _scope("sfwd_a"):
            for q1 in range(KSPLIT):
                s_forward(q1)

        with _scope("wwait"):
            wr_copy.wait()
            wi_copy.wait()
            start(w1_copies(0))

        def permute(src, row0):
            a = [None] * NT
            for ct in range(NT):
                a[(-ct) % NT] = pltpu.roll(src[ct], ct, 1) if ct else src[ct]
            for bit in range(4):
                mask = ((lane >> bit) & 1) == 1
                a = [jnp.where(mask, a[(m - (1 << bit)) % NT], a[m]) for m in range(NT)]
            for k1 in range(NT):
                wp_v[k1, pl.ds(row0, 8), :] = a[k1]

        with _scope("sfwd_b_wperm"):
            for i in range(18):
                for src, base in ((wr_v, 0), (wi_v, 144)):
                    permute([pltpu.bitcast(src[16 * i:16 * i + 16, ct * 128:(ct + 1) * 128], jnp.int32)
                             for ct in range(NT)], base + 8 * i)
            permute([_pack(*[jnp.broadcast_to(w[288:289, ct * 128:(ct + 1) * 128].astype(f32), (8, 128))
                             for w in (wr_v, wi_v)]) for ct in range(NT)], 288)
            for q1 in range(KSPLIT, 4):
                s_forward(q1)

        def s_inverse(k1, shift=None):
            wr, wi = [], []
            for r in (1, 2, 3, 4, 0):
                for sg in _sigmas(r):
                    wr.append(_half(wp_v[k1, pl.ds(sg // 2, 16, stride=9), :], sg % 2))
                    wi.append(_half(wp_v[k1, pl.ds(144 + sg // 2, 16, stride=9), :], sg % 2))
            u = wp_v[k1, 288:296, :]
            wr = jnp.concatenate(wr + [_half(u, 0)], axis=0)
            wi = jnp.concatenate(wi + [_half(u, 1)], axis=0)
            xr, xi = xr_v[k1], xi_v[k1]
            if shift:
                xr, xi = xr + shift[0], xi + shift[1]
            fr = xr * wr - xi * wi
            fi = xr * wi + xi * wr
            k = _dot_nt(fr + fi, _unpack(g_v[k1, 0]))
            return k + _dot_nt(fi, _unpack(g_v[k1, 1])), k - _dot_nt(fr, _unpack(g_v[k1, 2]))

        def s_inverse4(q1, shift=None):
            u = _radix4(*[s_inverse(q1 + 4 * q2, None if q2 else shift) for q2 in range(4)], +1)
            for a1 in range(4):
                v_v[a1, q1, 0], v_v[a1, q1, 1] = _twiddle16(u[a1], a1 * q1, +1)

        with _scope("sinv"):
            wm_copy(1).wait()
            start(w1_copies(1))
            modulation(act_v[...], 0, 4)
            for q1 in range(3, SA_AT, -1):
                s_inverse4(q1)
            for r0, piece in radix9_fwd(lambda r0: mod_col(0, r0, 16)):
                zs_v[pl.ds(r0, piece.shape[0]), :] = piece
            shift = ([], [])
            for r in range(5):
                z = d_forward(r, lambda r0, k: zs_v[r0:r0 + k, :])
                for i in group_rows(r):
                    for n in range(2):
                        shift[n].append(jnp.where(lane == 0, z[2 * i + 8 * n:2 * i + 8 * n + 8] * float(S), 0.0))
            for q1 in range(SA_AT, 0, -1):
                s_inverse4(q1)
            s_inverse4(0, [jnp.concatenate(v, axis=0) for v in shift])

        with _scope("dinv"):
            wm_copy(2).wait()
            start(w1_copies(2))
            modulation(act_v[...], 1152, 18)
            for r in range(5):
                rows = slice(64 * r, 64 * r + 64 if r < 4 else NL)
                for a1 in range(4):
                    v = _radix4(*[(v_v[a1, q1, 0, rows, :], v_v[a1, q1, 1, rows, :]) for q1 in range(4)], +1)
                    vmat = _unpack(jnp.concatenate([_pack(*e) for e in v], axis=1))
                    if r < 4:
                        pr, r0 = _dot(_unpack(f_v[5 + r]), vmat), 128 * r
                    else:
                        pr, r0 = _dot(_unpack(f_v[9, 0:32, 0:2 * G0]), vmat), 512
                    for a2 in range(4):
                        p_v[a1 + 4 * a2, r0:r0 + pr.shape[0], :] = pr[:, a2 * 128:(a2 + 1) * 128]
            mod_v[4 * D:5 * D, :] = 1.0 + mod_v[4 * D:5 * D, :]
            sb = [mod_col(3, 16 * i, 16) for i in range(D // 16)]
            mean_sb = _Mean()
            for v in sb:
                mean_sb.add(v)
            mean_sb = mean_sb.value()
            for i, v in enumerate(sb):
                mod_v[pl.ds(3 * D + 16 * i, 16), :] = v - mean_sb

        def split(ref, lead, r0):
            return jnp.concatenate([ref[(*lead, pl.ds(r0 + h, 8, stride=2), slice(None))] for h in range(2)], axis=0)

        def residual(t):
            cols = pl.ds(pl.multiple_of(t * 128, 128), 128)
            mean = _Mean()
            for i in range(4):
                pe = [p_v[t, pl.ds(512 + 16 * i, 16), :]] + [p_v[t, pl.ds(128 * r + 16 * i, 16), :] for r in range(4)]
                po = [p_v[t, pl.ds(128 * r + 64 + 16 * i, 16), :] for r in range(4)]
                ee = _radix9_even(*pe)
                oo = _radix9_odd(*po)
                for a in range(9):
                    ya = ee[0] if a == 0 else ee[a] - oo[a - 1] if a < 5 else ee[9 - a] + oo[8 - a]
                    r0 = 64 * a + 16 * i
                    u = pltpu.bitcast(x_v[pl.ds(r0, 16), cols], jnp.int32)
                    v = jnp.concatenate([_half(u, 0), _half(u, 1)], axis=0) + split(mod_v, (), 2 * D + r0) * ya
                    for h in range(2):
                        x1_v[t, pl.ds(r0 + h, 8, stride=2), :] = v[8 * h:8 * h + 8]
                    mean.add(v)
            return mean

        def norm_first(t, slot, m):
            var, mean = _Mean(), _Mean()
            for i in range(0, D, 16):
                d = split(x1_v, (t,), i) - m
                e = d * split(mod_v, (), 4 * D + i)
                e_v[slot, pl.ds(i, 16), :] = e
                var.add(d * d)
                mean.add(e)
            return var, mean

        def norm_second(slot, rs, m):
            var = _Mean()
            for i in range(0, D, 16):
                d = (e_v[slot, pl.ds(i, 16), :] - m) * rs + split(mod_v, (), 3 * D + i)
                h_v[slot, pl.ds(i, 16), :] = d
                var.add(d * d)
            return var

        def stage5_quad(t, _):
            scale = []
            for k0 in range(0, 4, GROUP5):
                slots = range(k0, k0 + GROUP5)
                means = [residual(4 * t + k) for k in slots]
                stats = [norm_first(4 * t + k, k, m.value()) for k, m in zip(slots, means)]
                spread = [norm_second(k, lax.rsqrt(v.value() + EPS), m.value()) for k, (v, m) in zip(slots, stats)]
                scale += [lax.rsqrt(v.value() + EPS) for v in spread]
            cols = pl.ds(pl.multiple_of(t * 128, 128), 128)
            for i in range(0, Q, 16):
                def block(mq, kq):
                    return h_v[kq, pl.ds(mq * Q + i, 16), :] * scale[kq]

                inner = [_strassen_lhs(*[block(2 * r + r2, 2 * c + c2) for r2, c2 in _QUADS]) for r, c in _QUADS]
                for q in range(7):
                    for p, op in enumerate(_strassen_lhs(*[ops[q] for ops in inner])):
                        a1_v[7 * p + q, pl.ds(i // 2, 8), cols] = _pack(op[0:8], op[8:16])
            return 0

        with _scope("stage5"):
            start(w1_copies(3))
            lax.fori_loop(0, NT // 4, stage5_quad, 0)

    def mlp(act_v, a2_v, m_v, out_v, b1_f, b2_f):
        pairs = ([((2, q), (2, min(q + 1, 6))) for q in range(0, 7, 2)] +
                 [((a, q), (b, q)) for a, b in ((3, 0), (4, 6), (1, 5)) for q in range(7)])
        place = {op: (n, side) for n, pair in enumerate(pairs) for side, op in reversed(list(enumerate(pair)))}

        def up(j):
            nt = fct // 4

            def tile(nq, t):
                return j * fct + 4 * t + nq

            def words(kq, nq, p, q):
                shift = zero_s[7 * p + (0 if p in SHARE_UP else q)]
                return jnp.concatenate([jnp.concatenate(
                    [w1_i[tile(nq, t) + shift, pl.ds(64 * (4 * k + kq), 64), :] for k in range(NT // 4)], axis=0)
                    for t in range(nt)], axis=1)

            cols = pl.ds(pl.multiple_of(j * 256, 256), 256)
            blocks, todo = {}, list(enumerate(pairs))
            for r, c, u in _strassen2(lambda n: _unpack(a1_v[n]), words, ORDER_UP, IN_UP, m_v if KEEP_UP else None):
                g = {rc: _gelu2(u[rc] + b1_f[pl.ds(tile(2 * c + rc[1], 0), 1), :]) for rc in _QUADS}
                blocks[r, 1 - c] = _strassen_lhs(g[0, 1], g[0, 0], g[1, 1], g[1, 0])
                for n, pair in list(todo):
                    if all(k in blocks for p, _ in pair for k, _ in _STRASSEN_LHS[p]) and (EAGER or len(blocks) == 4):
                        todo.remove((n, pair))
                        a2_v[n, :, cols] = jnp.concatenate(
                            [_signed_sum(_STRASSEN_LHS[p], lambda k: blocks[k][q]) for p, q in pair], axis=1).astype(bf)

        def hidden(n):
            pair, side = place[divmod(n, 7)]
            return jnp.concatenate(
                [a2_v[pair, :, pl.ds(256 * k + 128 * side, 128)] for k in range(F // 512)], axis=1)

        def up_block(jb, _):
            for u in range(UU):
                wait(w1_copies(jb * UU + u))
            for u in range(UU):
                up(jb * UU + u)
            return 0

        def down(j):
            def words(kq, nq, p, q):
                tile = 4 * j + nq + zero_s[7 * p + (0 if p in SHARE_DOWN else q)]
                return jnp.concatenate([w2_i[tile, pl.ds(64 * (4 * k + 3 - kq), 64), :] for k in range(F // 512)], axis=0)

            for r, c, y in _strassen2(hidden, words, ORDER_DOWN, IN_DOWN, m_v if KEEP_DOWN else None):
                for r2 in range(2):
                    r0 = (2 * r + r2) * Q
                    gate = mod_col(5, r0, Q)
                    halves = []
                    for c2 in range(2):
                        tile = 4 * j + 2 * c + c2
                        yt = 0.5 * y[r2, c2] + b2_f[pl.ds(tile, 1), :]
                        halves.append(x1_v[tile, pl.ds(r0, Q), :] + gate * yt)
                    out_v[j, r, c, pl.ds(r2 * Q, Q), :] = jnp.concatenate(halves, axis=1).astype(bf)
                out_copy(out_v, j, r, c).start()

        def down_block(jb, _):
            for u in range(UD):
                wait(w2_copies(jb * UD + u))
            for u in range(UD):
                down(jb * UD + u)
            return 0

        for j in range(4, nfc):
            start(w1_copies(j))
        b1_copy.wait()
        b2_copy.wait()
        b1_f[...] = b1_v[...].astype(f32)
        b2_f[...] = b2_v[...].astype(f32)
        with _scope("mlp_up"):
            def up_loop(jb, _):
                @pl.when(jb == 1)
                def _():
                    for j in range(nsc):
                        start(w2_copies(j))
                return up_block(jb, 0)

            lax.fori_loop(0, nfc // UU, up_loop, 0)
        with _scope("mlp_down"):
            lax.fori_loop(0, nsc // UD, down_block, 0)
        with _scope("outwait"):
            for j in range(nsc):
                for r, c in _QUADS:
                    out_copy(out_v, j, r, c).wait()

    def body(act_v):
        vmem = pltpu.VMEM
        i32 = jnp.int32
        pl.run_scoped(
            lambda *refs: front(act_v, *refs),
            vmem((D, S), bf), vmem((DF, S), bf), vmem((DF, S), bf), vmem(_FMAT.shape, i32),
            vmem(_SEEDS.shape, f32), vmem((1, D), bf), vmem((NT, 3, 64, 128), i32), vmem((NT, WROWS, 128), i32),
            vmem((H, S), i32), *[vmem((NT, NL, 128), f32)] * 2, *[vmem((4, 4, 2, NL, 128), f32)] * 2,
            vmem((NT, D, 128), f32), vmem((H, 128), i32), vmem((4, D, 128), f32), vmem((4, D, 128), f32))
        pl.run_scoped(
            lambda *refs: mlp(act_v, *refs),
            vmem((25, Q, F // 2), bf), vmem((7, 2, 2, Q, 128), f32), vmem((nsc, 2, 2, H, SC // 2), bf), vmem((F // 128, 128), f32),
            vmem((NT, 128), f32))

    pl.run_scoped(body, pltpu.VMEM((8, D), f32))


@jax.jit
def pallas_adaLN_cond__spectral_gfnet__mixer_token_mlp__prompt_kernel(A_x, A_w_r, A_w_i, B_x, B_w1, B_b1, B_w2, B_b2, c, w_mod):
    del B_x
    bf, f32, i32 = jnp.bfloat16, jnp.float32, jnp.int32
    hbm = pl.BlockSpec(memory_space=pl.ANY)
    out_t = pl.pallas_call(
        _kernel,
        out_shape=jax.ShapeDtypeStruct((D, S), bf),
        in_specs=[hbm] * 11,
        out_specs=hbm,
        scratch_shapes=[
            pltpu.VMEM((F // 128, S, 128), bf),
            pltpu.VMEM((NT, F, 128), bf),
            pltpu.VMEM((D, 6 * D), bf),
            pltpu.VMEM((F // 128, 128), bf),
            pltpu.VMEM((NT, 128), bf),
            pltpu.VMEM((6 * D, 128), f32),
            pltpu.VMEM((NT, D, 128), f32),
            pltpu.VMEM((49, Q // 2, S // 4), i32),
            pltpu.SMEM((49,), i32),
            pltpu.SemaphoreType.DMA((11,)),
            pltpu.SemaphoreType.DMA((XCH,)),
            pltpu.SemaphoreType.DMA((F // FC,)),
            pltpu.SemaphoreType.DMA((S // SC,)),
            pltpu.SemaphoreType.DMA((S // SC * 4,)),
        ],
        compiler_params=pltpu.CompilerParams(vmem_limit_bytes=120 * 1024 * 1024, flags=FLAGS),
    )(A_x[0].T, A_w_r.T, A_w_i.T, B_w1, B_w2, w_mod, _FMAT, _SEEDS,
      B_b1.reshape(F // 128, 128), B_b2.reshape(S // 128, 128), c)
    return out_t.T[None]
```

```python
import contextlib
import math

import jax
import jax.numpy as jnp
import numpy as np
from jax import lax
import jax.experimental.pallas as pl
import jax.experimental.pallas.tpu as pltpu

S, D, F = 2048, 576, 4608
DF = D // 2 + 1
EPS = 1e-5
NT = S // 128
G0 = 40
NL = 4 * 64 + G0
WROWS = 296
H, Q = D // 2, D // 4
XCH = 8
NUP, NDOWN = F // 512, S // 512
UP_UNROLL = 3
SCOPES = False

_C9 = [math.cos(2 * math.pi * j / 9) for j in range(9)]
_S9 = [math.sin(2 * math.pi * j / 9) for j in range(9)]


def _scope(name):
    return jax.named_scope(name) if SCOPES else contextlib.nullcontext()


def _classes(r):
    return [r, r + 9, 9 - r, 18 - r] if r else [0, 9]


def _bf16_pairs(m):
    u = np.ascontiguousarray(m, dtype=np.float32).view(np.uint32)
    u = (u + 0x7FFF + ((u >> 16) & 1)) >> 16
    return (u[..., 0::2, :] | (u[..., 1::2, :] << 16)).view(np.int32)


def _constants():
    def by8(re, im):
        n = re.shape[1]
        return np.stack([re.reshape(-1, 8, n), im.reshape(-1, 8, n)], 1).reshape(-1, n)

    d = np.arange(64)
    fwd, inv = np.zeros((5, 128, 128)), np.zeros((5, 128, 128))
    scale = 1.0 / (D * S)
    for r in range(1, 5):
        l = np.array([18 * m + res for res in _classes(r) for m in range(16)])
        angle = 2 * np.pi * np.outer(l, d) / D
        co, si = np.cos(angle), np.sin(angle)
        odd = _S9[3] * np.where(l % 9 == r, 1.0, -1.0)[:, None]
        fwd[r - 1] = by8(np.hstack([co, -odd * si]), np.hstack([-si, -odd * co]))
        inv[r - 1] = 2 * scale * np.block([[co.T, -si.T], [(odd * si).T, (odd * co).T]])
    l = np.array([18 * m + res for res in _classes(0) for m in range(16)] + [D // 2])
    angle = 2 * np.pi * np.outer(l, d) / D
    edge = (l == 0) | (l == D // 2)
    pad = ((0, G0 - len(l)), (0, 0))
    co, si = np.pad(np.cos(angle), pad), np.pad(np.where(edge[:, None], 0.0, np.sin(angle)), pad)
    fwd[4, :2 * G0, :64] = by8(co, -si)
    weight = scale * np.pad(np.where(edge, 1.0, 2.0), pad[0])[None, :]
    inv[4, :64, :2 * G0] = np.hstack([weight * co.T, -weight * si.T])

    b, p = np.arange(8)[:, None], np.arange(128)[None, :]
    first = 128 * (p % 16) + 16 * (p // 16)
    step = -127 + 0 * p
    wrap = step + np.where(p < 16, 112, -16)
    seeds = []
    for rows in (b, b + 8, 16 + 0 * b):
        for k in (first, step, wrap):
            z = np.exp(-2j * np.pi * rows * k / S)
            seeds += [z.real, z.imag]
    return _bf16_pairs(np.concatenate([fwd, inv], 0)), np.concatenate(seeds, 0).astype(np.float32)


_DFT64, _SEEDS = _constants()


def _radix9_even(h0, e1, e2, e3, e4):
    p = h0 + e3
    q = e1 + e2 + e4
    g = h0 - 0.5 * e3
    u, v = e1 - e4, e2 - e4
    a = _C9[1] * u + _C9[2] * v
    b = _C9[2] * u + _C9[4] * v
    return p + q, g + a, g + b, p - 0.5 * q, g - a - b


def _radix9_odd(o1, o2, o3, o4):
    u, v = o1 + o2, o2 + o4
    a = (_S9[1] / _S9[3]) * u + (_S9[4] / _S9[3]) * v
    b = (_S9[2] / _S9[3]) * u - (_S9[1] / _S9[3]) * v
    return a + o3, b - o3, o1 - o2 + o4, b - a + o3


def _radix4(z0, z1, z2, z3, sign):
    ar, ai = z0[0] + z2[0], z0[1] + z2[1]
    br, bi = z0[0] - z2[0], z0[1] - z2[1]
    cr, ci = z1[0] + z3[0], z1[1] + z3[1]
    dr, di = z1[0] - z3[0], z1[1] - z3[1]
    plus, minus = (br - di, bi + dr), (br + di, bi - dr)
    if sign < 0:
        plus, minus = minus, plus
    return (ar + cr, ai + ci), plus, (ar - cr, ai - ci), minus


def _twiddle16(z, n, sign):
    zr, zi = z
    if n == 0:
        return z
    if n == 4:
        return (-zi, zr) if sign > 0 else (zi, -zr)
    c, s = math.cos(2 * math.pi * n / 16), sign * math.sin(2 * math.pi * n / 16)
    if n % 4 == 2:
        if (c > 0) == (s > 0):
            return c * (zr - zi), c * (zr + zi)
        return c * (zr + zi), c * (zi - zr)
    return c * zr - s * zi, c * zi + s * zr


def _cmul(a, b):
    return a[0] * b[0] - a[1] * b[1], a[0] * b[1] + a[1] * b[0]


def _gelu2(x):
    k = math.sqrt(2 / math.pi)
    return x + x * jnp.tanh(x * (k + (k * 0.044715) * (x * x)))


class _Mean:
    def __init__(self):
        self.total = None

    def add(self, piece):
        self.total = piece if self.total is None else self.total + piece

    def value(self):
        return jnp.sum(self.total[0:8] + self.total[8:16], axis=0, keepdims=True) * (1.0 / D)


def _as_bf16(words):
    return pltpu.bitcast(words, jnp.bfloat16)


def _word_half(words, high):
    return pltpu.bitcast(words & jnp.int32(-65536) if high else words << 16, jnp.float32)


def _dot(a, b):
    return jnp.dot(a, b, preferred_element_type=jnp.float32)


def _dot_nt(a, b):
    return lax.dot_general(a, b, (((1,), (1,)), ((), ())), preferred_element_type=jnp.float32)


_QUADS = ((0, 0), (0, 1), (1, 0), (1, 1))
_LEFT = ((((0, 0), 1), ((1, 1), 1)), (((1, 0), 1), ((1, 1), 1)), (((0, 0), 1),), (((1, 1), 1),),
         (((0, 0), 1), ((0, 1), 1)), (((1, 0), 1), ((0, 0), -1)), (((0, 1), 1), ((1, 1), -1)))
_RIGHT = ((((0, 0), 1), ((1, 1), 1)), (((0, 0), 1),), (((0, 1), 1), ((1, 1), -1)), (((1, 0), 1), ((0, 0), -1)),
          (((1, 1), 1),), (((0, 0), 1), ((0, 1), 1)), (((1, 0), 1), ((1, 1), 1)))
_OUTPUT = (((0, 0), ((0, 1), (3, 1), (4, -1), (6, 1))), ((0, 1), ((2, 1), (4, 1))),
           ((1, 0), ((1, 1), (3, 1))), ((1, 1), ((0, 1), (1, -1), (2, 1), (5, 1))))
ORDER_UP = (4, 2, 1, 3, 0, 6, 5)
ORDER_DOWN = (2, 4, 1, 3, 0, 6, 5)
ORDER_IN = (4, 2, 1, 3, 0, 6, 5)
_PAIRS = ([((2, q), (2, min(q + 1, 6))) for q in range(0, 7, 2)] +
          [((a, q), (b, q)) for a, b in ((3, 0), (4, 6), (1, 5)) for q in range(7)])
_PLACE = {op: (n, side) for n, pair in enumerate(_PAIRS) for side, op in ((1, pair[1]), (0, pair[0]))}


def _signed_sum(terms, get):
    total = get(terms[0][0])
    for key, sign in terms[1:]:
        total = total + get(key) if sign > 0 else total - get(key)
    return total


def _left_operands(blocks):
    return [_signed_sum(terms, blocks.get) for terms in _LEFT]


def _paired(pair, inner):
    return jnp.concatenate(
        [_signed_sum(_LEFT[p], lambda rc: inner[rc][q]) for p, q in pair], axis=1).astype(jnp.bfloat16)


def _strassen_level(product, order):
    done = {}
    for n in order:
        done[n] = product(n)
        for (r, c), terms in _OUTPUT:
            if n in dict(terms) and all(k in done for k, _ in terms):
                yield r, c, lambda f, terms=terms: _signed_sum(terms, lambda k: f(done[k]))


def _strassen2(left_ref, right, order):
    def outer(p):
        def inner(q):
            def block(b, c):
                return right(2 * b[0] + c[0], 2 * b[1] + c[1], p)

            if len(_RIGHT[p]) == 1 and len(_RIGHT[q]) == 1:
                rhs = block(_RIGHT[p][0][0], _RIGHT[q][0][0])
            else:
                rhs = _signed_sum(_RIGHT[q], lambda c: _signed_sum(
                    _RIGHT[p], lambda b: block(b, c).astype(jnp.float32))).astype(jnp.bfloat16)
            n, side = _PLACE[p, q]
            lhs = jnp.concatenate(
                [left_ref[n, :, k + 128 * side:k + 128 * (side + 1)] for k in range(0, left_ref.shape[2], 256)],
                axis=1)
            return _dot(lhs, rhs)

        return {(r, c): combine(lambda m: m) for r, c, combine in _strassen_level(inner, ORDER_IN)}

    for r, c, combine in _strassen_level(outer, order):
        yield r, c, {rc: combine(lambda m: m[rc]) for rc in _QUADS}


def _kernel(x_hbm, wr_hbm, wi_hbm, w1_hbm, w2_hbm, wm_hbm, f_hbm, seed_hbm, b1_hbm, b2_hbm, c_hbm,
            out_hbm,
            w1_v, w2_v, b1_v, b2_v, mod_v, x1_v, a1_v, zero_s, sem_in, sem_x, sem_w1, sem_w2, sem_out):
    f32, bf16, i32 = jnp.float32, jnp.bfloat16, jnp.int32

    def tile_copies(src, dst, sem, j):
        return [pltpu.make_async_copy(src.at[:, pl.ds(pl.multiple_of((4 * j + t) * 128, 128), 128)],
                                      dst.at[4 * j + t], sem.at[j]) for t in range(4)]

    def w1_copies(j):
        return tile_copies(w1_hbm, w1_v, sem_w1, j)

    def w2_copies(j):
        return tile_copies(w2_hbm, w2_v, sem_w2, j)

    def start(copies):
        for copy in copies:
            copy.start()

    def wait(copies):
        for copy in copies:
            copy.wait()

    bias_copies = [pltpu.make_async_copy(b1_hbm, b1_v, sem_in.at[0]),
                   pltpu.make_async_copy(b2_hbm, b2_v, sem_in.at[1])]

    def mod_col(which, row, n=16):
        return mod_v[which * D + row:which * D + row + n, :]

    def spectral(x_v, wr_v, wi_v, wm_v, f_v, seed_v, c_v, act_v, g_v, wp_v, t_v, u_v, xr_v, xi_v, v_v, p_v,
                 ts_v, e_v, h_v):
        def x_copy(i):
            cols = pl.ds(pl.multiple_of(i * (S // XCH), S // XCH), S // XCH)
            return pltpu.make_async_copy(x_hbm.at[:, cols], x_v.at[:, cols], sem_x.at[i])

        seed_copy, c_copy, f_copy, wr_copy, wi_copy = [
            pltpu.make_async_copy(src, dst, sem_in.at[2 + i]) for i, (src, dst) in enumerate(
                ((seed_hbm, seed_v), (c_hbm, c_v), (f_hbm, f_v), (wr_hbm, wr_v), (wi_hbm, wi_v)))]
        mod_cols = ((512, 2 * D), (0, 512), (2 * D, 6 * D))
        wm_copies = [pltpu.make_async_copy(wm_hbm.at[:, lo:hi], wm_v.at[:, lo:hi], sem_in.at[7 + i])
                     for i, (lo, hi) in enumerate(mod_cols)]

        start([seed_copy, c_copy, wm_copies[0], x_copy(0)])
        for i in range(7):
            zero_s[i] = 0

        lane = lax.broadcasted_iota(i32, (8, 128), 1)
        with _scope("twiddle"):
            seed_copy.wait()
            x_copy(1).start()
            seeds = [(seed_v[16 * i:16 * i + 8, :], seed_v[16 * i + 8:16 * i + 16, :]) for i in range(9)]
            for half in range(2):
                first, step, wrap = seeds[3 * half:3 * half + 3]
                for i in range(8):
                    rows = slice(16 * i + 8 * half, 16 * i + 8 * half + 8)
                    g = first
                    for k1 in range(NT):
                        g_v[k1, 0, rows, :], g_v[k1, 1, rows, :], g_v[k1, 2, rows, :] = g[0], g[1] - g[0], g[1] + g[0]
                        if k1 + 1 < NT:
                            at = (lane & 15) == k1
                            g = _cmul(g, (jnp.where(at, wrap[0], step[0]), jnp.where(at, wrap[1], step[1])))
                    if i < 7:
                        first, step, wrap = [_cmul(z, w) for z, w in zip((first, step, wrap), seeds[6:])]

        def modulation(part):
            lo, hi = mod_cols[part]
            row = _dot(act_v[...], wm_v[:, lo:hi])
            for t in range(0, hi - lo, 128):
                mod_v[lo + t:lo + t + 128, :] = jnp.broadcast_to(row[0:1, t:t + 128], (128, 128)).T

        with _scope("mod0"):
            c_copy.wait()
            x_copy(2).start()
            cond = c_v[...].astype(f32)
            act_v[...] = jnp.broadcast_to(cond * jax.nn.sigmoid(cond), (8, D))
            wm_copies[0].wait()
            x_copy(3).start()
            modulation(0)
            mod_v[D:2 * D, :] = 1.0 + mod_v[D:2 * D, :]

        def radix9_forward(dst, cols, piece):
            for i in range(0, 64, 16):
                h = [piece(64 * a + i) for a in range(9)]
                even = _radix9_even(h[0], *[h[a] + h[9 - a] for a in range(1, 5)])
                odd = _radix9_odd(*[h[a] - h[9 - a] for a in range(1, 5)])
                dst[512 + i:512 + i + 16, cols] = even[0]
                for r in range(4):
                    dst[128 * r + i:128 * r + i + 16, cols] = even[r + 1]
                    dst[128 * r + 64 + i:128 * r + 64 + i + 16, cols] = odd[r]

        def first_norm(i, _):
            x_copy(i).wait()
            pl.when(i + 4 < XCH)(lambda: x_copy(i + 4).start())
            for n, copy in enumerate((f_copy, wr_copy, wi_copy, wm_copies[1])):
                pl.when(i == XCH - 4 + n)(copy.start)
            tiles = range(NT // XCH)
            cols = [pl.ds(pl.multiple_of((i * len(tiles) + n) * 128, 128), 128) for n in tiles]
            mean, var = [_Mean() for _ in tiles], [_Mean() for _ in tiles]
            for n in tiles:
                for row in range(0, D, 16):
                    mean[n].add(x_v[row:row + 16, cols[n]].astype(f32))
            for n in tiles:
                m = mean[n].value()
                for row in range(0, D, 16):
                    d = x_v[row:row + 16, cols[n]].astype(f32) - m
                    e_v[n, row:row + 16, :] = d
                    var[n].add(d * d)
            for n in tiles:
                scale = lax.rsqrt(var[n].value() + EPS)
                radix9_forward(t_v, cols[n], lambda row: e_v[n, row:row + 16, :] * scale * mod_col(1, row))
            return 0

        with _scope("first_norm"):
            lax.fori_loop(0, XCH, first_norm, 0)

        def d_forward(r, rhs):
            if r < 4:
                return _dot(_as_bf16(f_v[r]), rhs(slice(128 * r, 128 * r + 128)).astype(bf16))
            return _dot(_as_bf16(f_v[4, 0:G0, 0:64]), rhs(slice(512, D)).astype(bf16))

        def group_rows(r):
            return range(0, 64 if r < 4 else G0, 8)

        with _scope("dfwd"):
            f_copy.wait()
            start([wm_copies[2]] + bias_copies)
            for r in range(5):
                for a1 in range(4):
                    z = d_forward(r, lambda rows: jnp.concatenate(
                        [t_v[rows, 128 * a:128 * a + 128] for a in range(a1, NT, 4)], axis=1))
                    for i in group_rows(r):
                        u = _radix4(*[(z[2 * i:2 * i + 8, t:t + 128], z[2 * i + 8:2 * i + 16, t:t + 128])
                                      for t in range(0, 512, 128)], -1)
                        rows = slice(64 * r + i, 64 * r + i + 8)
                        for q1 in range(4):
                            u_v[a1, q1, 0, rows, :], u_v[a1, q1, 1, rows, :] = _twiddle16(u[q1], a1 * q1, -1)

        def s_forward(q1):
            y = _radix4(*[(u_v[a1, q1, 0], u_v[a1, q1, 1]) for a1 in range(4)], -1)
            for q2, (yr, yi) in enumerate(y):
                k1 = q1 + 4 * q2
                both, real, imag = [_dot(v, g_v[k1, n].astype(bf16)) for n, v in enumerate((yr + yi, yr, yi))]
                xr_v[k1], xi_v[k1] = both - imag, both + real

        def regroup(tiles, row):
            a = [None] * NT
            for c in range(NT):
                a[-c % NT] = pltpu.roll(tiles[c], c, 1) if c else tiles[c]
            for bit in range(4):
                take = ((lane >> bit) & 1) == 1
                a = [jnp.where(take, a[(m - (1 << bit)) % NT], a[m]) for m in range(NT)]
            for k1 in range(NT):
                wp_v[k1, row:row + 8, :] = a[k1]

        with _scope("sfwd_a"):
            s_forward(0)
            s_forward(1)
        with _scope("sfwd_b"):
            wait([wr_copy, wi_copy])
            start(w1_copies(0))
            for i in range(18):
                for src, base in ((wr_v, 0), (wi_v, 144)):
                    regroup([pltpu.bitcast(src[16 * i:16 * i + 16, t:t + 128], i32) for t in range(0, S, 128)],
                            base + 8 * i)
            last = []
            for t in range(0, S, 128):
                low, high = [pltpu.bitcast(jnp.broadcast_to(w[DF - 1:DF, t:t + 128].astype(f32), (8, 128)), i32)
                             for w in (wr_v, wi_v)]
                last.append(lax.shift_right_logical(low, 16) | high)
            regroup(last, 288)
            s_forward(2)
            s_forward(3)

        def s_inverse(q1, shift=None):
            q = []
            for k1 in range(q1, NT, 4):
                wr, wi = [jnp.concatenate(
                    [_word_half(wp_v[k1, pl.ds(base + res // 2, 16, stride=9), :], res % 2)
                     for r in (1, 2, 3, 4, 0) for res in _classes(r)] + [_word_half(wp_v[k1, 288:296, :], base)],
                    axis=0) for base in (0, 144)]
                xr, xi = xr_v[k1], xi_v[k1]
                if k1 == 0:
                    xr, xi = xr + shift[0], xi + shift[1]
                fr, fi = _cmul((xr, xi), (wr, wi))
                both, imag, real = [_dot_nt(v, g_v[k1, n].astype(bf16)) for n, v in enumerate((fr + fi, fi, fr))]
                q.append((both + imag, both - real))
            for a1, u in enumerate(_radix4(*q, +1)):
                v_v[a1, q1, 0], v_v[a1, q1, 1] = _twiddle16(u, a1 * q1, +1)

        with _scope("sinv"):
            wm_copies[1].wait()
            start(w1_copies(1))
            modulation(1)
            s_inverse(3)
            radix9_forward(ts_v, slice(None), lambda row: mod_col(0, row))
            shift = ([], [])
            for r in range(5):
                z = d_forward(r, lambda rows: ts_v[rows, :])
                for i in group_rows(r):
                    for part in range(2):
                        row = 2 * i + 8 * part
                        shift[part].append(jnp.where(lane == 0, z[row:row + 8] * float(S), 0.0))
            s_inverse(2)
            s_inverse(1)
            s_inverse(0, [jnp.concatenate(part, axis=0) for part in shift])

        with _scope("dinv"):
            wm_copies[2].wait()
            start(w1_copies(2))
            modulation(2)
            for r in range(5):
                rows = slice(64 * r, 64 * r + 64 if r < 4 else NL)
                for a1 in range(4):
                    v = _radix4(*[(v_v[a1, q1, 0, rows, :], v_v[a1, q1, 1, rows, :]) for q1 in range(4)], +1)
                    rhs = jnp.concatenate([jnp.concatenate(pair, axis=0) for pair in v], axis=1).astype(bf16)
                    p = _dot(_as_bf16(f_v[5 + r] if r < 4 else f_v[9, 0:32, 0:2 * G0]), rhs)
                    for a2 in range(4):
                        p_v[a1 + 4 * a2, 128 * r:128 * r + p.shape[0], :] = p[:, 128 * a2:128 * a2 + 128]
            mod_v[4 * D:5 * D, :] = 1.0 + mod_v[4 * D:5 * D, :]
            shifts, mean = [mod_col(3, row) for row in range(0, D, 16)], _Mean()
            for piece in shifts:
                mean.add(piece)
            mean = mean.value()
            for i, piece in enumerate(shifts):
                mod_v[3 * D + 16 * i:3 * D + 16 * i + 16, :] = piece - mean

        def residual(t):
            cols = pl.ds(pl.multiple_of(t * 128, 128), 128)
            mean = _Mean()
            for i in range(0, 64, 16):
                even = _radix9_even(*[p_v[t, row + i:row + i + 16, :] for row in (512, 0, 128, 256, 384)])
                odd = _radix9_odd(*[p_v[t, row + i:row + i + 16, :] for row in (64, 192, 320, 448)])
                for a in range(9):
                    y = even[0] if a == 0 else even[a] - odd[a - 1] if a < 5 else even[9 - a] + odd[8 - a]
                    row = 64 * a + i
                    x1 = x_v[row:row + 16, cols].astype(f32) + mod_col(2, row) * y
                    x1_v[t, row:row + 16, :] = x1
                    mean.add(x1)
            return mean

        def second_norm(t, slot, m):
            var, mean = _Mean(), _Mean()
            for row in range(0, D, 16):
                d = x1_v[t, row:row + 16, :] - m
                e = d * mod_col(4, row)
                e_v[slot, row:row + 16, :] = e
                var.add(d * d)
                mean.add(e)
            return var, mean

        def third_norm(slot, scale, m):
            var = _Mean()
            for row in range(0, D, 16):
                d = (e_v[slot, row:row + 16, :] - m) * scale + mod_col(3, row)
                h_v[slot, row:row + 16, :] = d
                var.add(d * d)
            return var

        def mlp_operands(t, _):
            scales = []
            for slots in ((0, 1), (2, 3)):
                means = [residual(4 * t + k) for k in slots]
                stats = [second_norm(4 * t + k, k, m.value()) for k, m in zip(slots, means)]
                spread = [third_norm(k, lax.rsqrt(v.value() + EPS), m.value()) for k, (v, m) in zip(slots, stats)]
                scales += [lax.rsqrt(v.value() + EPS) for v in spread]
            cols = pl.ds(pl.multiple_of(t * 256, 256), 256)
            for i in range(0, Q, 16):
                inner = {(r, c): _left_operands({
                    (r2, c2): h_v[2 * c + c2, (2 * r + r2) * Q + i:(2 * r + r2) * Q + i + 16, :] * scales[2 * c + c2]
                    for r2, c2 in _QUADS}) for r, c in _QUADS}
                for n, pair in enumerate(_PAIRS):
                    a1_v[n, i:i + 16, cols] = _paired(pair, inner)
            return 0

        with _scope("norms"):
            start(w1_copies(3))
            lax.fori_loop(0, NT // 4, mlp_operands, 0)

    def mlp(a2_v, out_v, b1_f, b2_f):
        def weight_block(ref, tile, kq, p):
            words = ref.bitcast(i32)
            return _as_bf16(jnp.concatenate(
                [words[tile + zero_s[p], row + 64 * kq:row + 64 * kq + 64, :]
                 for row in range(0, words.shape[1], 256)], axis=0))

        def up(j):
            cols = pl.ds(pl.multiple_of(j * 256, 256), 256)
            inner, todo = {}, list(enumerate(_PAIRS))
            for r, c, u in _strassen2(a1_v, lambda kq, nq, p: weight_block(w1_v, 4 * j + nq, kq, p), ORDER_UP):
                inner[r, 1 - c] = _left_operands({
                    (r2, 1 - c2): _gelu2(u[r2, c2] + b1_f[pl.ds(4 * j + 2 * c + c2, 1), :]) for r2, c2 in _QUADS})
                for n, pair in list(todo):
                    if all(rc in inner for p, _ in pair for rc, _ in _LEFT[p]):
                        todo.remove((n, pair))
                        a2_v[n, :, cols] = _paired(pair, inner)

        def up_chunks(step, _):
            @pl.when(step == 1)
            def _():
                for j in range(NDOWN):
                    start(w2_copies(j))

            for n in range(UP_UNROLL):
                wait(w1_copies(step * UP_UNROLL + n))
            for n in range(UP_UNROLL):
                up(step * UP_UNROLL + n)
            return 0

        def out_copy(j, r, c):
            cols = pl.ds(pl.multiple_of(j * 512 + c * 256, 256), 256)
            return pltpu.make_async_copy(out_v.at[j, r, c], out_hbm.at[pl.ds(r * H, H), cols],
                                         sem_out.at[4 * j + 2 * r + c])

        def down(j, _):
            wait(w2_copies(j))
            for r, c, y in _strassen2(a2_v, lambda kq, nq, p: weight_block(w2_v, 4 * j + nq, 3 - kq, p), ORDER_DOWN):
                for r2 in range(2):
                    row = (2 * r + r2) * Q
                    tiles = []
                    for c2 in range(2):
                        tile = 4 * j + 2 * c + c2
                        mixed = 0.5 * y[r2, c2] + b2_f[pl.ds(tile, 1), :]
                        tiles.append(x1_v[tile, row:row + Q, :] + mod_col(5, row, Q) * mixed)
                    out_v[j, r, c, r2 * Q:(r2 + 1) * Q, :] = jnp.concatenate(tiles, axis=1).astype(bf16)
                out_copy(j, r, c).start()
            return 0

        for j in range(4, NUP):
            start(w1_copies(j))
        wait(bias_copies)
        b1_f[...] = b1_v[...].astype(f32)
        b2_f[...] = b2_v[...].astype(f32)
        with _scope("up"):
            lax.fori_loop(0, NUP // UP_UNROLL, up_chunks, 0)
        with _scope("down"):
            lax.fori_loop(0, NDOWN, down, 0)
        with _scope("out"):
            wait([out_copy(j, r, c) for j in range(NDOWN) for r, c in _QUADS])

    vmem = pltpu.VMEM
    pl.run_scoped(
        spectral,
        vmem((D, S), bf16), vmem((DF, S), bf16), vmem((DF, S), bf16), vmem((D, 6 * D), bf16),
        vmem(_DFT64.shape, i32), vmem(_SEEDS.shape, f32), vmem((1, D), bf16), vmem((8, D), f32),
        vmem((NT, 3, 128, 128), f32), vmem((NT, WROWS, 128), i32), vmem((D, S), f32),
        vmem((4, 4, 2, NL, 128), f32), vmem((NT, NL, 128), f32), vmem((NT, NL, 128), f32),
        vmem((4, 4, 2, NL, 128), f32), vmem((NT, D, 128), f32),
        vmem((D, 128), f32), vmem((4, D, 128), f32), vmem((4, D, 128), f32))
    pl.run_scoped(
        mlp,
        vmem((len(_PAIRS), Q, 256 * NUP), bf16), vmem((NDOWN, 2, 2, H, 256), bf16),
        vmem((F // 128, 128), f32), vmem((NT, 128), f32))


@jax.jit
def pallas_adaLN_cond__spectral_gfnet__mixer_token_mlp__prompt_kernel(A_x, A_w_r, A_w_i, B_x, B_w1, B_b1, B_w2, B_b2, c, w_mod):
    del B_x
    bf16 = jnp.bfloat16
    hbm = pl.BlockSpec(memory_space=pl.ANY)
    out = pl.pallas_call(
        _kernel,
        out_shape=jax.ShapeDtypeStruct((D, S), bf16),
        in_specs=[hbm] * 11,
        out_specs=hbm,
        scratch_shapes=[
            pltpu.VMEM((F // 128, S, 128), bf16),
            pltpu.VMEM((NT, F, 128), bf16),
            pltpu.VMEM((F // 128, 128), bf16),
            pltpu.VMEM((NT, 128), bf16),
            pltpu.VMEM((6 * D, 128), jnp.float32),
            pltpu.VMEM((NT, D, 128), jnp.float32),
            pltpu.VMEM((len(_PAIRS), Q, 256 * NDOWN), bf16),
            pltpu.SMEM((7,), jnp.int32),
            pltpu.SemaphoreType.DMA((10,)),
            pltpu.SemaphoreType.DMA((XCH,)),
            pltpu.SemaphoreType.DMA((NUP,)),
            pltpu.SemaphoreType.DMA((NDOWN,)),
            pltpu.SemaphoreType.DMA((4 * NDOWN,)),
        ],
        compiler_params=pltpu.CompilerParams(vmem_limit_bytes=120 * 1024 * 1024),
    )(A_x.reshape(S, D).T, A_w_r.T, A_w_i.T, B_w1, B_w2, w_mod, _DFT64, _SEEDS,
      B_b1.reshape(F // 128, 128), B_b2.reshape(NT, 128), c)
    return out.T.reshape(1, S, D)
```

```python
import contextlib
import math

import jax
import jax.numpy as jnp
import numpy as np
from jax import lax
import jax.experimental.pallas as pl
import jax.experimental.pallas.tpu as pltpu

S, D, F = 2048, 576, 4608
DF = D // 2 + 1
EPS = 1e-5
NT = S // 128
G0 = 40
NL = 4 * 64 + G0
WROWS = 296
H, Q = D // 2, D // 4
XCH = 8
NUP, NDOWN = F // 512, S // 512
UP_UNROLL = 3
SCOPES = False

_C9 = [math.cos(2 * math.pi * j / 9) for j in range(9)]
_S9 = [math.sin(2 * math.pi * j / 9) for j in range(9)]


def _scope(name):
    return jax.named_scope(name) if SCOPES else contextlib.nullcontext()


def _classes(r):
    return [r, r + 9, 9 - r, 18 - r] if r else [0, 9]


def _bf16_pairs(m):
    u = np.ascontiguousarray(m, dtype=np.float32).view(np.uint32)
    u = (u + 0x7FFF + ((u >> 16) & 1)) >> 16
    return (u[..., 0::2, :] | (u[..., 1::2, :] << 16)).view(np.int32)


def _constants():
    def by8(re, im):
        n = re.shape[1]
        return np.stack([re.reshape(-1, 8, n), im.reshape(-1, 8, n)], 1).reshape(-1, n)

    d = np.arange(64)
    fwd, inv = np.zeros((5, 128, 128)), np.zeros((5, 128, 128))
    scale = 1.0 / (D * S)
    for r in range(1, 5):
        l = np.array([18 * m + res for res in _classes(r) for m in range(16)])
        angle = 2 * np.pi * np.outer(l, d) / D
        co, si = np.cos(angle), np.sin(angle)
        odd = _S9[3] * np.where(l % 9 == r, 1.0, -1.0)[:, None]
        fwd[r - 1] = by8(np.hstack([co, -odd * si]), np.hstack([-si, -odd * co]))
        inv[r - 1] = 2 * scale * np.block([[co.T, -si.T], [(odd * si).T, (odd * co).T]])
    l = np.array([18 * m + res for res in _classes(0) for m in range(16)] + [D // 2])
    angle = 2 * np.pi * np.outer(l, d) / D
    edge = (l == 0) | (l == D // 2)
    pad = ((0, G0 - len(l)), (0, 0))
    co, si = np.pad(np.cos(angle), pad), np.pad(np.where(edge[:, None], 0.0, np.sin(angle)), pad)
    fwd[4, :2 * G0, :64] = by8(co, -si)
    weight = scale * np.pad(np.where(edge, 1.0, 2.0), pad[0])[None, :]
    inv[4, :64, :2 * G0] = np.hstack([weight * co.T, -weight * si.T])

    b, p = np.arange(8)[:, None], np.arange(128)[None, :]
    first = 128 * (p % 16) + 16 * (p // 16)
    step = -127 + 0 * p
    wrap = step + np.where(p < 16, 112, -16)
    seeds = []
    for rows in (b, b + 8, 16 + 0 * b):
        for k in (first, step, wrap):
            z = np.exp(-2j * np.pi * rows * k / S)
            seeds += [z.real, z.imag]
    return _bf16_pairs(np.concatenate([fwd, inv], 0)), np.concatenate(seeds, 0).astype(np.float32)


_DFT64, _SEEDS = _constants()


def _radix9_even(h0, e1, e2, e3, e4):
    p = h0 + e3
    q = e1 + e2 + e4
    g = h0 - 0.5 * e3
    u, v = e1 - e4, e2 - e4
    a = _C9[1] * u + _C9[2] * v
    b = _C9[2] * u + _C9[4] * v
    return p + q, g + a, g + b, p - 0.5 * q, g - a - b


def _radix9_odd(o1, o2, o3, o4):
    u, v = o1 + o2, o2 + o4
    a = (_S9[1] / _S9[3]) * u + (_S9[4] / _S9[3]) * v
    b = (_S9[2] / _S9[3]) * u - (_S9[1] / _S9[3]) * v
    return a + o3, b - o3, o1 - o2 + o4, b - a + o3


def _radix4(z0, z1, z2, z3, sign):
    ar, ai = z0[0] + z2[0], z0[1] + z2[1]
    br, bi = z0[0] - z2[0], z0[1] - z2[1]
    cr, ci = z1[0] + z3[0], z1[1] + z3[1]
    dr, di = z1[0] - z3[0], z1[1] - z3[1]
    plus, minus = (br - di, bi + dr), (br + di, bi - dr)
    if sign < 0:
        plus, minus = minus, plus
    return (ar + cr, ai + ci), plus, (ar - cr, ai - ci), minus


def _twiddle16(z, n, sign):
    zr, zi = z
    if n == 0:
        return z
    if n == 4:
        return (-zi, zr) if sign > 0 else (zi, -zr)
    c, s = math.cos(2 * math.pi * n / 16), sign * math.sin(2 * math.pi * n / 16)
    if n % 4 == 2:
        if (c > 0) == (s > 0):
            return c * (zr - zi), c * (zr + zi)
        return c * (zr + zi), c * (zi - zr)
    return c * zr - s * zi, c * zi + s * zr


def _cmul(a, b):
    return a[0] * b[0] - a[1] * b[1], a[0] * b[1] + a[1] * b[0]


def _gelu2(x):
    k = math.sqrt(2 / math.pi)
    return x + x * jnp.tanh(x * (k + (k * 0.044715) * (x * x)))


class _Mean:
    def __init__(self):
        self.total = None

    def add(self, piece):
        self.total = piece if self.total is None else self.total + piece

    def value(self):
        return jnp.sum(self.total[0:8] + self.total[8:16], axis=0, keepdims=True) * (1.0 / D)


def _as_bf16(words):
    return pltpu.bitcast(words, jnp.bfloat16)


def _word_half(words, high):
    return pltpu.bitcast(words & jnp.int32(-65536) if high else words << 16, jnp.float32)


def _dot(a, b):
    return jnp.dot(a, b, preferred_element_type=jnp.float32)


def _dot_nt(a, b):
    return lax.dot_general(a, b, (((1,), (1,)), ((), ())), preferred_element_type=jnp.float32)


_QUADS = ((0, 0), (0, 1), (1, 0), (1, 1))
_LEFT = ((((0, 0), 1), ((1, 1), 1)), (((1, 0), 1), ((1, 1), 1)), (((0, 0), 1),), (((1, 1), 1),),
         (((0, 0), 1), ((0, 1), 1)), (((1, 0), 1), ((0, 0), -1)), (((0, 1), 1), ((1, 1), -1)))
_RIGHT = ((((0, 0), 1), ((1, 1), 1)), (((0, 0), 1),), (((0, 1), 1), ((1, 1), -1)), (((1, 0), 1), ((0, 0), -1)),
          (((1, 1), 1),), (((0, 0), 1), ((0, 1), 1)), (((1, 0), 1), ((1, 1), 1)))
_OUTPUT = (((0, 0), ((0, 1), (3, 1), (4, -1), (6, 1))), ((0, 1), ((2, 1), (4, 1))),
           ((1, 0), ((1, 1), (3, 1))), ((1, 1), ((0, 1), (1, -1), (2, 1), (5, 1))))
ORDER_UP = (4, 2, 1, 3, 0, 6, 5)
ORDER_DOWN = (2, 4, 1, 3, 0, 6, 5)
ORDER_IN = (4, 1, 2, 3, 0, 6, 5)
_PAIRS = ([((2, q), (2, min(q + 1, 6))) for q in range(0, 7, 2)] +
          [((a, q), (b, q)) for a, b in ((3, 0), (4, 6), (1, 5)) for q in range(7)])
_PLACE = {op: (n, side) for n, pair in enumerate(_PAIRS) for side, op in ((1, pair[1]), (0, pair[0]))}


def _signed_sum(terms, get):
    total = get(terms[0][0])
    for key, sign in terms[1:]:
        total = total + get(key) if sign > 0 else total - get(key)
    return total


def _left_operands(blocks):
    return [_signed_sum(terms, blocks.get) for terms in _LEFT]


def _paired(pair, inner):
    return jnp.concatenate(
        [_signed_sum(_LEFT[p], lambda rc: inner[rc][q]) for p, q in pair], axis=1).astype(jnp.bfloat16)


def _strassen_level(product, order):
    done = {}
    for n in order:
        done[n] = product(n)
        for (r, c), terms in _OUTPUT:
            if n in dict(terms) and all(k in done for k, _ in terms):
                yield r, c, lambda f, terms=terms: _signed_sum(terms, lambda k: f(done[k]))


def _strassen2(left_ref, right, order):
    def outer(p):
        def inner(q):
            def block(b, c):
                return right(2 * b[0] + c[0], 2 * b[1] + c[1], 7 * p + (q if len(_RIGHT[p]) == 1 else 0))

            if len(_RIGHT[p]) == 1 and len(_RIGHT[q]) == 1:
                rhs = block(_RIGHT[p][0][0], _RIGHT[q][0][0])
            else:
                rhs = _signed_sum(_RIGHT[q], lambda c: _signed_sum(
                    _RIGHT[p], lambda b: block(b, c).astype(jnp.float32))).astype(jnp.bfloat16)
            n, side = _PLACE[p, q]
            lhs = jnp.concatenate(
                [left_ref[n, :, k + 128 * side:k + 128 * (side + 1)] for k in range(0, left_ref.shape[2], 256)],
                axis=1)
            return _dot(lhs, rhs)

        return {(r, c): combine(lambda m: m) for r, c, combine in _strassen_level(inner, ORDER_IN)}

    for r, c, combine in _strassen_level(outer, order):
        yield r, c, {rc: combine(lambda m: m[rc]) for rc in _QUADS}


def _kernel(x_hbm, wr_hbm, wi_hbm, w1_hbm, w2_hbm, wm_hbm, f_hbm, seed_hbm, b1_hbm, b2_hbm, c_hbm,
            out_hbm,
            w1_v, w2_v, b1_v, b2_v, mod_v, x1_v, a1_v, zero_s, sem_in, sem_x, sem_w1, sem_w2, sem_out):
    f32, bf16, i32 = jnp.float32, jnp.bfloat16, jnp.int32

    def tile_copies(src, dst, sem, j):
        return [pltpu.make_async_copy(src.at[:, pl.ds(pl.multiple_of((4 * j + t) * 128, 128), 128)],
                                      dst.at[4 * j + t], sem.at[j]) for t in range(4)]

    def w1_copies(j):
        return tile_copies(w1_hbm, w1_v, sem_w1, j)

    def w2_copies(j):
        return tile_copies(w2_hbm, w2_v, sem_w2, j)

    def start(copies):
        for copy in copies:
            copy.start()

    def wait(copies):
        for copy in copies:
            copy.wait()

    bias_copies = [pltpu.make_async_copy(b1_hbm, b1_v, sem_in.at[0]),
                   pltpu.make_async_copy(b2_hbm, b2_v, sem_in.at[1])]

    def mod_col(which, row, n=16):
        return mod_v[which * D + row:which * D + row + n, :]

    def spectral(x_v, wr_v, wi_v, wm_v, f_v, seed_v, c_v, act_v, g_v, wp_v, t_v, u_v, xr_v, xi_v, v_v, p_v,
                 ts_v, e_v, h_v):
        def x_copy(i):
            cols = pl.ds(pl.multiple_of(i * (S // XCH), S // XCH), S // XCH)
            return pltpu.make_async_copy(x_hbm.at[:, cols], x_v.at[:, cols], sem_x.at[i])

        seed_copy, c_copy, f_copy, wr_copy, wi_copy = [
            pltpu.make_async_copy(src, dst, sem_in.at[2 + i]) for i, (src, dst) in enumerate(
                ((seed_hbm, seed_v), (c_hbm, c_v), (f_hbm, f_v), (wr_hbm, wr_v), (wi_hbm, wi_v)))]
        mod_cols = ((512, 2 * D), (0, 512), (2 * D, 6 * D))
        wm_copies = [pltpu.make_async_copy(wm_hbm.at[:, lo:hi], wm_v.at[:, lo:hi], sem_in.at[7 + i])
                     for i, (lo, hi) in enumerate(mod_cols)]

        start([seed_copy, c_copy, wm_copies[0], x_copy(0)])
        for i in range(49):
            zero_s[i] = 0

        lane = lax.broadcasted_iota(i32, (8, 128), 1)
        with _scope("twiddle"):
            seed_copy.wait()
            x_copy(1).start()
            seeds = [(seed_v[16 * i:16 * i + 8, :], seed_v[16 * i + 8:16 * i + 16, :]) for i in range(9)]
            for half in range(2):
                first, step, wrap = seeds[3 * half:3 * half + 3]
                for i in range(8):
                    rows = slice(16 * i + 8 * half, 16 * i + 8 * half + 8)
                    g = first
                    for k1 in range(NT):
                        g_v[k1, 0, rows, :], g_v[k1, 1, rows, :], g_v[k1, 2, rows, :] = g[0], g[1] - g[0], g[1] + g[0]
                        if k1 + 1 < NT:
                            at = (lane & 15) == k1
                            g = _cmul(g, (jnp.where(at, wrap[0], step[0]), jnp.where(at, wrap[1], step[1])))
                    if i < 7:
                        first, step, wrap = [_cmul(z, w) for z, w in zip((first, step, wrap), seeds[6:])]

        def modulation(part):
            lo, hi = mod_cols[part]
            row = _dot(act_v[...], wm_v[:, lo:hi])
            for t in range(0, hi - lo, 128):
                mod_v[lo + t:lo + t + 128, :] = jnp.broadcast_to(row[0:1, t:t + 128], (128, 128)).T

        with _scope("mod0"):
            c_copy.wait()
            x_copy(2).start()
            cond = c_v[...].astype(f32)
            act_v[...] = jnp.broadcast_to(cond * jax.nn.sigmoid(cond), (8, D))
            wm_copies[0].wait()
            x_copy(3).start()
            modulation(0)
            mod_v[D:2 * D, :] = 1.0 + mod_v[D:2 * D, :]

        def radix9_forward(dst, cols, piece):
            for i in range(0, 64, 16):
                h = [piece(64 * a + i) for a in range(9)]
                even = _radix9_even(h[0], *[h[a] + h[9 - a] for a in range(1, 5)])
                odd = _radix9_odd(*[h[a] - h[9 - a] for a in range(1, 5)])
                dst[512 + i:512 + i + 16, cols] = even[0]
                for r in range(4):
                    dst[128 * r + i:128 * r + i + 16, cols] = even[r + 1]
                    dst[128 * r + 64 + i:128 * r + 64 + i + 16, cols] = odd[r]

        def first_norm(i, _):
            x_copy(i).wait()
            pl.when(i + 4 < XCH)(lambda: x_copy(i + 4).start())
            for n, copy in enumerate((f_copy, wr_copy, wi_copy, wm_copies[1])):
                pl.when(i == XCH - 4 + n)(copy.start)
            tiles = range(NT // XCH)
            cols = [pl.ds(pl.multiple_of((i * len(tiles) + n) * 128, 128), 128) for n in tiles]
            mean, var = [_Mean() for _ in tiles], [_Mean() for _ in tiles]
            for n in tiles:
                for row in range(0, D, 16):
                    mean[n].add(x_v[row:row + 16, cols[n]].astype(f32))
            for n in tiles:
                m = mean[n].value()
                for row in range(0, D, 16):
                    d = x_v[row:row + 16, cols[n]].astype(f32) - m
                    e_v[n, row:row + 16, :] = d
                    var[n].add(d * d)
            for n in tiles:
                scale = lax.rsqrt(var[n].value() + EPS)
                radix9_forward(t_v, cols[n], lambda row: e_v[n, row:row + 16, :] * scale * mod_col(1, row))
            return 0

        with _scope("first_norm"):
            lax.fori_loop(0, XCH, first_norm, 0)

        def d_forward(r, rhs):
            if r < 4:
                return _dot(_as_bf16(f_v[r]), rhs(slice(128 * r, 128 * r + 128)).astype(bf16))
            return _dot(_as_bf16(f_v[4, 0:G0, 0:64]), rhs(slice(512, D)).astype(bf16))

        def group_rows(r):
            return range(0, 64 if r < 4 else G0, 8)

        with _scope("dfwd"):
            f_copy.wait()
            start([wm_copies[2]] + bias_copies)
            for r in range(5):
                for a1 in range(4):
                    z = d_forward(r, lambda rows: jnp.concatenate(
                        [t_v[rows, 128 * a:128 * a + 128] for a in range(a1, NT, 4)], axis=1))
                    for i in group_rows(r):
                        u = _radix4(*[(z[2 * i:2 * i + 8, t:t + 128], z[2 * i + 8:2 * i + 16, t:t + 128])
                                      for t in range(0, 512, 128)], -1)
                        rows = slice(64 * r + i, 64 * r + i + 8)
                        for q1 in range(4):
                            u_v[a1, q1, 0, rows, :], u_v[a1, q1, 1, rows, :] = _twiddle16(u[q1], a1 * q1, -1)

        def s_forward(q1):
            y = _radix4(*[(u_v[a1, q1, 0], u_v[a1, q1, 1]) for a1 in range(4)], -1)
            for q2, (yr, yi) in enumerate(y):
                k1 = q1 + 4 * q2
                both, real, imag = [_dot(v, g_v[k1, n].astype(bf16)) for n, v in enumerate((yr + yi, yr, yi))]
                xr_v[k1], xi_v[k1] = both - imag, both + real

        def regroup(tiles, row):
            a = [None] * NT
            for c in range(NT):
                a[-c % NT] = pltpu.roll(tiles[c], c, 1) if c else tiles[c]
            for bit in range(4):
                take = ((lane >> bit) & 1) == 1
                a = [jnp.where(take, a[(m - (1 << bit)) % NT], a[m]) for m in range(NT)]
            for k1 in range(NT):
                wp_v[k1, row:row + 8, :] = a[k1]

        with _scope("sfwd_a"):
            s_forward(0)
            s_forward(1)
        with _scope("sfwd_b"):
            wait([wr_copy, wi_copy])
            start(w1_copies(0))
            for i in range(18):
                for src, base in ((wr_v, 0), (wi_v, 144)):
                    regroup([pltpu.bitcast(src[16 * i:16 * i + 16, t:t + 128], i32) for t in range(0, S, 128)],
                            base + 8 * i)
            last = []
            for t in range(0, S, 128):
                low, high = [pltpu.bitcast(jnp.broadcast_to(w[DF - 1:DF, t:t + 128].astype(f32), (8, 128)), i32)
                             for w in (wr_v, wi_v)]
                last.append(lax.shift_right_logical(low, 16) | high)
            regroup(last, 288)
            s_forward(2)
            s_forward(3)

        def s_inverse(q1, shift=None):
            q = []
            for k1 in range(q1, NT, 4):
                wr, wi = [jnp.concatenate(
                    [_word_half(wp_v[k1, pl.ds(base + res // 2, 16, stride=9), :], res % 2)
                     for r in (1, 2, 3, 4, 0) for res in _classes(r)] + [_word_half(wp_v[k1, 288:296, :], base)],
                    axis=0) for base in (0, 144)]
                xr, xi = xr_v[k1], xi_v[k1]
                if k1 == 0:
                    xr, xi = xr + shift[0], xi + shift[1]
                fr, fi = _cmul((xr, xi), (wr, wi))
                both, imag, real = [_dot_nt(v, g_v[k1, n].astype(bf16)) for n, v in enumerate((fr + fi, fi, fr))]
                q.append((both + imag, both - real))
            for a1, u in enumerate(_radix4(*q, +1)):
                v_v[a1, q1, 0], v_v[a1, q1, 1] = _twiddle16(u, a1 * q1, +1)

        with _scope("sinv"):
            wm_copies[1].wait()
            start(w1_copies(1))
            modulation(1)
            s_inverse(3)
            radix9_forward(ts_v, slice(None), lambda row: mod_col(0, row))
            shift = ([], [])
            for r in range(5):
                z = d_forward(r, lambda rows: ts_v[rows, :])
                for i in group_rows(r):
                    for part in range(2):
                        row = 2 * i + 8 * part
                        shift[part].append(jnp.where(lane == 0, z[row:row + 8] * float(S), 0.0))
            s_inverse(2)
            s_inverse(1)
            s_inverse(0, [jnp.concatenate(part, axis=0) for part in shift])

        with _scope("dinv"):
            wm_copies[2].wait()
            start(w1_copies(2))
            modulation(2)
            for r in range(5):
                rows = slice(64 * r, 64 * r + 64 if r < 4 else NL)
                for a1 in range(4):
                    v = _radix4(*[(v_v[a1, q1, 0, rows, :], v_v[a1, q1, 1, rows, :]) for q1 in range(4)], +1)
                    rhs = jnp.concatenate([jnp.concatenate(pair, axis=0) for pair in v], axis=1).astype(bf16)
                    p = _dot(_as_bf16(f_v[5 + r] if r < 4 else f_v[9, 0:32, 0:2 * G0]), rhs)
                    for a2 in range(4):
                        p_v[a1 + 4 * a2, 128 * r:128 * r + p.shape[0], :] = p[:, 128 * a2:128 * a2 + 128]
            mod_v[4 * D:5 * D, :] = 1.0 + mod_v[4 * D:5 * D, :]
            shifts, mean = [mod_col(3, row) for row in range(0, D, 16)], _Mean()
            for piece in shifts:
                mean.add(piece)
            mean = mean.value()
            for i, piece in enumerate(shifts):
                mod_v[3 * D + 16 * i:3 * D + 16 * i + 16, :] = piece - mean

        def residual(t):
            cols = pl.ds(pl.multiple_of(t * 128, 128), 128)
            mean = _Mean()
            for i in range(0, 64, 16):
                even = _radix9_even(*[p_v[t, row + i:row + i + 16, :] for row in (512, 0, 128, 256, 384)])
                odd = _radix9_odd(*[p_v[t, row + i:row + i + 16, :] for row in (64, 192, 320, 448)])
                for a in range(9):
                    y = even[0] if a == 0 else even[a] - odd[a - 1] if a < 5 else even[9 - a] + odd[8 - a]
                    row = 64 * a + i
                    x1 = x_v[row:row + 16, cols].astype(f32) + mod_col(2, row) * y
                    x1_v[t, row:row + 16, :] = x1
                    mean.add(x1)
            return mean

        def second_norm(t, slot, m):
            var, mean = _Mean(), _Mean()
            for row in range(0, D, 16):
                d = x1_v[t, row:row + 16, :] - m
                e = d * mod_col(4, row)
                e_v[slot, row:row + 16, :] = e
                var.add(d * d)
                mean.add(e)
            return var, mean

        def third_norm(slot, scale, m):
            var = _Mean()
            for row in range(0, D, 16):
                d = (e_v[slot, row:row + 16, :] - m) * scale + mod_col(3, row)
                h_v[slot, row:row + 16, :] = d
                var.add(d * d)
            return var

        def mlp_operands(t, _):
            scales = []
            for slots in ((0, 1), (2, 3)):
                means = [residual(4 * t + k) for k in slots]
                stats = [second_norm(4 * t + k, k, m.value()) for k, m in zip(slots, means)]
                spread = [third_norm(k, lax.rsqrt(v.value() + EPS), m.value()) for k, (v, m) in zip(slots, stats)]
                scales += [lax.rsqrt(v.value() + EPS) for v in spread]
            cols = pl.ds(pl.multiple_of(t * 256, 256), 256)
            for i in range(0, Q, 16):
                inner = {(r, c): _left_operands({
                    (r2, c2): h_v[2 * c + c2, (2 * r + r2) * Q + i:(2 * r + r2) * Q + i + 16, :] * scales[2 * c + c2]
                    for r2, c2 in _QUADS}) for r, c in _QUADS}
                for n, pair in enumerate(_PAIRS):
                    a1_v[n, i:i + 16, cols] = _paired(pair, inner)
            return 0

        with _scope("norms"):
            start(w1_copies(3))
            lax.fori_loop(0, NT // 4, mlp_operands, 0)

    def mlp(a2_v, out_v, b1_f, b2_f):
        def weight_block(ref, tile, kq, tag):
            words = ref.bitcast(i32)
            return _as_bf16(jnp.concatenate(
                [words[tile + zero_s[tag], row + 64 * kq:row + 64 * kq + 64, :]
                 for row in range(0, words.shape[1], 256)], axis=0))

        def up(j):
            cols = pl.ds(pl.multiple_of(j * 256, 256), 256)
            inner, todo = {}, list(enumerate(_PAIRS))
            for r, c, u in _strassen2(a1_v, lambda kq, nq, tag: weight_block(w1_v, 4 * j + nq, kq, tag), ORDER_UP):
                inner[r, 1 - c] = _left_operands({
                    (r2, 1 - c2): _gelu2(u[r2, c2] + b1_f[pl.ds(4 * j + 2 * c + c2, 1), :]) for r2, c2 in _QUADS})
                for n, pair in list(todo):
                    if all(rc in inner for p, _ in pair for rc, _ in _LEFT[p]):
                        todo.remove((n, pair))
                        a2_v[n, :, cols] = _paired(pair, inner)

        def up_chunks(step, _):
            @pl.when(step == 1)
            def _():
                for j in range(NDOWN):
                    start(w2_copies(j))

            for n in range(UP_UNROLL):
                wait(w1_copies(step * UP_UNROLL + n))
            for n in range(UP_UNROLL):
                up(step * UP_UNROLL + n)
            return 0

        def out_copy(j, r, c):
            cols = pl.ds(pl.multiple_of(j * 512 + c * 256, 256), 256)
            return pltpu.make_async_copy(out_v.at[j, r, c], out_hbm.at[pl.ds(r * H, H), cols],
                                         sem_out.at[4 * j + 2 * r + c])

        def down(j, _):
            wait(w2_copies(j))
            for r, c, y in _strassen2(
                    a2_v, lambda kq, nq, tag: weight_block(w2_v, 4 * j + nq, 3 - kq, tag), ORDER_DOWN):
                for r2 in range(2):
                    row = (2 * r + r2) * Q
                    tiles = []
                    for c2 in range(2):
                        tile = 4 * j + 2 * c + c2
                        mixed = 0.5 * y[r2, c2] + b2_f[pl.ds(tile, 1), :]
                        tiles.append(x1_v[tile, row:row + Q, :] + mod_col(5, row, Q) * mixed)
                    out_v[j, r, c, r2 * Q:(r2 + 1) * Q, :] = jnp.concatenate(tiles, axis=1).astype(bf16)
                out_copy(j, r, c).start()
            return 0

        for j in range(4, NUP):
            start(w1_copies(j))
        wait(bias_copies)
        b1_f[...] = b1_v[...].astype(f32)
        b2_f[...] = b2_v[...].astype(f32)
        with _scope("up"):
            lax.fori_loop(0, NUP // UP_UNROLL, up_chunks, 0)
        with _scope("down"):
            lax.fori_loop(0, NDOWN, down, 0)
        with _scope("out"):
            wait([out_copy(j, r, c) for j in range(NDOWN) for r, c in _QUADS])

    vmem = pltpu.VMEM
    pl.run_scoped(
        spectral,
        vmem((D, S), bf16), vmem((DF, S), bf16), vmem((DF, S), bf16), vmem((D, 6 * D), bf16),
        vmem(_DFT64.shape, i32), vmem(_SEEDS.shape, f32), vmem((1, D), bf16), vmem((8, D), f32),
        vmem((NT, 3, 128, 128), f32), vmem((NT, WROWS, 128), i32), vmem((D, S), f32),
        vmem((4, 4, 2, NL, 128), f32), vmem((NT, NL, 128), f32), vmem((NT, NL, 128), f32),
        vmem((4, 4, 2, NL, 128), f32), vmem((NT, D, 128), f32),
        vmem((D, 128), f32), vmem((4, D, 128), f32), vmem((4, D, 128), f32))
    pl.run_scoped(
        mlp,
        vmem((len(_PAIRS), Q, 256 * NUP), bf16), vmem((NDOWN, 2, 2, H, 256), bf16),
        vmem((F // 128, 128), f32), vmem((NT, 128), f32))


@jax.jit
def pallas_adaLN_cond__spectral_gfnet__mixer_token_mlp__prompt_kernel(A_x, A_w_r, A_w_i, B_x, B_w1, B_b1, B_w2, B_b2, c, w_mod):
    del B_x
    bf16 = jnp.bfloat16
    hbm = pl.BlockSpec(memory_space=pl.ANY)
    out = pl.pallas_call(
        _kernel,
        out_shape=jax.ShapeDtypeStruct((D, S), bf16),
        in_specs=[hbm] * 11,
        out_specs=hbm,
        scratch_shapes=[
            pltpu.VMEM((F // 128, S, 128), bf16),
            pltpu.VMEM((NT, F, 128), bf16),
            pltpu.VMEM((F // 128, 128), bf16),
            pltpu.VMEM((NT, 128), bf16),
            pltpu.VMEM((6 * D, 128), jnp.float32),
            pltpu.VMEM((NT, D, 128), jnp.float32),
            pltpu.VMEM((len(_PAIRS), Q, 256 * NDOWN), bf16),
            pltpu.SMEM((49,), jnp.int32),
            pltpu.SemaphoreType.DMA((10,)),
            pltpu.SemaphoreType.DMA((XCH,)),
            pltpu.SemaphoreType.DMA((NUP,)),
            pltpu.SemaphoreType.DMA((NDOWN,)),
            pltpu.SemaphoreType.DMA((4 * NDOWN,)),
        ],
        compiler_params=pltpu.CompilerParams(vmem_limit_bytes=120 * 1024 * 1024),
    )(A_x.reshape(S, D).T, A_w_r.T, A_w_i.T, B_w1, B_w2, w_mod, _DFT64, _SEEDS,
      B_b1.reshape(F // 128, 128), B_b2.reshape(NT, 128), c)
    return out.T.reshape(1, S, D)
```

```python
import math

import jax
import jax.numpy as jnp
import numpy as np
from jax import lax
import jax.experimental.pallas as pl
import jax.experimental.pallas.tpu as pltpu

S, D, F = 2048, 576, 4608
DF = D // 2 + 1
EPS = 1e-5
NT = S // 128
G0 = 40
NL = 4 * 64 + G0
WROWS = 296
H, Q = D // 2, D // 4
XCH = 8
NUP, NDOWN = F // 512, S // 512
UP_UNROLL = 3

_C9 = [math.cos(2 * math.pi * j / 9) for j in range(9)]
_S9 = [math.sin(2 * math.pi * j / 9) for j in range(9)]


def _classes(r):
    return [r, r + 9, 9 - r, 18 - r] if r else [0, 9]


def _bf16_pairs(m):
    u = np.ascontiguousarray(m, dtype=np.float32).view(np.uint32)
    u = (u + 0x7FFF + ((u >> 16) & 1)) >> 16
    return (u[..., 0::2, :] | (u[..., 1::2, :] << 16)).view(np.int32)


def _constants():
    def by8(re, im):
        n = re.shape[1]
        return np.stack([re.reshape(-1, 8, n), im.reshape(-1, 8, n)], 1).reshape(-1, n)

    d = np.arange(64)
    fwd, inv = np.zeros((5, 128, 128)), np.zeros((5, 128, 128))
    scale = 1.0 / (D * S)
    for r in range(1, 5):
        l = np.array([18 * m + res for res in _classes(r) for m in range(16)])
        angle = 2 * np.pi * np.outer(l, d) / D
        co, si = np.cos(angle), np.sin(angle)
        odd = _S9[3] * np.where(l % 9 == r, 1.0, -1.0)[:, None]
        fwd[r - 1] = by8(np.hstack([co, -odd * si]), np.hstack([-si, -odd * co]))
        inv[r - 1] = 2 * scale * np.block([[co.T, -si.T], [(odd * si).T, (odd * co).T]])
    l = np.array([18 * m + res for res in _classes(0) for m in range(16)] + [D // 2])
    angle = 2 * np.pi * np.outer(l, d) / D
    edge = (l == 0) | (l == D // 2)
    pad = ((0, G0 - len(l)), (0, 0))
    co, si = np.pad(np.cos(angle), pad), np.pad(np.where(edge[:, None], 0.0, np.sin(angle)), pad)
    fwd[4, :2 * G0, :64] = by8(co, -si)
    weight = scale * np.pad(np.where(edge, 1.0, 2.0), pad[0])[None, :]
    inv[4, :64, :2 * G0] = np.hstack([weight * co.T, -weight * si.T])

    b, p = np.arange(8)[:, None], np.arange(128)[None, :]
    first = 128 * (p % 16) + 16 * (p // 16)
    step = -127 + 0 * p
    wrap = step + np.where(p < 16, 112, -16)
    seeds = []
    for rows in (b, b + 8, 16 + 0 * b):
        for k in (first, step, wrap):
            z = np.exp(-2j * np.pi * rows * k / S)
            seeds += [z.real, z.imag]
    return _bf16_pairs(np.concatenate([fwd, inv], 0)), np.concatenate(seeds, 0).astype(np.float32)


_DFT64, _SEEDS = _constants()


def _radix9_even(h0, e1, e2, e3, e4):
    p = h0 + e3
    q = e1 + e2 + e4
    g = h0 - 0.5 * e3
    u, v = e1 - e4, e2 - e4
    a = _C9[1] * u + _C9[2] * v
    b = _C9[2] * u + _C9[4] * v
    return p + q, g + a, g + b, p - 0.5 * q, g - a - b


def _radix9_odd(o1, o2, o3, o4):
    u, v = o1 + o2, o2 + o4
    a = (_S9[1] / _S9[3]) * u + (_S9[4] / _S9[3]) * v
    b = (_S9[2] / _S9[3]) * u - (_S9[1] / _S9[3]) * v
    return a + o3, b - o3, o1 - o2 + o4, b - a + o3


def _radix4(z0, z1, z2, z3, sign):
    ar, ai = z0[0] + z2[0], z0[1] + z2[1]
    br, bi = z0[0] - z2[0], z0[1] - z2[1]
    cr, ci = z1[0] + z3[0], z1[1] + z3[1]
    dr, di = z1[0] - z3[0], z1[1] - z3[1]
    plus, minus = (br - di, bi + dr), (br + di, bi - dr)
    if sign < 0:
        plus, minus = minus, plus
    return (ar + cr, ai + ci), plus, (ar - cr, ai - ci), minus


def _twiddle16(z, n, sign):
    zr, zi = z
    if n == 0:
        return z
    if n == 4:
        return (-zi, zr) if sign > 0 else (zi, -zr)
    c, s = math.cos(2 * math.pi * n / 16), sign * math.sin(2 * math.pi * n / 16)
    if n % 4 == 2:
        if (c > 0) == (s > 0):
            return c * (zr - zi), c * (zr + zi)
        return c * (zr + zi), c * (zi - zr)
    return c * zr - s * zi, c * zi + s * zr


def _cmul(a, b):
    return a[0] * b[0] - a[1] * b[1], a[0] * b[1] + a[1] * b[0]


def _gelu2(x):
    k = math.sqrt(2 / math.pi)
    return x + x * jnp.tanh(x * (k + (k * 0.044715) * (x * x)))


class _Mean:
    def __init__(self):
        self.total = None

    def add(self, piece):
        self.total = piece if self.total is None else self.total + piece

    def value(self):
        return jnp.sum(self.total[0:8] + self.total[8:16], axis=0, keepdims=True) * (1.0 / D)


def _as_bf16(words):
    return pltpu.bitcast(words, jnp.bfloat16)


def _word_half(words, high):
    return pltpu.bitcast(words & jnp.int32(-65536) if high else words << 16, jnp.float32)


def _dot(a, b):
    return jnp.dot(a, b, preferred_element_type=jnp.float32)


def _dot_nt(a, b):
    return lax.dot_general(a, b, (((1,), (1,)), ((), ())), preferred_element_type=jnp.float32)


_QUADS = ((0, 0), (0, 1), (1, 0), (1, 1))
_LEFT = ((((0, 0), 1), ((1, 1), 1)), (((1, 0), 1), ((1, 1), 1)), (((0, 0), 1),), (((1, 1), 1),),
         (((0, 0), 1), ((0, 1), 1)), (((1, 0), 1), ((0, 0), -1)), (((0, 1), 1), ((1, 1), -1)))
_RIGHT = ((((0, 0), 1), ((1, 1), 1)), (((0, 0), 1),), (((0, 1), 1), ((1, 1), -1)), (((1, 0), 1), ((0, 0), -1)),
          (((1, 1), 1),), (((0, 0), 1), ((0, 1), 1)), (((1, 0), 1), ((1, 1), 1)))
_OUTPUT = (((0, 0), ((0, 1), (3, 1), (4, -1), (6, 1))), ((0, 1), ((2, 1), (4, 1))),
           ((1, 0), ((1, 1), (3, 1))), ((1, 1), ((0, 1), (1, -1), (2, 1), (5, 1))))
ORDER_UP = (4, 2, 1, 3, 0, 6, 5)
ORDER_DOWN = (2, 4, 1, 3, 0, 6, 5)
ORDER_IN = (4, 1, 2, 3, 0, 6, 5)
_PAIRS = ([((2, q), (2, min(q + 1, 6))) for q in range(0, 7, 2)] +
          [((a, q), (b, q)) for a, b in ((3, 0), (4, 6), (1, 5)) for q in range(7)])
_PLACE = {op: (n, side) for n, pair in enumerate(_PAIRS) for side, op in ((1, pair[1]), (0, pair[0]))}


def _signed_sum(terms, get):
    total = get(terms[0][0])
    for key, sign in terms[1:]:
        total = total + get(key) if sign > 0 else total - get(key)
    return total


def _left_operands(blocks):
    return [_signed_sum(terms, blocks.get) for terms in _LEFT]


def _paired(pair, inner):
    return jnp.concatenate(
        [_signed_sum(_LEFT[p], lambda rc: inner[rc][q]) for p, q in pair], axis=1).astype(jnp.bfloat16)


def _strassen_level(product, order):
    done = {}
    for n in order:
        done[n] = product(n)
        for (r, c), terms in _OUTPUT:
            if n in dict(terms) and all(k in done for k, _ in terms):
                yield r, c, lambda f, terms=terms: _signed_sum(terms, lambda k: f(done[k]))


def _strassen2(left_ref, right, order):
    def outer(p):
        def inner(q):
            def block(b, c):
                return right(2 * b[0] + c[0], 2 * b[1] + c[1], 7 * p + (q if len(_RIGHT[p]) == 1 else 0))

            if len(_RIGHT[p]) == 1 and len(_RIGHT[q]) == 1:
                rhs = block(_RIGHT[p][0][0], _RIGHT[q][0][0])
            else:
                rhs = _signed_sum(_RIGHT[q], lambda c: _signed_sum(
                    _RIGHT[p], lambda b: block(b, c).astype(jnp.float32))).astype(jnp.bfloat16)
            n, side = _PLACE[p, q]
            lhs = jnp.concatenate(
                [left_ref[n, :, k + 128 * side:k + 128 * (side + 1)] for k in range(0, left_ref.shape[2], 256)],
                axis=1)
            return _dot(lhs, rhs)

        return {(r, c): combine(lambda m: m) for r, c, combine in _strassen_level(inner, ORDER_IN)}

    for r, c, combine in _strassen_level(outer, order):
        yield r, c, {rc: combine(lambda m: m[rc]) for rc in _QUADS}


def _kernel(x_hbm, wr_hbm, wi_hbm, w1_hbm, w2_hbm, wm_hbm, f_hbm, seed_hbm, b1_hbm, b2_hbm, c_hbm,
            out_hbm,
            w1_v, w2_v, b1_v, b2_v, mod_v, x1_v, a1_v, zero_s, sem_in, sem_x, sem_w1, sem_w2, sem_out):
    f32, bf16, i32 = jnp.float32, jnp.bfloat16, jnp.int32

    def tile_copies(src, dst, sem, j):
        return [pltpu.make_async_copy(src.at[:, pl.ds(pl.multiple_of((4 * j + t) * 128, 128), 128)],
                                      dst.at[4 * j + t], sem.at[j]) for t in range(4)]

    def w1_copies(j):
        return tile_copies(w1_hbm, w1_v, sem_w1, j)

    def w2_copies(j):
        return tile_copies(w2_hbm, w2_v, sem_w2, j)

    def start(copies):
        for copy in copies:
            copy.start()

    def wait(copies):
        for copy in copies:
            copy.wait()

    bias_copies = [pltpu.make_async_copy(b1_hbm, b1_v, sem_in.at[0]),
                   pltpu.make_async_copy(b2_hbm, b2_v, sem_in.at[1])]

    def mod_col(which, row, n=16):
        return mod_v[which * D + row:which * D + row + n, :]

    def spectral(x_v, wr_v, wi_v, wm_v, f_v, seed_v, c_v, act_v, g_v, wp_v, t_v, u_v, xr_v, xi_v, v_v, p_v,
                 ts_v, e_v, h_v):
        def x_copy(i):
            cols = pl.ds(pl.multiple_of(i * (S // XCH), S // XCH), S // XCH)
            return pltpu.make_async_copy(x_hbm.at[:, cols], x_v.at[:, cols], sem_x.at[i])

        seed_copy, c_copy, f_copy, wr_copy, wi_copy = [
            pltpu.make_async_copy(src, dst, sem_in.at[2 + i]) for i, (src, dst) in enumerate(
                ((seed_hbm, seed_v), (c_hbm, c_v), (f_hbm, f_v), (wr_hbm, wr_v), (wi_hbm, wi_v)))]
        mod_cols = ((512, 2 * D), (0, 512), (2 * D, 6 * D))
        wm_copies = [pltpu.make_async_copy(wm_hbm.at[:, lo:hi], wm_v.at[:, lo:hi], sem_in.at[7 + i])
                     for i, (lo, hi) in enumerate(mod_cols)]

        start([seed_copy, c_copy, wm_copies[0], x_copy(0)])
        for i in range(49):
            zero_s[i] = 0

        lane = lax.broadcasted_iota(i32, (8, 128), 1)
        seed_copy.wait()
        x_copy(1).start()
        seeds = [(seed_v[16 * i:16 * i + 8, :], seed_v[16 * i + 8:16 * i + 16, :]) for i in range(9)]
        for half in range(2):
            first, step, wrap = seeds[3 * half:3 * half + 3]
            for i in range(8):
                rows = slice(16 * i + 8 * half, 16 * i + 8 * half + 8)
                g = first
                for k1 in range(NT):
                    g_v[k1, 0, rows, :], g_v[k1, 1, rows, :], g_v[k1, 2, rows, :] = g[0], g[1] - g[0], g[1] + g[0]
                    if k1 + 1 < NT:
                        at = (lane & 15) == k1
                        g = _cmul(g, (jnp.where(at, wrap[0], step[0]), jnp.where(at, wrap[1], step[1])))
                if i < 7:
                    first, step, wrap = [_cmul(z, w) for z, w in zip((first, step, wrap), seeds[6:])]

        def modulation(part):
            lo, hi = mod_cols[part]
            row = _dot(act_v[...], wm_v[:, lo:hi])
            for t in range(0, hi - lo, 128):
                mod_v[lo + t:lo + t + 128, :] = jnp.broadcast_to(row[0:1, t:t + 128], (128, 128)).T

        c_copy.wait()
        x_copy(2).start()
        cond = c_v[...].astype(f32)
        act_v[...] = jnp.broadcast_to(cond * jax.nn.sigmoid(cond), (8, D))
        wm_copies[0].wait()
        x_copy(3).start()
        modulation(0)
        mod_v[D:2 * D, :] = 1.0 + mod_v[D:2 * D, :]

        def radix9_forward(dst, cols, piece):
            for i in range(0, 64, 16):
                h = [piece(64 * a + i) for a in range(9)]
                even = _radix9_even(h[0], *[h[a] + h[9 - a] for a in range(1, 5)])
                odd = _radix9_odd(*[h[a] - h[9 - a] for a in range(1, 5)])
                dst[512 + i:512 + i + 16, cols] = even[0]
                for r in range(4):
                    dst[128 * r + i:128 * r + i + 16, cols] = even[r + 1]
                    dst[128 * r + 64 + i:128 * r + 64 + i + 16, cols] = odd[r]

        def first_norm(i, _):
            x_copy(i).wait()
            pl.when(i + 4 < XCH)(lambda: x_copy(i + 4).start())
            for n, copy in enumerate((f_copy, wr_copy, wi_copy, wm_copies[1])):
                pl.when(i == XCH - 4 + n)(copy.start)
            tiles = range(NT // XCH)
            cols = [pl.ds(pl.multiple_of((i * len(tiles) + n) * 128, 128), 128) for n in tiles]
            mean, var = [_Mean() for _ in tiles], [_Mean() for _ in tiles]
            for n in tiles:
                for row in range(0, D, 16):
                    mean[n].add(x_v[row:row + 16, cols[n]].astype(f32))
            for n in tiles:
                m = mean[n].value()
                for row in range(0, D, 16):
                    d = x_v[row:row + 16, cols[n]].astype(f32) - m
                    e_v[n, row:row + 16, :] = d
                    var[n].add(d * d)
            for n in tiles:
                scale = lax.rsqrt(var[n].value() + EPS)
                radix9_forward(t_v, cols[n], lambda row: e_v[n, row:row + 16, :] * scale * mod_col(1, row))
            return 0

        lax.fori_loop(0, XCH, first_norm, 0)

        def d_forward(r, rhs):
            if r < 4:
                return _dot(_as_bf16(f_v[r]), rhs(slice(128 * r, 128 * r + 128)).astype(bf16))
            return _dot(_as_bf16(f_v[4, 0:G0, 0:64]), rhs(slice(512, D)).astype(bf16))

        def group_rows(r):
            return range(0, 64 if r < 4 else G0, 8)

        f_copy.wait()
        start([wm_copies[2]] + bias_copies)
        for r in range(5):
            for a1 in range(4):
                z = d_forward(r, lambda rows: jnp.concatenate(
                    [t_v[rows, 128 * a:128 * a + 128] for a in range(a1, NT, 4)], axis=1))
                for i in group_rows(r):
                    u = _radix4(*[(z[2 * i:2 * i + 8, t:t + 128], z[2 * i + 8:2 * i + 16, t:t + 128])
                                  for t in range(0, 512, 128)], -1)
                    rows = slice(64 * r + i, 64 * r + i + 8)
                    for q1 in range(4):
                        u_v[a1, q1, 0, rows, :], u_v[a1, q1, 1, rows, :] = _twiddle16(u[q1], a1 * q1, -1)

        def s_forward(q1):
            y = _radix4(*[(u_v[a1, q1, 0], u_v[a1, q1, 1]) for a1 in range(4)], -1)
            for q2, (yr, yi) in enumerate(y):
                k1 = q1 + 4 * q2
                both, real, imag = [_dot(v, g_v[k1, n].astype(bf16)) for n, v in enumerate((yr + yi, yr, yi))]
                xr_v[k1], xi_v[k1] = both - imag, both + real

        def regroup(tiles, row):
            a = [None] * NT
            for c in range(NT):
                a[-c % NT] = pltpu.roll(tiles[c], c, 1) if c else tiles[c]
            for bit in range(4):
                take = ((lane >> bit) & 1) == 1
                a = [jnp.where(take, a[(m - (1 << bit)) % NT], a[m]) for m in range(NT)]
            for k1 in range(NT):
                wp_v[k1, row:row + 8, :] = a[k1]

        s_forward(0)
        s_forward(1)
        wait([wr_copy, wi_copy])
        start(w1_copies(0))
        for i in range(18):
            for src, base in ((wr_v, 0), (wi_v, 144)):
                regroup([pltpu.bitcast(src[16 * i:16 * i + 16, t:t + 128], i32) for t in range(0, S, 128)],
                        base + 8 * i)
        last = []
        for t in range(0, S, 128):
            low, high = [pltpu.bitcast(jnp.broadcast_to(w[DF - 1:DF, t:t + 128].astype(f32), (8, 128)), i32)
                         for w in (wr_v, wi_v)]
            last.append(lax.shift_right_logical(low, 16) | high)
        regroup(last, 288)
        s_forward(2)
        s_forward(3)

        def s_inverse(q1, shift=None):
            q = []
            for k1 in range(q1, NT, 4):
                wr, wi = [jnp.concatenate(
                    [_word_half(wp_v[k1, pl.ds(base + res // 2, 16, stride=9), :], res % 2)
                     for r in (1, 2, 3, 4, 0) for res in _classes(r)] +
                    [_word_half(wp_v[k1, 288:296, :], base > 0)], axis=0) for base in (0, 144)]
                xr, xi = xr_v[k1], xi_v[k1]
                if k1 == 0:
                    xr, xi = xr + shift[0], xi + shift[1]
                fr, fi = _cmul((xr, xi), (wr, wi))
                both, imag, real = [_dot_nt(v, g_v[k1, n].astype(bf16)) for n, v in enumerate((fr + fi, fi, fr))]
                q.append((both + imag, both - real))
            for a1, u in enumerate(_radix4(*q, +1)):
                v_v[a1, q1, 0], v_v[a1, q1, 1] = _twiddle16(u, a1 * q1, +1)

        wm_copies[1].wait()
        start(w1_copies(1))
        modulation(1)
        s_inverse(3)
        radix9_forward(ts_v, slice(None), lambda row: mod_col(0, row))
        shift = ([], [])
        for r in range(5):
            z = d_forward(r, lambda rows: ts_v[rows, :])
            for i in group_rows(r):
                for part in range(2):
                    row = 2 * i + 8 * part
                    shift[part].append(jnp.where(lane == 0, z[row:row + 8] * float(S), 0.0))
        s_inverse(2)
        s_inverse(1)
        s_inverse(0, [jnp.concatenate(part, axis=0) for part in shift])

        wm_copies[2].wait()
        start(w1_copies(2))
        modulation(2)
        for r in range(5):
            rows = slice(64 * r, 64 * r + 64 if r < 4 else NL)
            for a1 in range(4):
                v = _radix4(*[(v_v[a1, q1, 0, rows, :], v_v[a1, q1, 1, rows, :]) for q1 in range(4)], +1)
                rhs = jnp.concatenate([jnp.concatenate(pair, axis=0) for pair in v], axis=1).astype(bf16)
                p = _dot(_as_bf16(f_v[5 + r] if r < 4 else f_v[9, 0:32, 0:2 * G0]), rhs)
                for a2 in range(4):
                    p_v[a1 + 4 * a2, 128 * r:128 * r + p.shape[0], :] = p[:, 128 * a2:128 * a2 + 128]
        mod_v[4 * D:5 * D, :] = 1.0 + mod_v[4 * D:5 * D, :]
        shifts, mean = [mod_col(3, row) for row in range(0, D, 16)], _Mean()
        for piece in shifts:
            mean.add(piece)
        mean = mean.value()
        for i, piece in enumerate(shifts):
            mod_v[3 * D + 16 * i:3 * D + 16 * i + 16, :] = piece - mean

        def residual(t):
            cols = pl.ds(pl.multiple_of(t * 128, 128), 128)
            mean = _Mean()
            for i in range(0, 64, 16):
                even = _radix9_even(*[p_v[t, row + i:row + i + 16, :] for row in (512, 0, 128, 256, 384)])
                odd = _radix9_odd(*[p_v[t, row + i:row + i + 16, :] for row in (64, 192, 320, 448)])
                for a in range(9):
                    y = even[0] if a == 0 else even[a] - odd[a - 1] if a < 5 else even[9 - a] + odd[8 - a]
                    row = 64 * a + i
                    x1 = x_v[row:row + 16, cols].astype(f32) + mod_col(2, row) * y
                    x1_v[t, row:row + 16, :] = x1
                    mean.add(x1)
            return mean

        def second_norm(t, slot, m):
            var, mean = _Mean(), _Mean()
            for row in range(0, D, 16):
                d = x1_v[t, row:row + 16, :] - m
                e = d * mod_col(4, row)
                e_v[slot, row:row + 16, :] = e
                var.add(d * d)
                mean.add(e)
            return var, mean

        def third_norm(slot, scale, m):
            var = _Mean()
            for row in range(0, D, 16):
                d = (e_v[slot, row:row + 16, :] - m) * scale + mod_col(3, row)
                h_v[slot, row:row + 16, :] = d
                var.add(d * d)
            return var

        def mlp_operands(t, _):
            scales = []
            for slots in ((0, 1), (2, 3)):
                means = [residual(4 * t + k) for k in slots]
                stats = [second_norm(4 * t + k, k, m.value()) for k, m in zip(slots, means)]
                spread = [third_norm(k, lax.rsqrt(v.value() + EPS), m.value()) for k, (v, m) in zip(slots, stats)]
                scales += [lax.rsqrt(v.value() + EPS) for v in spread]
            cols = pl.ds(pl.multiple_of(t * 256, 256), 256)
            for i in range(0, Q, 16):
                inner = {(r, c): _left_operands({
                    (r2, c2): h_v[2 * c + c2, (2 * r + r2) * Q + i:(2 * r + r2) * Q + i + 16, :] * scales[2 * c + c2]
                    for r2, c2 in _QUADS}) for r, c in _QUADS}
                for n, pair in enumerate(_PAIRS):
                    a1_v[n, i:i + 16, cols] = _paired(pair, inner)
            return 0

        start(w1_copies(3))
        lax.fori_loop(0, NT // 4, mlp_operands, 0)

    def mlp(a2_v, out_v, b1_f, b2_f):
        def weight_block(ref, tile, kq, tag):
            words = ref.bitcast(i32)
            return _as_bf16(jnp.concatenate(
                [words[tile + zero_s[tag], row + 64 * kq:row + 64 * kq + 64, :]
                 for row in range(0, words.shape[1], 256)], axis=0))

        def up(j):
            cols = pl.ds(pl.multiple_of(j * 256, 256), 256)
            inner, todo = {}, list(enumerate(_PAIRS))
            for r, c, u in _strassen2(a1_v, lambda kq, nq, tag: weight_block(w1_v, 4 * j + nq, kq, tag), ORDER_UP):
                inner[r, 1 - c] = _left_operands({
                    (r2, 1 - c2): _gelu2(u[r2, c2] + b1_f[pl.ds(4 * j + 2 * c + c2, 1), :]) for r2, c2 in _QUADS})
                for n, pair in list(todo):
                    if all(rc in inner for p, _ in pair for rc, _ in _LEFT[p]):
                        todo.remove((n, pair))
                        a2_v[n, :, cols] = _paired(pair, inner)

        def up_chunks(step, _):
            @pl.when(step == 1)
            def _():
                for j in range(NDOWN):
                    start(w2_copies(j))

            for n in range(UP_UNROLL):
                wait(w1_copies(step * UP_UNROLL + n))
            for n in range(UP_UNROLL):
                up(step * UP_UNROLL + n)
            return 0

        def out_copy(j, r, c):
            cols = pl.ds(pl.multiple_of(j * 512 + c * 256, 256), 256)
            return pltpu.make_async_copy(out_v.at[j, r, c], out_hbm.at[pl.ds(r * H, H), cols],
                                         sem_out.at[4 * j + 2 * r + c])

        def down(j, _):
            wait(w2_copies(j))
            for r, c, y in _strassen2(
                    a2_v, lambda kq, nq, tag: weight_block(w2_v, 4 * j + nq, 3 - kq, tag), ORDER_DOWN):
                for r2 in range(2):
                    row = (2 * r + r2) * Q
                    tiles = []
                    for c2 in range(2):
                        tile = 4 * j + 2 * c + c2
                        mixed = 0.5 * y[r2, c2] + b2_f[pl.ds(tile, 1), :]
                        tiles.append(x1_v[tile, row:row + Q, :] + mod_col(5, row, Q) * mixed)
                    out_v[j, r, c, r2 * Q:(r2 + 1) * Q, :] = jnp.concatenate(tiles, axis=1).astype(bf16)
                out_copy(j, r, c).start()
            return 0

        for j in range(4, NUP):
            start(w1_copies(j))
        wait(bias_copies)
        b1_f[...] = b1_v[...].astype(f32)
        b2_f[...] = b2_v[...].astype(f32)
        lax.fori_loop(0, NUP // UP_UNROLL, up_chunks, 0)
        lax.fori_loop(0, NDOWN, down, 0)
        wait([out_copy(j, r, c) for j in range(NDOWN) for r, c in _QUADS])

    vmem = pltpu.VMEM
    pl.run_scoped(
        spectral,
        vmem((D, S), bf16), vmem((DF, S), bf16), vmem((DF, S), bf16), vmem((D, 6 * D), bf16),
        vmem(_DFT64.shape, i32), vmem(_SEEDS.shape, f32), vmem((1, D), bf16), vmem((8, D), f32),
        vmem((NT, 3, 128, 128), f32), vmem((NT, WROWS, 128), i32), vmem((D, S), f32),
        vmem((4, 4, 2, NL, 128), f32), vmem((NT, NL, 128), f32), vmem((NT, NL, 128), f32),
        vmem((4, 4, 2, NL, 128), f32), vmem((NT, D, 128), f32),
        vmem((D, 128), f32), vmem((4, D, 128), f32), vmem((4, D, 128), f32))
    pl.run_scoped(
        mlp,
        vmem((len(_PAIRS), Q, 256 * NUP), bf16), vmem((NDOWN, 2, 2, H, 256), bf16),
        vmem((F // 128, 128), f32), vmem((NT, 128), f32))


@jax.jit
def pallas_adaLN_cond__spectral_gfnet__mixer_token_mlp__prompt_kernel(
    A_x, A_w_r, A_w_i, B_x, B_w1, B_b1, B_w2, B_b2, c, w_mod,
):
    del B_x
    bf16 = jnp.bfloat16
    hbm = pl.BlockSpec(memory_space=pl.ANY)
    out = pl.pallas_call(
        _kernel,
        out_shape=jax.ShapeDtypeStruct((D, S), bf16),
        in_specs=[hbm] * 11,
        out_specs=hbm,
        scratch_shapes=[
            pltpu.VMEM((F // 128, S, 128), bf16),
            pltpu.VMEM((NT, F, 128), bf16),
            pltpu.VMEM((F // 128, 128), bf16),
            pltpu.VMEM((NT, 128), bf16),
            pltpu.VMEM((6 * D, 128), jnp.float32),
            pltpu.VMEM((NT, D, 128), jnp.float32),
            pltpu.VMEM((len(_PAIRS), Q, 256 * NDOWN), bf16),
            pltpu.SMEM((49,), jnp.int32),
            pltpu.SemaphoreType.DMA((10,)),
            pltpu.SemaphoreType.DMA((XCH,)),
            pltpu.SemaphoreType.DMA((NUP,)),
            pltpu.SemaphoreType.DMA((NDOWN,)),
            pltpu.SemaphoreType.DMA((4 * NDOWN,)),
        ],
        compiler_params=pltpu.CompilerParams(vmem_limit_bytes=120 * 1024 * 1024),
    )(A_x.reshape(S, D).T, A_w_r.T, A_w_i.T, B_w1, B_w2, w_mod, _DFT64, _SEEDS,
      B_b1.reshape(F // 128, 128), B_b2.reshape(NT, 128), c)
    return out.T.reshape(1, S, D)
```
